```python
import jax
import jax.numpy as jnp

def _softmax(x, axis=-1):
    return jax.nn.softmax(x, axis=axis)

def _gelu(x):
    return jax.nn.gelu(x, approximate=True)

def _silu(x):
    return jax.nn.silu(x)

def _sigmoid(x):
    return jax.nn.sigmoid(x)

def _layernorm(x, axis=-1, eps=1e-05):
    m = jnp.mean(x, axis=axis, keepdims=True)
    v = jnp.var(x, axis=axis, keepdims=True)
    return (x - m) / jnp.sqrt(v + eps)

def _scatter_add(tgt, idx, src, axis=0):
    return tgt.at[idx].add(src)

def _segment_sum(src, seg, n):
    return jax.ops.segment_sum(src, seg, n)

class _Rng:

    def __init__(self, key):
        self._k = key

    def _next(self):
        self._k, sub = jax.random.split(self._k)
        return sub

    def normal(self, shape):
        return jax.random.normal(self._next(), shape, dtype=jnp.bfloat16)

    def randint(self, lo, hi, shape):
        return jax.random.randint(self._next(), shape, lo, hi, dtype=jnp.int32)

    def uniform(self, shape, lo=0.0, hi=1.0):
        return jax.random.uniform(self._next(), shape, jnp.bfloat16, lo, hi)

    def permutation(self, n):
        return jax.random.permutation(self._next(), n)
kernel_name = 'adaLN_cond__ssm_conv_h3__glu_gated_swiglu__prompt'

def setup_inputs():
    _rng = _Rng(jax.random.key(int.from_bytes(__import__("os").urandom(4), "little")))
    _w = lambda a: (lambda t: t.astype(jnp.bfloat16) if jnp.issubdtype(t.dtype, jnp.floating) else t)(jnp.asarray(a))

    def _A_setup():
        B, S, D = (1, 2048, 640)
        ks = 4
        return {'q': _w((lambda *s: _rng.normal(s) * 0.05)(B, S, D)), 'k': _w((lambda *s: _rng.normal(s) * 0.05)(B, S, D)), 'v': _w((lambda *s: _rng.normal(s) * 0.05)(B, S, D)), 'shift_k': _w((lambda *s: _rng.normal(s) * 0.05)(D, ks) * 0.5), 'ssm_k': _w((lambda *s: _rng.normal(s) * 0.05)(D, S) * (1.0 / S ** 0.5)), 'ssm_D': _w((lambda *s: _rng.normal(s) * 0.05)(D))}
    _A_in = _A_setup()

    def _B_setup():
        B, S, D, F = (1, 2048, 640, 1536)
        return {'x': _w((lambda *s: _rng.normal(s) * 0.05)(B, S, D)), 'w1': _w((lambda *s: _rng.normal(s) * 0.05)(D, F) * (2.0 / D) ** 0.5), 'w3': _w((lambda *s: _rng.normal(s) * 0.05)(D, F) * (2.0 / D) ** 0.5), 'w2': _w((lambda *s: _rng.normal(s) * 0.05)(F, D) * (2.0 / F) ** 0.5)}
    _B_in = _B_setup()
    return {'A_q': _A_in['q'], 'A_k': _A_in['k'], 'A_v': _A_in['v'], 'A_shift_k': _A_in['shift_k'], 'A_ssm_k': _A_in['ssm_k'], 'A_ssm_D': _A_in['ssm_D'], 'B_x': _B_in['x'], 'B_w1': _B_in['w1'], 'B_w3': _B_in['w3'], 'B_w2': _B_in['w2'], 'c': _w((lambda *s: _rng.normal(s) * 0.05)(1, 640)), 'w_mod': _w((lambda *s: _rng.normal(s) * 0.05)(640, 6 * 640) * 640 ** (-0.5))}

def reference(A_q, A_k, A_v, A_shift_k, A_ssm_k, A_ssm_D, B_x, B_w1, B_w3, B_w2, c, w_mod):

    def _A_ref(q, k, v, shift_k, ssm_k, ssm_D):
        B, S, D = q.shape
        ks = shift_k.shape[-1]
        k_pad = jnp.pad(k, ((0, 0), (ks - 1, 0), (0, 0)))
        k_shift = jnp.zeros_like(k)
        for t in range(ks):
            k_shift = k_shift + k_pad[:, t:t + S, :] * shift_k[:, ks - 1 - t][None, None, :]
        kv = k_shift * v
        L = 2 * S
        kv_pad = jnp.pad(kv, ((0, 0), (0, S), (0, 0)))
        kf_pad = jnp.pad(ssm_k, ((0, 0), (0, S)))
        kv_f = (lambda x, axes=(-2, -1): jnp.fft.rfft2(x.astype(jnp.float32), axes=axes))(kv_pad[:, None, :, :], axes=(1, 2))
        kf_f = (lambda x, axes=(-2, -1): jnp.fft.rfft2(x.astype(jnp.float32), axes=axes))(kf_pad[:, None, :], axes=(1, 2))
        kf_f = (lambda x, *d: x.transpose(*d))(kf_f, 1, 2, 0)
        y_f = kv_f * kf_f[None, :, :, :]
        y = (lambda x, s, axes=(-2, -1): jnp.fft.irfft2(x, s=s, axes=axes).astype(jnp.bfloat16))(y_f, (1, L), axes=(1, 2))[:, 0, :S, :]
        y = y + kv * ssm_D[None, None, :]
        return q * y

    def _B_ref(x, w1, w3, w2):
        gate = jnp.einsum('bsd,df->bsf', x, w1)
        up = jnp.einsum('bsd,df->bsf', x, w3)
        h = _silu(gate) * up
        out = jnp.einsum('bsf,fd->bsd', h, w2)
        return out
    x = A_q
    mod = (_silu(c) @ w_mod).reshape(c.shape[0], 6, 1, -1)
    sa, ca, ga, sb, cb, gb = (mod[:, 0].copy(), mod[:, 1].copy(), mod[:, 2].copy(), mod[:, 3].copy(), mod[:, 4].copy(), mod[:, 5].copy())
    h = _layernorm(x, axis=-1) * (1 + ca) + sa
    x = x + ga * _A_ref(h, A_k, A_v, A_shift_k, A_ssm_k, A_ssm_D)
    h = _layernorm(x, axis=-1) * (1 + cb) + sb
    x = x + gb * _B_ref(h, B_w1, B_w3, B_w2)
    return x
```

```python
import functools, os
import numpy as np
import jax
import jax.numpy as jnp
from jax.experimental import pallas as pl
from jax.experimental.pallas import tpu as pltpu

S, D, FF = 2048, 640, 1536
CH = 128
NCH = S // CH
BM = 256
NST = S // BM
FC = 512
EPS = 1e-5
KPAD = 64
RB = 8
KR = int(os.environ.get('KR', 32))
LR = int(os.environ.get('LR', 16))
f32, bf16 = jnp.float32, jnp.bfloat16
SKIP = os.environ.get('SKIP', '')
GPAT = os.environ.get('GPAT', '1')
NCS = int(os.environ.get('NCS', 6))
NBS = int(os.environ.get('NBS', 2))
C0 = int(os.environ.get('C0', 1))


def _dft_consts():
    f = np.concatenate([np.arange(0, CH, 2), np.arange(1, CH, 2)])
    n = np.arange(CH)
    th = np.pi * (2 * f[:, None] + 1) * n[None, :] / (2 * CH)
    fm = np.concatenate([np.cos(th), -np.sin(th)], axis=0)
    gm = fm.T / CH
    return fm.astype(np.float32), gm.astype(np.float32)


def _schedule(pro_chunks=4, steps=6, T=21):
    done = set(); touched = set()
    def mk(u, j):
        s = u + j
        src = s + 1 if s in touched else 0
        touched.add(s); done.add((u, j))
        return (u, j, s + 1, src)
    pro = [mk(u, s - u) for s in range(pro_chunks) for u in range(s + 1)]
    table = []
    for i in range(1, steps + 1):
        n = 2 * i + 4
        avail = sorted((u + j, u, j) for u in range(n) for j in range(n)
                       if u + j < NCH and (u, j) not in done)
        pick = avail[:T]
        assert len(pick) == T
        table.append([mk(u, j) for s, u, j in pick])
        for s in range(2 * i + 4):
            assert all((u, s - u) in done for u in range(s + 1))
    assert len(done) == NCH * (NCH + 1) // 2
    return pro, table

PRO_TERMS, TABLE = _schedule()
T_SLOTS = len(TABLE[0])
N_CSTEPS = len(TABLE)


def _kernel(q_hbm, k_hbm, v_hbm, sk_ref, ssm_hbm, dd_ref, w1_hbm, w3_hbm, w2_hbm, c_ref, wm_hbm,
            fm_ref, gm_ref,
            o_ref,
            mod_s, skt_s, q_s, k_s, v_s, ssm_s, wm_s, w1_s, w3_s, w2_s,
            xf, hf, pp, kv_s, yy_s, y_s, h2a, h2b, x1a, x1b, tbl, sems):
    step = pl.program_id(0)

    NG = NST
    def cp_q(g): return pltpu.make_async_copy(q_hbm.at[0, pl.ds(g * BM, BM), :], q_s.at[pl.ds(g * BM, BM), :], sems.at[0 * NG + g])
    def cp_k(g): return pltpu.make_async_copy(k_hbm.at[0, pl.ds(g * BM, BM), :], k_s.at[pl.ds(KPAD + g * BM, BM), :], sems.at[1 * NG + g])
    def cp_v(g): return pltpu.make_async_copy(v_hbm.at[0, pl.ds(g * BM, BM), :], v_s.at[pl.ds(g * BM, BM), :], sems.at[2 * NG + g])
    def cp_s(g): return pltpu.make_async_copy(ssm_hbm.at[:, pl.ds(g * BM, BM)], ssm_s.at[g], sems.at[3 * NG + g])
    NFC = FF // FC
    SB = 4 * NG
    def cp_wm(p): return pltpu.make_async_copy(wm_hbm.at[:, pl.ds(p * D, D)], wm_s.at[:, pl.ds(p * D, D)], sems.at[SB + p])
    def cp_w1(c): return pltpu.make_async_copy(w1_hbm.at[:, pl.ds(c * FC, FC)], w1_s.at[:, pl.ds(c * FC, FC)], sems.at[SB + 6 + c])
    def cp_w3(c): return pltpu.make_async_copy(w3_hbm.at[:, pl.ds(c * FC, FC)], w3_s.at[:, pl.ds(c * FC, FC)], sems.at[SB + 6 + NFC + c])
    def cp_w2(c): return pltpu.make_async_copy(w2_hbm.at[pl.ds(c * FC, FC), :], w2_s.at[pl.ds(c * FC, FC), :], sems.at[SB + 6 + 2 * NFC + c])

    in_reg = [False]
    def al(x, m):
        return x if isinstance(x, int) else pl.multiple_of(x, m)

    def kv_piece(g, r):
        if 'k' in SKIP and not isinstance(g, int): return
        r0 = al(g * BM + r, KR)
        kw = k_s[pl.ds(al(r0 + (KPAD - 16), 16), KR + 16), :].astype(f32)
        ks = kw[16:, :] * skt_s[0:1, :]
        for j in range(1, 4):
            ks = ks + kw[16 - j:16 - j + KR, :] * skt_s[j:j + 1, :]
        kv_s[r:r + KR, :] = (ks * v_s[pl.ds(r0, KR), :].astype(f32)).astype(bf16)

    def x_dot(g, h):
        if 'x' in SKIP and not isinstance(g, int): return
        xf[2 * g + h] = jnp.dot(fm_ref[...], kv_s[h * CH:(h + 1) * CH, :], preferred_element_type=f32)

    def h_dot(g, h):
        if 'h' in SKIP and not isinstance(g, int): return
        hc = ssm_s[g, :, h * CH:(h + 1) * CH]
        hf[2 * g + h] = jax.lax.dot_general(fm_ref[...], hc, (((1,), (1,)), ((), ())), preferred_element_type=f32)

    def d_tasks(g):
        t = [(100, functools.partial(h_dot, g, 0)), (100, functools.partial(h_dot, g, 1))]
        for h in range(2):
            for r in range(h * CH, (h + 1) * CH, KR):
                t.append((280, functools.partial(kv_piece, g, r)))
            t.append((100, functools.partial(x_dot, g, h)))
        return t

    def term_piece(u, j, dst, src, r):
        xr = xf[u, r:r + RB, :]; xi = xf[u, CH + r:CH + r + RB, :]
        hr = hf[j, r:r + RB, :]; hi = hf[j, CH + r:CH + r + RB, :]
        pr = pp[src, r:r + RB, :]; pi = pp[src, CH + r:CH + r + RB, :]
        nr = pr + (xr * hr - xi * hi)
        ni = pi + (xr * hi + xi * hr)
        pp[dst, r:r + RB, :] = nr
        pp[dst, CH + r:CH + r + RB, :] = ni

    cache = {}
    def dyn_piece(row, t, r):
        if 'c' in SKIP: return
        b = (row * T_SLOTS + t) * 4
        k = r // RB
        if GPAT[k % len(GPAT)] == '1' or k == 0:
            cache['idx'] = (tbl[b], tbl[b + 1], tbl[b + 2], tbl[b + 3])
        term_piece(*cache['idx'], r)

    H = CH // 2
    def yy_piece(g, h, r):
        if 'y' in SKIP and not isinstance(g, int): return
        n = 2 * g + h
        cre = pp[n + 1, r:r + 16, :]; pim = pp[n, CH + r:CH + r + 16, :]
        cim = pp[n + 1, CH + r:CH + r + 16, :]; pre = pp[n, r:r + 16, :]
        if r < H:
            a = cre - pim; b = cim + pre
        else:
            a = cre + pim; b = cim - pre
        yy_s[h, r:r + 16, :] = a.astype(bf16)
        yy_s[h, CH + r:CH + r + 16, :] = b.astype(bf16)

    def inv_dot(h):
        if 'i' in SKIP and in_reg[0]: return
        y_s[h * CH:(h + 1) * CH, :] = jnp.dot(gm_ref[...], yy_s[h], preferred_element_type=f32)

    def _ln(x):
        m = jnp.mean(x, axis=-1, keepdims=True)
        xc = x - m
        v = jnp.mean(xc * xc, axis=-1, keepdims=True)
        return xc * jax.lax.rsqrt(v + EPS)

    def ln_piece(g, r, h2_dst, x1_dst):
        if 'l' in SKIP and not isinstance(g, int): return
        x = q_s[pl.ds(al(g * BM + r, LR), LR), :].astype(f32)
        y = y_s[r:r + LR, :]
        sa = mod_s[0:1, 0 * D:1 * D]; ca = mod_s[0:1, 1 * D:2 * D]; ga = mod_s[0:1, 2 * D:3 * D]
        sb = mod_s[0:1, 3 * D:4 * D]; cb = mod_s[0:1, 4 * D:5 * D]
        h1 = _ln(x) * (1.0 + ca) + sa
        x1 = x + ga * (h1 * y)
        h2 = _ln(x1) * (1.0 + cb) + sb
        x1_dst[r:r + LR, :] = x1
        h2_dst[r:r + LR, :] = h2.astype(bf16)

    def b_tasks(g, h2_dst, x1_dst):
        t = []
        for h in range(2):
            for r in range(0, CH, 16):
                t.append((40, functools.partial(yy_piece, g, h, r)))
            t.append((100, functools.partial(inv_dot, h)))
        for r in range(0, BM, LR):
            t.append((200, functools.partial(ln_piece, g, r, h2_dst, x1_dst)))
        return t

    def ffn(h2_src, x1_src, slots, pre=None):
        def emit(k):
            for _, th in slots[k]:
                th()
        if pre is None: pre = lambda k: None
        emit(0)
        h2 = h2_src[...]
        acc = None
        for c in range(FF // FC):
            pre(3 * c)
            g = jnp.dot(h2, w1_s[:, c * FC:(c + 1) * FC], preferred_element_type=f32); emit(3 * c + 1)
            pre(3 * c + 1)
            u = jnp.dot(h2, w3_s[:, c * FC:(c + 1) * FC], preferred_element_type=f32)
            hg = 0.5 * g
            hh = ((hg + hg * jnp.tanh(hg)) * u).astype(bf16); emit(3 * c + 2)
            pre(3 * c + 2)
            p = jnp.dot(hh, w2_s[c * FC:(c + 1) * FC, :], preferred_element_type=f32); emit(3 * c + 3)
            acc = p if acc is None else acc + p
        pre(9)
        gb = mod_s[0:1, 5 * D:6 * D]
        o_ref[0] = (x1_src[...] + gb * acc).astype(o_ref.dtype)

    def split(tasks, n):
        tot = sum(c for c, _ in tasks); out = [[] for _ in range(n)]; acc = 0.0
        for c, th in tasks:
            k = min(n - 1, int((acc + 0.5 * c) * n / tot)); out[k].append((c, th)); acc += c
        return out

    def rotate():
        in_reg[0] = True
        if 'r' in SKIP: return
        h2a[...] = h2b[...]
        x1a[...] = x1b[...]

    def mod_part(p):
        c = c_ref[...].astype(f32)
        sc = (c * jax.nn.sigmoid(c)).astype(bf16)
        mod_s[:, p * D:(p + 1) * D] = jnp.dot(jnp.broadcast_to(sc, (8, D)), wm_s[:, p * D:(p + 1) * D], preferred_element_type=f32)

    @pl.when(step == 0)
    @jax.named_scope("step0")
    def _():
        cp_s(0).start(); cp_k(0).start(); cp_v(0).start()
        cp_q(0).start()
        for p in (2, 1, 0, 4, 3): cp_wm(p).start()
        cp_w1(0).start(); cp_w3(0).start()
        cp_s(1).start(); cp_k(1).start(); cp_v(1).start()
        cp_w2(0).start()
        cp_w1(1).start(); cp_w3(1).start()
        cp_q(1).start()
        cp_w2(1).start()
        cp_w1(2).start(); cp_w3(2).start()
        cp_w2(2).start()
        cp_wm(5).start()
        for g in range(2, NG):
            cp_s(g).start(); cp_k(g).start(); cp_v(g).start(); cp_q(g).start()
        for i, row in enumerate(TABLE):
            for t, term in enumerate(row):
                for e in range(4):
                    tbl[(i * T_SLOTS + t) * 4 + e] = jnp.int32(term[e])
        pp[0] = jnp.zeros(pp.shape[1:], f32)
        k_s[KPAD - 16:KPAD, :] = jnp.zeros((16, D), bf16)
        skt_s[0:4, :] = sk_ref[...].astype(f32)
        cp_s(0).wait(); cp_k(0).wait(); cp_v(0).wait()
        for _, th in d_tasks(0): th()
        hf[0, 0:CH, :] = hf[0, 0:CH, :] + dd_ref[...].astype(f32).reshape(1, D)
        for term in PRO_TERMS[:3]:
            for r in range(0, CH, RB): term_piece(*term, r)
        bt = b_tasks(0, h2a, x1a)
        nln = BM // LR
        for _, th in bt[:-nln]: th()
        for p in (2, 1, 0, 4, 3):
            cp_wm(p).wait()
            mod_part(p)
        cp_q(0).wait()
        for _, th in bt[-nln:]: th()
        ct = [(40, functools.partial(term_piece, *term, r)) for term in PRO_TERMS[3:] for r in range(0, CH, RB)]
        bt1 = b_tasks(1, h2b, x1b)
        def pre(k):
            if k == 0: cp_w1(0).wait()
            if k == 1: cp_w3(0).wait()
            if k == 2:
                cp_s(1).wait(); cp_k(1).wait(); cp_v(1).wait()
                for _, th in d_tasks(1): th()
                cp_w2(0).wait()
            if k == 3: cp_w1(1).wait()
            if k == 4: cp_w3(1).wait()
            if k == 5:
                cp_q(1).wait(); cp_w2(1).wait()
            if k == 6: cp_w1(2).wait()
            if k == 7: cp_w3(2).wait()
            if k == 8: cp_w2(2).wait()
            if k == 9:
                cp_wm(5).wait(); mod_part(5)
        cs = split(ct, 2)
        bs = split(bt1, 2)
        slots = [[], [], [], cs[0], cs[1], [], bs[0], bs[1], [], []]
        ffn(h2a, x1a, slots, pre)

    @pl.when(jnp.logical_and(step >= 1, step <= N_CSTEPS))
    @jax.named_scope("waits")
    def _():
        g = step + 1
        cp_s(g).wait(); cp_k(g).wait(); cp_v(g).wait(); cp_q(g).wait()

    @pl.when(jnp.logical_and(step >= 1, step <= N_CSTEPS))
    @jax.named_scope("stepN")
    def _():
        rotate()
        g = step + 1
        ct = [(40, functools.partial(dyn_piece, step - 1, t, r)) for t in range(T_SLOTS) for r in range(0, CH, RB)]
        cs = split(ct, NCS)
        bs = split(b_tasks(g, h2b, x1b), NBS)
        slots = [d_tasks(g)] + [[] for _ in range(C0 - 1)] + cs + bs
        slots += [[] for _ in range(10 - len(slots))]
        ffn(h2a, x1a, slots)

    @pl.when(step == NST - 1)
    @jax.named_scope("step7")
    def _():
        ffn(h2b, x1b, [[] for _ in range(10)])


@jax.jit
def pallas_adaLN_cond__ssm_conv_h3__glu_gated_swiglu__prompt_kernel(A_q, A_k, A_v, A_shift_k, A_ssm_k, A_ssm_D, B_x, B_w1, B_w3, B_w2, c, w_mod):
    fm, gm = _dft_consts()
    fm = jnp.asarray(fm, bf16); gm = jnp.asarray(gm, bf16)
    any_spec = pl.BlockSpec(memory_space=pl.ANY)
    vm = pl.BlockSpec(memory_space=pltpu.VMEM)
    return pl.pallas_call(
        _kernel,
        grid=(NST,),
        in_specs=[any_spec, any_spec, any_spec, vm, any_spec, vm, any_spec, any_spec, any_spec, vm, any_spec, vm, vm],
        out_specs=pl.BlockSpec((1, BM, D), lambda i: (0, i, 0)),
        out_shape=jax.ShapeDtypeStruct((1, S, D), bf16),
        scratch_shapes=[
            pltpu.VMEM((8, 6 * D), f32), pltpu.VMEM((8, D), f32),
            pltpu.VMEM((S, D), bf16), pltpu.VMEM((S + KPAD, D), bf16), pltpu.VMEM((S, D), bf16),
            pltpu.VMEM((NST, D, BM), bf16), pltpu.VMEM((D, 6 * D), bf16),
            pltpu.VMEM((D, FF), bf16), pltpu.VMEM((D, FF), bf16), pltpu.VMEM((FF, D), bf16),
            pltpu.VMEM((NCH, 2 * CH, D), f32), pltpu.VMEM((NCH, 2 * CH, D), f32), pltpu.VMEM((NCH + 1, 2 * CH, D), f32),
            pltpu.VMEM((BM, D), bf16), pltpu.VMEM((2, 2 * CH, D), bf16), pltpu.VMEM((BM, D), f32),
            pltpu.VMEM((BM, D), bf16), pltpu.VMEM((BM, D), bf16), pltpu.VMEM((BM, D), f32), pltpu.VMEM((BM, D), f32),
            pltpu.SMEM((N_CSTEPS * T_SLOTS * 4,), jnp.int32),
            pltpu.SemaphoreType.DMA((4 * NST + 6 + 3 * (FF // FC),)),
        ],
        compiler_params=pltpu.CompilerParams(dimension_semantics=("arbitrary",), vmem_limit_bytes=110 * 1024 * 1024),
    )(A_q, A_k, A_v, A_shift_k.T, A_ssm_k, A_ssm_D, B_w1, B_w3, B_w2, c, w_mod, fm, gm)
```

```python
import functools, os
import numpy as np
import jax
import jax.numpy as jnp
from jax.experimental import pallas as pl
from jax.experimental.pallas import tpu as pltpu

S, D, FF = 2048, 640, 1536
CH = 128
NCH = S // CH
BM = 256
NST = S // BM
FC = 512
NFC = FF // FC
EPS = 1e-5
KPAD = 64
RB = 8
KR = int(os.environ.get('KR', 64))
LR = int(os.environ.get('LR', 128))
f32, bf16 = jnp.float32, jnp.bfloat16
NCS = int(os.environ.get('NCS', 6))
NBS = int(os.environ.get('NBS', 2))
C0 = int(os.environ.get('C0', 1))
ORD = int(os.environ.get('ORD', 0))
L0 = int(os.environ.get('L0', 64))
PROF = int(os.environ.get('PROF', 0))
FAST = int(os.environ.get('FAST', 0))


def scope(name):
    if PROF:
        return jax.named_scope(name)
    import contextlib
    return contextlib.nullcontext()


def _dft_consts():
    f = np.concatenate([np.arange(0, CH, 2), np.arange(1, CH, 2)])
    n = np.arange(CH)
    th = np.pi * (2 * f[:, None] + 1) * n[None, :] / (2 * CH)
    fm = np.concatenate([np.cos(th), -np.sin(th)], axis=0)
    gm = fm.T / CH
    return fm.astype(np.float32), gm.astype(np.float32)


def _schedule(pro_chunks=4, steps=6, T=21):
    done = set(); touched = set()
    def mk(u, j):
        s = u + j
        src = s + 1 if s in touched else 0
        touched.add(s); done.add((u, j))
        return (u, j, s + 1, src)
    pro = [mk(u, s - u) for s in range(pro_chunks) for u in range(s + 1)]
    table = []
    for i in range(1, steps + 1):
        n = 2 * i + 4
        avail = sorted((u + j, u, j) for u in range(n) for j in range(n)
                       if u + j < NCH and (u, j) not in done)
        pick = avail[:T]
        assert len(pick) == T
        table.append([mk(u, j) for s, u, j in pick])
        for s in range(2 * i + 4):
            assert all((u, s - u) in done for u in range(s + 1))
    assert len(done) == NCH * (NCH + 1) // 2
    return pro, table

PRO_TERMS, TABLE = _schedule()
T_SLOTS = len(TABLE[0])
N_CSTEPS = len(TABLE)


def _kernel(q_hbm, k_hbm, v_hbm, sk_hbm, ssm_hbm, dd_hbm, w1_hbm, w3_hbm, w2_hbm, c_hbm, wm_hbm,
            fm_hbm, gm_hbm,
            o_ref,
            mod_s, skt_s, q_s, k_s, v_s, ssm_s, wm_s, w1_s, w3_s, w2_s,
            xf, hf, pp, kv_s, yy_s, h2_s, x1_s, xn_s, fm_s, gm_s, sk_s, dd_s, c_s, tbl, sems):
    step = pl.program_id(0)

    def al(x, m):
        return x if isinstance(x, int) else pl.multiple_of(x, m)

    NG = NST
    SB = 4 * NG
    def cp_q(g): return pltpu.make_async_copy(q_hbm.at[0, pl.ds(g * BM, BM), :], q_s.at[g], sems.at[0 * NG + g])
    def cp_k(g):
        if isinstance(g, int) and g == 0:
            return pltpu.make_async_copy(k_hbm.at[0, pl.ds(0, BM), :], k_s.at[0, pl.ds(KPAD, BM), :], sems.at[1 * NG + g])
        return pltpu.make_async_copy(k_hbm.at[0, pl.ds(al(g * BM - 16, 16), BM + 16), :], k_s.at[g, pl.ds(KPAD - 16, BM + 16), :], sems.at[1 * NG + g])
    def cp_v(g): return pltpu.make_async_copy(v_hbm.at[0, pl.ds(g * BM, BM), :], v_s.at[g], sems.at[2 * NG + g])
    def cp_s(g): return pltpu.make_async_copy(ssm_hbm.at[:, pl.ds(g * BM, BM)], ssm_s.at[g], sems.at[3 * NG + g])
    def cp_wm(p): return pltpu.make_async_copy(wm_hbm.at[:, pl.ds(p * D, D)], wm_s.at[:, pl.ds(p * D, D)], sems.at[SB + p])
    def cp_w1(c): return pltpu.make_async_copy(w1_hbm.at[:, pl.ds(c * FC, FC)], w1_s.at[:, pl.ds(c * FC, FC)], sems.at[SB + 6 + c])
    def cp_w3(c): return pltpu.make_async_copy(w3_hbm.at[:, pl.ds(c * FC, FC)], w3_s.at[:, pl.ds(c * FC, FC)], sems.at[SB + 6 + NFC + c])
    def cp_w2(c): return pltpu.make_async_copy(w2_hbm.at[pl.ds(c * FC, FC), :], w2_s.at[pl.ds(c * FC, FC), :], sems.at[SB + 6 + 2 * NFC + c])
    SS = SB + 6 + 3 * NFC
    def cp_small():
        return [pltpu.make_async_copy(a, b, sems.at[SS + i]) for i, (a, b) in enumerate(
            [(fm_hbm, fm_s), (sk_hbm, sk_s), (dd_hbm, dd_s), (gm_hbm, gm_s), (c_hbm, c_s)])]

    def kv_piece(g, r):
        kw = k_s[g, KPAD - 16 + r:KPAD + r + KR, :].astype(f32)
        ks = kw[16:, :] * skt_s[0:1, :]
        for j in range(1, 4):
            ks = ks + kw[16 - j:16 - j + KR, :] * skt_s[j:j + 1, :]
        kv_s[r:r + KR, :] = (ks * v_s[g, r:r + KR, :].astype(f32)).astype(bf16)

    def x_dot(g, h):
        xf[2 * g + h] = jnp.dot(fm_s[...], kv_s[h * CH:(h + 1) * CH, :], preferred_element_type=f32)

    def h_dot(g, h):
        hc = ssm_s[g, :, h * CH:(h + 1) * CH]
        hf[2 * g + h] = jax.lax.dot_general(fm_s[...], hc, (((1,), (1,)), ((), ())), preferred_element_type=f32)

    def d_tasks(g):
        t = [(100, functools.partial(h_dot, g, 0)), (100, functools.partial(h_dot, g, 1))]
        for h in range(2):
            for r in range(h * CH, (h + 1) * CH, KR):
                t.append((280 * KR // 32, functools.partial(kv_piece, g, r)))
            t.append((100, functools.partial(x_dot, g, h)))
        return t

    def term_piece(u, j, dst, src, r):
        xr = xf[u, r:r + RB, :]; xi = xf[u, CH + r:CH + r + RB, :]
        hr = hf[j, r:r + RB, :]; hi = hf[j, CH + r:CH + r + RB, :]
        pr = pp[src, r:r + RB, :]; pi = pp[src, CH + r:CH + r + RB, :]
        nr = pr + (xr * hr - xi * hi)
        ni = pi + (xr * hi + xi * hr)
        pp[dst, r:r + RB, :] = nr
        pp[dst, CH + r:CH + r + RB, :] = ni

    def dyn_piece(row, t, r):
        b = (row * T_SLOTS + t) * 4
        term_piece(tbl[b], tbl[b + 1], tbl[b + 2], tbl[b + 3], r)

    H = CH // 2
    def yy_piece(g, h, r):
        n = 2 * g + h
        cre = pp[n + 1, r:r + 16, :]; pim = pp[n, CH + r:CH + r + 16, :]
        cim = pp[n + 1, CH + r:CH + r + 16, :]; pre = pp[n, r:r + 16, :]
        if r < H:
            a = cre - pim; b = cim + pre
        else:
            a = cre + pim; b = cim - pre
        yy_s[h, r:r + 16, :] = a.astype(bf16)
        yy_s[h, CH + r:CH + r + 16, :] = b.astype(bf16)

    def inv_dot(slot, h):
        x1_s[slot, h * CH:(h + 1) * CH, :] = jnp.dot(gm_s[...], yy_s[h], preferred_element_type=f32)

    def _ln(x):
        m = jnp.mean(x, axis=-1, keepdims=True)
        xc = x - m
        v = jnp.mean(xc * xc, axis=-1, keepdims=True)
        return xc * jax.lax.rsqrt(v + EPS)

    def ln_piece(g, slot, r):
        ln_piece_n(g, slot, r, LR)

    def ln_piece_n(g, slot, r, LR):
        x = q_s[g, r:r + LR, :].astype(f32)
        y = x1_s[slot, r:r + LR, :]
        sa = mod_s[0:1, 0 * D:1 * D]; ca = mod_s[0:1, 1 * D:2 * D]; ga = mod_s[0:1, 2 * D:3 * D]
        sb = mod_s[0:1, 3 * D:4 * D]; cb = mod_s[0:1, 4 * D:5 * D]
        h1 = _ln(x) * (1.0 + ca) + sa
        x1 = x + ga * (h1 * y)
        h2 = _ln(x1) * (1.0 + cb) + sb
        x1_s[slot, r:r + LR, :] = x1
        h2_s[slot, r:r + LR, :] = h2.astype(bf16)

    def ln_phase1(g, slot, r, n):
        x = q_s[g, r:r + n, :].astype(f32)
        y = x1_s[slot, r:r + n, :]
        sa = mod_s[0:1, 0 * D:1 * D]; ca = mod_s[0:1, 1 * D:2 * D]; ga = mod_s[0:1, 2 * D:3 * D]
        h1 = _ln(x) * (1.0 + ca) + sa
        x1 = x + ga * (h1 * y)
        x1_s[slot, r:r + n, :] = x1
        xn_s[r:r + n, :] = _ln(x1)

    def ln_phase2(slot, r, n):
        sb = mod_s[0:1, 3 * D:4 * D]; cb = mod_s[0:1, 4 * D:5 * D]
        h2_s[slot, r:r + n, :] = (xn_s[r:r + n, :] * (1.0 + cb) + sb).astype(bf16)

    def inv_tasks(g, slot):
        t = []
        for h in range(2):
            for r in range(0, CH, 16):
                t.append((40, functools.partial(yy_piece, g, h, r)))
            t.append((100, functools.partial(inv_dot, slot, h)))
        return t

    def ln_tasks(g, slot):
        return [(200 * LR // 16, functools.partial(ln_piece, g, slot, r)) for r in range(0, BM, LR)]

    def ffn(slot, slots, pre=None):
        def emit(k):
            for _, th in slots[k]:
                th()
        if pre is None: pre = lambda k: None
        h2 = h2_s[slot]
        emit(0)
        acc = None
        for c in range(NFC):
            pre(3 * c)
            g = jnp.dot(h2, w1_s[:, c * FC:(c + 1) * FC], preferred_element_type=f32); emit(3 * c + 1)
            pre(3 * c + 1)
            u = jnp.dot(h2, w3_s[:, c * FC:(c + 1) * FC], preferred_element_type=f32)
            hg = 0.5 * g
            hh = ((hg + hg * jnp.tanh(hg)) * u).astype(bf16); emit(3 * c + 2)
            pre(3 * c + 2)
            p = jnp.dot(hh, w2_s[c * FC:(c + 1) * FC, :], preferred_element_type=f32); emit(3 * c + 3)
            acc = p if acc is None else acc + p
        pre(9)
        gb = mod_s[0:1, 5 * D:6 * D]
        o_ref[0] = (x1_s[slot] + gb * acc).astype(o_ref.dtype)

    def split(tasks, n):
        tot = sum(c for c, _ in tasks); out = [[] for _ in range(n)]; acc = 0.0
        for c, th in tasks:
            k = min(n - 1, int((acc + 0.5 * c) * n / tot)); out[k].append((c, th)); acc += c
        return out

    def mod_part(p):
        c = c_s[...].astype(f32)
        sc = (c * jax.nn.sigmoid(c)).astype(bf16)
        mod_s[:, p * D:(p + 1) * D] = jnp.dot(jnp.broadcast_to(sc, (8, D)), wm_s[:, p * D:(p + 1) * D], preferred_element_type=f32)

    @pl.when(step == 0)
    def _():
      with scope("step0"):
        if FAST:
            cps = cp_small()
            for g in range(NG): cps += [cp_s(g), cp_k(g), cp_v(g), cp_q(g)]
            cps += [cp_wm(p) for p in range(6)] + [cp_w1(c) for c in range(NFC)] + [cp_w3(c) for c in range(NFC)] + [cp_w2(c) for c in range(NFC)]
            for c_ in cps: c_.start()
            for i, row in enumerate(TABLE):
                for t, term in enumerate(row):
                    for e in range(4):
                        tbl[(i * T_SLOTS + t) * 4 + e] = jnp.int32(term[e])
            for c_ in cps: c_.wait()
            pp[0] = jnp.zeros(pp.shape[1:], f32)
            skt_s[0:4, :] = sk_s[...].astype(f32)
            mod_s[...] = jnp.ones(mod_s.shape, f32)
            h2_s[...] = jnp.ones(h2_s.shape, bf16); x1_s[...] = jnp.ones(x1_s.shape, f32)
            o_ref[0] = jnp.zeros(o_ref.shape[1:], o_ref.dtype)
            return
        smalls = cp_small()
        cp_s(0).start()
        for c_ in smalls: c_.start()
        cp_k(0).start(); cp_v(0).start()
        cp_s(1).start(); cp_k(1).start(); cp_v(1).start()
        cp_q(0).start()
        for p in (2, 1, 0, 4, 3): cp_wm(p).start()
        cp_w1(0).start(); cp_w3(0).start(); cp_w2(0).start()
        cp_q(1).start()
        for c in range(1, NFC):
            cp_w1(c).start(); cp_w3(c).start(); cp_w2(c).start()
        cp_wm(5).start()
        for g in range(2, NG):
            cp_s(g).start(); cp_k(g).start(); cp_v(g).start(); cp_q(g).start()
        for i, row in enumerate(TABLE):
            for t, term in enumerate(row):
                for e in range(4):
                    tbl[(i * T_SLOTS + t) * 4 + e] = jnp.int32(term[e])
        pp[0] = jnp.zeros(pp.shape[1:], f32)
        k_s[0, KPAD - 16:KPAD, :] = jnp.zeros((16, D), bf16)
        with scope("w_g0"):
            for c_ in smalls: c_.wait()
            cp_s(0).wait(); cp_k(0).wait(); cp_v(0).wait()
        with scope("p_d0"):
            skt_s[0:4, :] = sk_s[...].astype(f32)
            for _, th in d_tasks(0): th()
            hf[0, 0:CH, :] = hf[0, 0:CH, :] + dd_s[...].astype(f32).reshape(1, D)
            for term in PRO_TERMS[:3]:
                for r in range(0, CH, RB): term_piece(*term, r)
            for _, th in inv_tasks(0, 0): th()
        with scope("w_g1"):
            cp_s(1).wait(); cp_k(1).wait(); cp_v(1).wait()
        with scope("p_d1"):
            for _, th in d_tasks(1): th()
            for term in PRO_TERMS[3:]:
                for r in range(0, CH, RB): term_piece(*term, r)
            for _, th in inv_tasks(1, 1): th()
        with scope("w_wm"):
            for p in (2, 1, 0): cp_wm(p).wait()
            cp_q(0).wait()
        with scope("p_ln0a"):
            for p in (2, 1, 0): mod_part(p)
            for r in range(0, BM, 64): ln_phase1(0, 0, r, 64)
        with scope("w_wm"):
            cp_wm(4).wait()
        with scope("p_mod"):
            mod_part(4)
        with scope("w_wm"):
            cp_wm(3).wait()
        with scope("p_ln0b"):
            mod_part(3)
            for r in range(0, BM, 64): ln_phase2(0, r, 64)
        def W(name, f):
            with scope(name): f()
        def pre(k):
            if k % 3 == 0 and k < 9: W("w_w1", lambda: cp_w1(k // 3).wait())
            if k % 3 == 1: W("w_w3", lambda: cp_w3(k // 3).wait())
            if k % 3 == 2: W("w_w2", lambda: cp_w2(k // 3).wait())
            if k == 3: W("w_q1", lambda: cp_q(1).wait())
            if k == 9:
                W("w_gb", lambda: cp_wm(5).wait()); mod_part(5)
        ls = [[(1, functools.partial(ln_piece_n, 1, 1, r, L0)) ] for r in range(0, BM, L0)]
        slots = [[], [], [], []] + ls
        slots += [[] for _ in range(10 - len(slots))]
        ffn(0, slots, pre)

    @pl.when(jnp.logical_and(step >= 1, step <= N_CSTEPS))
    def _():
      with scope("waits"):
        if FAST: return
        g = step + 1
        cp_s(g).wait(); cp_k(g).wait(); cp_v(g).wait(); cp_q(g).wait()

    @pl.when(jnp.logical_and(step >= 1, step <= N_CSTEPS))
    def _():
      with scope("stepN"):
        g = step + 1
        cur = step % 2
        nxt = 1 - cur
        ct = [(40, functools.partial(dyn_piece, step - 1, t, r)) for t in range(T_SLOTS) for r in range(0, CH, RB)]
        cs = split(ct, NCS)
        bs = split(inv_tasks(g, nxt) + ln_tasks(g, nxt), NBS)
        dt = d_tasks(g)
        if ORD == 0:
            slots = [dt] + cs + bs
        elif ORD == 1:
            cs[0] = dt + cs[0]
            slots = [[]] + cs + bs
        elif ORD == 2:
            cs[0] = dt[2:] + cs[0]
            slots = [dt[:2]] + cs + bs
        slots += [[] for _ in range(10 - len(slots))]
        ffn(cur, slots)

    @pl.when(step == NST - 1)
    def _():
      with scope("step7"):
        if FAST:
            o_ref[0] = jnp.zeros(o_ref.shape[1:], o_ref.dtype)
            return
        ffn((NST - 1) % 2, [[] for _ in range(10)])


@jax.jit
def pallas_adaLN_cond__ssm_conv_h3__glu_gated_swiglu__prompt_kernel(A_q, A_k, A_v, A_shift_k, A_ssm_k, A_ssm_D, B_x, B_w1, B_w3, B_w2, c, w_mod):
    fm, gm = _dft_consts()
    fm = jnp.asarray(fm, bf16); gm = jnp.asarray(gm, bf16)
    any_spec = pl.BlockSpec(memory_space=pl.ANY)
    return pl.pallas_call(
        _kernel,
        grid=(NST,),
        in_specs=[any_spec] * 13,
        out_specs=pl.BlockSpec((1, BM, D), lambda i: (0, i, 0)),
        out_shape=jax.ShapeDtypeStruct((1, S, D), bf16),
        scratch_shapes=[
            pltpu.VMEM((8, 6 * D), f32), pltpu.VMEM((8, D), f32),
            pltpu.VMEM((NST, BM, D), bf16), pltpu.VMEM((NST, KPAD + BM, D), bf16), pltpu.VMEM((NST, BM, D), bf16),
            pltpu.VMEM((NST, D, BM), bf16), pltpu.VMEM((D, 6 * D), bf16),
            pltpu.VMEM((D, FF), bf16), pltpu.VMEM((D, FF), bf16), pltpu.VMEM((FF, D), bf16),
            pltpu.VMEM((NCH, 2 * CH, D), f32), pltpu.VMEM((NCH, 2 * CH, D), f32), pltpu.VMEM((NCH + 1, 2 * CH, D), f32),
            pltpu.VMEM((BM, D), bf16), pltpu.VMEM((2, 2 * CH, D), bf16),
            pltpu.VMEM((2, BM, D), bf16), pltpu.VMEM((2, BM, D), f32), pltpu.VMEM((BM, D), f32),
            pltpu.VMEM((2 * CH, CH), bf16), pltpu.VMEM((CH, 2 * CH), bf16),
            pltpu.VMEM((4, D), bf16), pltpu.VMEM((D,), bf16), pltpu.VMEM((1, D), bf16),
            pltpu.SMEM((N_CSTEPS * T_SLOTS * 4,), jnp.int32),
            pltpu.SemaphoreType.DMA((4 * NST + 6 + 3 * NFC + 5,)),
        ],
        compiler_params=pltpu.CompilerParams(dimension_semantics=("arbitrary",), vmem_limit_bytes=110 * 1024 * 1024),
    )(A_q, A_k, A_v, A_shift_k.T, A_ssm_k, A_ssm_D, B_w1, B_w3, B_w2, c, w_mod, fm, gm)
```

```python
import functools

import jax
import jax.numpy as jnp
import numpy as np
from jax.experimental import pallas as pl
from jax.experimental.pallas import tpu as pltpu

S, D, FF = 2048, 640, 1536
CH = 128
NCH = S // CH
BM = 256
NG = S // BM
FC = 512
NFC = FF // FC
EPS = 1e-5
NSL = 3
NOS = 2
KPAD = 64
RB = 8
LSPL = 4
T0 = 11
f32, bf16 = jnp.float32, jnp.bfloat16


def _dft_consts():
    f = np.concatenate([np.arange(0, CH, 2), np.arange(1, CH, 2)])
    n = np.arange(CH)
    th = np.pi * (2 * f[:, None] + 1) * n[None, :] / (2 * CH)
    fm = np.concatenate([np.cos(th), -np.sin(th)], axis=0)
    gm = fm.T / CH
    return fm.astype(np.float32), gm.astype(np.float32)


def _schedule():
    done, touched = set(), set()

    def mk(u, j):
        s = u + j
        src = s + 1 if s in touched else 0
        touched.add(s)
        done.add((u, j))
        return (u, j, s + 1, src)

    pro = [mk(u, s - u) for s in range(4) for u in range(s + 1)]
    t_reg = (NCH * (NCH + 1) // 2 - len(pro) - T0) // 5
    table = []
    for i in range(1, 7):
        n = 2 * i + 4
        avail = sorted((u + j, u, j) for u in range(n) for j in range(n) if u + j < NCH and (u, j) not in done)
        table.append([mk(u, j) for _, u, j in avail[:(T0 if i == 1 else t_reg)]])
        assert len(table[-1]) == (T0 if i == 1 else t_reg)
        assert all((u, s - u) in done for s in range(n) for u in range(s + 1))
    assert len(done) == NCH * (NCH + 1) // 2
    return pro, table


PRO_TERMS, TABLE = _schedule()
T_SLOTS = len(TABLE[1])


def _kernel(q_hbm, k_hbm, v_hbm, sk_hbm, ssm_hbm, dd_hbm, w1_hbm, w3_hbm, w2_hbm, c_hbm, wm_hbm, fm_hbm, gm_hbm,
            o_hbm,
            mod_s, skt_s, q_s, k_s, v_s, ssm_s, wm_s, w1_s, w3_s, w2_s,
            xf, hf, pp, kv_s, yy_s, h2_s, x1_s, xn_s, o_s, fm_s, gm_s, sk_s, dd_s, c_s, tbl, sems, osems):
    step = pl.program_id(0)

    def al(x, m):
        return x if isinstance(x, int) else pl.multiple_of(x, m)

    SB = 4 * NG

    def cp_q(g):
        return pltpu.make_async_copy(q_hbm.at[0, pl.ds(g * BM, BM), :], q_s.at[g], sems.at[g])

    def cp_k(g):
        if isinstance(g, int) and g == 0:
            return pltpu.make_async_copy(k_hbm.at[0, pl.ds(0, BM), :], k_s.at[0, pl.ds(KPAD, BM), :], sems.at[NG])
        return pltpu.make_async_copy(k_hbm.at[0, pl.ds(al(g * BM - 16, 16), BM + 16), :],
                                     k_s.at[g, pl.ds(KPAD - 16, BM + 16), :], sems.at[NG + g])

    def cp_v(g):
        return pltpu.make_async_copy(v_hbm.at[0, pl.ds(g * BM, BM), :], v_s.at[g], sems.at[2 * NG + g])

    def cp_s(g):
        return pltpu.make_async_copy(ssm_hbm.at[:, pl.ds(g * BM, BM)], ssm_s.at[g], sems.at[3 * NG + g])

    def cp_wm(p):
        return pltpu.make_async_copy(wm_hbm.at[:, pl.ds(p * D, D)], wm_s.at[:, pl.ds(p * D, D)], sems.at[SB + p])

    def cp_w1(c):
        return pltpu.make_async_copy(w1_hbm.at[:, pl.ds(c * FC, FC)], w1_s.at[:, pl.ds(c * FC, FC)],
                                     sems.at[SB + 6 + c])

    def cp_w3(c):
        return pltpu.make_async_copy(w3_hbm.at[:, pl.ds(c * FC, FC)], w3_s.at[:, pl.ds(c * FC, FC)],
                                     sems.at[SB + 6 + NFC + c])

    def cp_w2(c):
        return pltpu.make_async_copy(w2_hbm.at[pl.ds(c * FC, FC), :], w2_s.at[pl.ds(c * FC, FC), :],
                                     sems.at[SB + 6 + 2 * NFC + c])

    def cp_small():
        pairs = [(fm_hbm, fm_s), (sk_hbm, sk_s), (dd_hbm, dd_s), (gm_hbm, gm_s), (c_hbm, c_s)]
        return [pltpu.make_async_copy(a, b, sems.at[SB + 6 + 3 * NFC + i]) for i, (a, b) in enumerate(pairs)]

    def cp_conv(g):
        return [cp_s(g), cp_k(g), cp_v(g)]

    def cp_o(g, oslot, r0=0, n=BM, sem=None):
        return pltpu.make_async_copy(o_s.at[oslot, pl.ds(r0, n), :], o_hbm.at[0, pl.ds(al(g * BM + r0, 16), n), :],
                                     osems.at[oslot if sem is None else sem])

    def start(*cs):
        for c_ in cs:
            c_.start()

    def wait(*cs):
        for c_ in cs:
            c_.wait()

    def run(tasks):
        for t in tasks:
            t()

    def kv_chunk(g, h):
        r = h * CH
        kw = k_s[g, KPAD - 16 + r:KPAD + r + CH, :].astype(f32)
        ks = kw[16:, :] * skt_s[0:1, :]
        for j in range(1, 4):
            ks = ks + kw[16 - j:16 - j + CH, :] * skt_s[j:j + 1, :]
        kv_s[r:r + CH, :] = (ks * v_s[g, r:r + CH, :].astype(f32)).astype(bf16)

    def x_dot(g, h):
        xf[2 * g + h] = jnp.dot(fm_s[...], kv_s[h * CH:(h + 1) * CH, :], preferred_element_type=f32)

    def h_dot(g, h):
        hf[2 * g + h] = jax.lax.dot_general(fm_s[...], ssm_s[g, :, h * CH:(h + 1) * CH], (((1,), (1,)), ((), ())),
                                            preferred_element_type=f32)

    def fwd_tasks(g):
        part = functools.partial
        return [part(h_dot, g, 0), part(h_dot, g, 1), part(kv_chunk, g, 0), part(x_dot, g, 0),
                part(kv_chunk, g, 1), part(x_dot, g, 1)]

    def term_piece(u, j, dst, src, r):
        xr = xf[u, r:r + RB, :]; xi = xf[u, CH + r:CH + r + RB, :]
        hr = hf[j, r:r + RB, :]; hi = hf[j, CH + r:CH + r + RB, :]
        pr = pp[src, r:r + RB, :]; pi = pp[src, CH + r:CH + r + RB, :]
        nr = pr + (xr * hr - xi * hi)
        ni = pi + (xr * hi + xi * hr)
        pp[dst, r:r + RB, :] = nr
        pp[dst, CH + r:CH + r + RB, :] = ni

    def static_terms(terms):
        for term in terms:
            for r in range(0, CH, RB):
                term_piece(*term, r)

    def table_piece(row, t, r):
        b = (row * T_SLOTS + t) * 4
        term_piece(tbl[b], tbl[b + 1], tbl[b + 2], tbl[b + 3], r)

    def table_tasks(row, nterms, nparts):
        ts = [functools.partial(table_piece, row, t, r) for t in range(nterms) for r in range(0, CH, RB)]
        return [ts[len(ts) * k // nparts:len(ts) * (k + 1) // nparts] for k in range(nparts)]

    def yy_piece(g, h, r):
        n = 2 * g + h
        cre = pp[n + 1, r:r + 16, :]; pim = pp[n, CH + r:CH + r + 16, :]
        cim = pp[n + 1, CH + r:CH + r + 16, :]; pre = pp[n, r:r + 16, :]
        if r < CH // 2:
            a = cre - pim; b = cim + pre
        else:
            a = cre + pim; b = cim - pre
        yy_s[h, r:r + 16, :] = a.astype(bf16)
        yy_s[h, CH + r:CH + r + 16, :] = b.astype(bf16)

    def inv_dot(slot, h):
        x1_s[slot, h * CH:(h + 1) * CH, :] = jnp.dot(gm_s[...], yy_s[h], preferred_element_type=f32)

    def inverse(g, slot):
        for h in range(2):
            for r in range(0, CH, 16):
                yy_piece(g, h, r)
            inv_dot(slot, h)

    def _ln(x):
        m = jnp.mean(x, axis=-1, keepdims=True)
        xc = x - m
        v = jnp.mean(xc * xc, axis=-1, keepdims=True)
        return xc * jax.lax.rsqrt(v + EPS)

    def mod_vec(p):
        return mod_s[0:1, p * D:(p + 1) * D]

    def mix(g, slot, r, n):
        x = q_s[g, r:r + n, :].astype(f32)
        x1 = x + (_ln(x) * mod_vec(1) + mod_vec(0)) * x1_s[slot, r:r + n, :]
        x1_s[slot, r:r + n, :] = x1
        return _ln(x1)

    def adaln(g, slot):
        h2_s[slot] = (mix(g, slot, 0, BM) * mod_vec(4) + mod_vec(3)).astype(bf16)

    def mod_part(p):
        c = c_s[...].astype(f32)
        sc = (c * jax.nn.sigmoid(c)).astype(bf16)
        mod_s[:, p * D:(p + 1) * D] = jnp.dot(jnp.broadcast_to(sc, (8, D)), wm_s[:, p * D:(p + 1) * D],
                                              preferred_element_type=f32)

    class Ffn:
        def __init__(self, slot):
            self.slot = slot
            self.h2 = h2_s[slot]
            self.acc = None

        def g(self, c):
            self.gate = jnp.dot(self.h2, w1_s[:, c * FC:(c + 1) * FC], preferred_element_type=f32)

        def u(self, c):
            up = jnp.dot(self.h2, w3_s[:, c * FC:(c + 1) * FC], preferred_element_type=f32)
            hg = 0.5 * self.gate
            self.hh = ((hg + hg * jnp.tanh(hg)) * up).astype(bf16)

        def d(self, c):
            p = jnp.dot(self.hh, w2_s[c * FC:(c + 1) * FC, :], preferred_element_type=f32)
            self.acc = p if self.acc is None else self.acc + p

        def out(self, g, oslot):
            o_s[oslot] = (x1_s[self.slot] + mod_vec(5) * self.acc).astype(bf16)
            cp_o(g, oslot).start()

    @pl.when(step == 0)
    def _():
        smalls = cp_small()
        start(cp_s(0), *smalls, cp_k(0), cp_v(0), *cp_conv(1), cp_q(0), cp_q(1))
        start(*[cp_wm(p) for p in (2, 1, 0, 4, 3)])
        start(cp_w1(0), cp_w3(0), cp_w2(0), cp_w1(1), cp_w3(1), cp_w2(1), *cp_conv(2))
        start(cp_w1(2), cp_w3(2), cp_w2(2), cp_wm(5), cp_q(2))
        for g in range(3, NG):
            start(*cp_conv(g), cp_q(g))
        for i, row in enumerate(TABLE):
            for t, term in enumerate(row):
                for e in range(4):
                    tbl[(i * T_SLOTS + t) * 4 + e] = jnp.int32(term[e])
        pp[0] = jnp.zeros(pp.shape[1:], f32)
        k_s[0, KPAD - 16:KPAD, :] = jnp.zeros((16, D), bf16)

        wait(*smalls, *cp_conv(0))
        skt_s[0:4, :] = sk_s[...].astype(f32)
        run(fwd_tasks(0))
        hf[0, 0:CH, :] = hf[0, 0:CH, :] + dd_s[...].astype(f32).reshape(1, D)
        static_terms(PRO_TERMS[:3])
        inverse(0, 0)
        wait(*cp_conv(1))
        run(fwd_tasks(1))
        static_terms(PRO_TERMS[3:])
        inverse(1, 1)

        wait(cp_wm(2), cp_wm(1), cp_wm(0), cp_q(0), cp_q(1))
        for p in (2, 1, 0):
            mod_part(p)
        ga = mod_s[:, 2 * D:3 * D]
        mod_s[:, 0:D] = ga * mod_s[:, 0:D]
        mod_s[:, D:2 * D] = ga * (1.0 + mod_s[:, D:2 * D])
        for g in range(2):
            for r in range(0, BM, 64):
                xn_s[g, r:r + 64, :] = mix(g, g, r, 64)
        wait(cp_wm(4))
        mod_part(4)
        mod_s[:, 4 * D:5 * D] = 1.0 + mod_s[:, 4 * D:5 * D]
        wait(cp_wm(3))
        mod_part(3)
        for g in range(2):
            for r in range(0, BM, 64):
                h2_s[g, r:r + 64, :] = (xn_s[g, r:r + 64, :] * mod_vec(4) + mod_vec(3)).astype(bf16)

        fa, fb = Ffn(0), Ffn(1)
        wait(cp_w1(0)); fa.g(0)
        wait(cp_w3(0)); fa.u(0); fb.g(0)
        wait(cp_w2(0)); fb.u(0); fa.d(0); fb.d(0)
        wait(cp_w1(1), cp_w3(1), cp_w2(1))
        fa.g(1); fa.u(1); fb.g(1); fb.u(1); fa.d(1); fb.d(1)
        wait(cp_w1(2), cp_w3(2), cp_w2(2), cp_q(2), cp_wm(5), *cp_conv(2))
        cs = table_tasks(0, T0, 3)
        mod_part(5)
        run(fwd_tasks(2)); fa.g(2); run(cs[0]); fa.u(2); run(cs[1]); fb.g(2); run(cs[2]); fb.u(2)
        inverse(2, 2); adaln(2, 2)
        fa.d(2); fa.out(0, 0); fb.d(2); fb.out(1, 1)

    gi = step + 1

    @pl.when(step >= 1)
    def _():
        cp_o(gi - 2, jax.lax.rem(gi, NOS)).wait()

    @pl.when(jnp.logical_and(step >= 1, step <= NG - 3))
    def _():
        wait(*cp_conv(gi + 1), cp_q(gi + 1))

    @pl.when(jnp.logical_and(step >= 1, step <= NG - 3))
    def _():
        g = gi + 1
        nxt = jax.lax.rem(g, NSL)
        cs = table_tasks(gi - 1, T_SLOTS, 7)
        f = Ffn(jax.lax.rem(gi, NSL))
        f.g(0); run(fwd_tasks(g)); run(cs[0])
        f.u(0); run(cs[1])
        f.d(0); run(cs[2])
        f.g(1); run(cs[3])
        f.u(1); run(cs[4])
        f.d(1); run(cs[5])
        f.g(2); run(cs[6])
        f.u(2); inverse(g, nxt); adaln(g, nxt)
        f.d(2)
        f.out(gi, jax.lax.rem(gi, NOS))

    @pl.when(step == NG - 2)
    def _():
        g = NG - 1
        slot, oslot = g % NSL, g % NOS
        f = Ffn(slot)
        for c in range(NFC - 1):
            f.g(c); f.u(c); f.d(c)
        f.g(NFC - 1); f.u(NFC - 1)
        n = BM // LSPL
        for k in range(LSPL):
            rows = slice(k * n, (k + 1) * n)
            p = jnp.dot(f.hh[rows], w2_s[(NFC - 1) * FC:, :], preferred_element_type=f32)
            o_s[oslot, rows, :] = (x1_s[slot, rows, :] + mod_vec(5) * (f.acc[rows] + p)).astype(bf16)
            cp_o(g, oslot, k * n, n, sem=NOS + k).start()
        cp_o(g - 1, (g - 1) % NOS).wait()
        for k in range(LSPL):
            cp_o(g, oslot, k * n, n, sem=NOS + k).wait()


@jax.jit
def pallas_adaLN_cond__ssm_conv_h3__glu_gated_swiglu__prompt_kernel(
    A_q: jax.Array,
    A_k: jax.Array,
    A_v: jax.Array,
    A_shift_k: jax.Array,
    A_ssm_k: jax.Array,
    A_ssm_D: jax.Array,
    B_x: jax.Array,
    B_w1: jax.Array,
    B_w3: jax.Array,
    B_w2: jax.Array,
    c: jax.Array,
    w_mod: jax.Array,
):
    fm, gm = _dft_consts()
    any_spec = pl.BlockSpec(memory_space=pl.ANY)
    vm = pltpu.VMEM
    scratch = [
        vm((8, 6 * D), f32), vm((8, D), f32),
        vm((NG, BM, D), bf16), vm((NG, KPAD + BM, D), bf16), vm((NG, BM, D), bf16),
        vm((NG, D, BM), bf16), vm((D, 6 * D), bf16),
        vm((D, FF), bf16), vm((D, FF), bf16), vm((FF, D), bf16),
        vm((NCH, 2 * CH, D), f32), vm((NCH, 2 * CH, D), f32), vm((NCH + 1, 2 * CH, D), f32),
        vm((BM, D), bf16), vm((2, 2 * CH, D), bf16),
        vm((NSL, BM, D), bf16), vm((NSL, BM, D), f32), vm((2, BM, D), f32), vm((NOS, BM, D), bf16),
        vm((2 * CH, CH), bf16), vm((CH, 2 * CH), bf16), vm((4, D), bf16), vm((D,), bf16), vm((1, D), bf16),
        pltpu.SMEM((len(TABLE) * T_SLOTS * 4,), jnp.int32),
        pltpu.SemaphoreType.DMA((4 * NG + 6 + 3 * NFC + 5,)),
        pltpu.SemaphoreType.DMA((NOS + LSPL,)),
    ]
    return pl.pallas_call(
        _kernel,
        grid=(NG - 1,),
        in_specs=[any_spec] * 13,
        out_specs=any_spec,
        out_shape=jax.ShapeDtypeStruct((1, S, D), bf16),
        scratch_shapes=scratch,
        compiler_params=pltpu.CompilerParams(dimension_semantics=("arbitrary",),
                                             vmem_limit_bytes=110 * 1024 * 1024),
    )(A_q, A_k, A_v, A_shift_k.T, A_ssm_k, A_ssm_D, B_w1, B_w3, B_w2, c, w_mod,
      jnp.asarray(fm, bf16), jnp.asarray(gm, bf16))
```

```python
import functools

import jax
import jax.numpy as jnp
import numpy as np
from jax.experimental import pallas as pl
from jax.experimental.pallas import tpu as pltpu

S, D, FF = 2048, 640, 1536
CH = 128
NCH = S // CH
BM = 256
NG = S // BM
FC = 512
NFC = FF // FC
EPS = 1e-5
NSL = 3
NOS = 2
KPAD = 64
RB = 8
LSPL = 4
T0 = 11
f32, bf16 = jnp.float32, jnp.bfloat16


def _dft_consts():
    f = np.concatenate([np.arange(0, CH, 2), np.arange(1, CH, 2)])
    n = np.arange(CH)
    th = np.pi * (2 * f[:, None] + 1) * n[None, :] / (2 * CH)
    fm = np.concatenate([np.cos(th), -np.sin(th)], axis=0)
    gm = fm.T / CH
    return fm.astype(np.float32), gm.astype(np.float32)


def _schedule():
    done, touched = set(), set()

    def mk(u, j):
        s = u + j
        src = s + 1 if s in touched else 0
        touched.add(s)
        done.add((u, j))
        return (u, j, s + 1, src)

    pro = [mk(u, s - u) for s in range(4) for u in range(s + 1)]
    t_reg = (NCH * (NCH + 1) // 2 - len(pro) - T0) // 5
    table = []
    for i in range(1, 7):
        n = 2 * i + 4
        avail = sorted((u + j, u, j) for u in range(n) for j in range(n) if u + j < NCH and (u, j) not in done)
        table.append([mk(u, j) for _, u, j in avail[:(T0 if i == 1 else t_reg)]])
        assert len(table[-1]) == (T0 if i == 1 else t_reg)
        assert all((u, s - u) in done for s in range(n) for u in range(s + 1))
    assert len(done) == NCH * (NCH + 1) // 2
    return pro, table


PRO_TERMS, TABLE = _schedule()
T_SLOTS = len(TABLE[1])


def _kernel(q_hbm, k_hbm, v_hbm, sk_hbm, ssm_hbm, dd_hbm, w1_hbm, w3_hbm, w2_hbm, c_hbm, wm_hbm, fm_hbm, gm_hbm,
            o_hbm,
            mod_s, skt_s, q_s, k_s, v_s, ssm_s, wm_s, w1_s, w3_s, w2_s,
            xf, hf, pp, kv_s, yy_s, h2_s, x1_s, xn_s, o_s, fm_s, gm_s, sk_s, dd_s, c_s, tbl, sems, osems):
    step = pl.program_id(0)

    def al(x, m):
        return x if isinstance(x, int) else pl.multiple_of(x, m)

    SB = 4 * NG

    def cp_q(g):
        return pltpu.make_async_copy(q_hbm.at[0, pl.ds(g * BM, BM), :], q_s.at[g], sems.at[g])

    def cp_k(g):
        if isinstance(g, int) and g == 0:
            return pltpu.make_async_copy(k_hbm.at[0, pl.ds(0, BM), :], k_s.at[0, pl.ds(KPAD, BM), :], sems.at[NG])
        return pltpu.make_async_copy(k_hbm.at[0, pl.ds(al(g * BM - 16, 16), BM + 16), :],
                                     k_s.at[g, pl.ds(KPAD - 16, BM + 16), :], sems.at[NG + g])

    def cp_v(g):
        return pltpu.make_async_copy(v_hbm.at[0, pl.ds(g * BM, BM), :], v_s.at[g], sems.at[2 * NG + g])

    def cp_s(g):
        return pltpu.make_async_copy(ssm_hbm.at[:, pl.ds(g * BM, BM)], ssm_s.at[g], sems.at[3 * NG + g])

    def cp_wm(p0, n):
        return pltpu.make_async_copy(wm_hbm.at[:, pl.ds(p0 * D, n * D)], wm_s.at[:, pl.ds(p0 * D, n * D)],
                                     sems.at[SB + p0])

    def cp_w1(c):
        return pltpu.make_async_copy(w1_hbm.at[:, pl.ds(c * FC, FC)], w1_s.at[:, pl.ds(c * FC, FC)],
                                     sems.at[SB + 6 + c])

    def cp_w3(c):
        return pltpu.make_async_copy(w3_hbm.at[:, pl.ds(c * FC, FC)], w3_s.at[:, pl.ds(c * FC, FC)],
                                     sems.at[SB + 6 + NFC + c])

    def cp_w2(c):
        return pltpu.make_async_copy(w2_hbm.at[pl.ds(c * FC, FC), :], w2_s.at[pl.ds(c * FC, FC), :],
                                     sems.at[SB + 6 + 2 * NFC + c])

    def cp_small():
        pairs = [(fm_hbm, fm_s), (sk_hbm, sk_s), (dd_hbm, dd_s), (gm_hbm, gm_s), (c_hbm, c_s)]
        return [pltpu.make_async_copy(a, b, sems.at[SB + 6 + 3 * NFC + i]) for i, (a, b) in enumerate(pairs)]

    def cp_conv(g):
        return [cp_s(g), cp_k(g), cp_v(g)]

    def cp_o(g, oslot, r0=0, n=BM, sem=None):
        return pltpu.make_async_copy(o_s.at[oslot, pl.ds(r0, n), :], o_hbm.at[0, pl.ds(al(g * BM + r0, 16), n), :],
                                     osems.at[oslot if sem is None else sem])

    def start(*cs):
        for c_ in cs:
            c_.start()

    def wait(*cs):
        for c_ in cs:
            c_.wait()

    def run(tasks):
        for t in tasks:
            t()

    def kv_chunk(g, h):
        r = h * CH
        kw = k_s[g, KPAD - 16 + r:KPAD + r + CH, :].astype(f32)
        ks = kw[16:, :] * skt_s[0:1, :]
        for j in range(1, 4):
            ks = ks + kw[16 - j:16 - j + CH, :] * skt_s[j:j + 1, :]
        kv_s[r:r + CH, :] = (ks * v_s[g, r:r + CH, :].astype(f32)).astype(bf16)

    def x_dot(g, h):
        xf[2 * g + h] = jnp.dot(fm_s[...], kv_s[h * CH:(h + 1) * CH, :], preferred_element_type=f32)

    def h_dot(g, h):
        hf[2 * g + h] = jax.lax.dot_general(fm_s[...], ssm_s[g, :, h * CH:(h + 1) * CH], (((1,), (1,)), ((), ())),
                                            preferred_element_type=f32)

    def fwd_tasks(g):
        part = functools.partial
        return [part(h_dot, g, 0), part(h_dot, g, 1), part(kv_chunk, g, 0), part(x_dot, g, 0),
                part(kv_chunk, g, 1), part(x_dot, g, 1)]

    def term_piece(u, j, dst, src, r):
        xr = xf[u, r:r + RB, :]; xi = xf[u, CH + r:CH + r + RB, :]
        hr = hf[j, r:r + RB, :]; hi = hf[j, CH + r:CH + r + RB, :]
        pr = pp[src, r:r + RB, :]; pi = pp[src, CH + r:CH + r + RB, :]
        nr = pr + (xr * hr - xi * hi)
        ni = pi + (xr * hi + xi * hr)
        pp[dst, r:r + RB, :] = nr
        pp[dst, CH + r:CH + r + RB, :] = ni

    def static_terms(terms):
        for term in terms:
            for r in range(0, CH, RB):
                term_piece(*term, r)

    def table_piece(row, t, r):
        b = (row * T_SLOTS + t) * 4
        term_piece(tbl[b], tbl[b + 1], tbl[b + 2], tbl[b + 3], r)

    def table_tasks(row, nterms, nparts):
        ts = [functools.partial(table_piece, row, t, r) for t in range(nterms) for r in range(0, CH, RB)]
        return [ts[len(ts) * k // nparts:len(ts) * (k + 1) // nparts] for k in range(nparts)]

    def yy_piece(g, h, r):
        n = 2 * g + h
        cre = pp[n + 1, r:r + 16, :]; pim = pp[n, CH + r:CH + r + 16, :]
        cim = pp[n + 1, CH + r:CH + r + 16, :]; pre = pp[n, r:r + 16, :]
        if r < CH // 2:
            a = cre - pim; b = cim + pre
        else:
            a = cre + pim; b = cim - pre
        yy_s[h, r:r + 16, :] = a.astype(bf16)
        yy_s[h, CH + r:CH + r + 16, :] = b.astype(bf16)

    def inv_dot(slot, h):
        x1_s[slot, h * CH:(h + 1) * CH, :] = jnp.dot(gm_s[...], yy_s[h], preferred_element_type=f32)

    def inverse(g, slot):
        for h in range(2):
            for r in range(0, CH, 16):
                yy_piece(g, h, r)
            inv_dot(slot, h)

    def _ln(x):
        m = jnp.mean(x, axis=-1, keepdims=True)
        xc = x - m
        v = jnp.mean(xc * xc, axis=-1, keepdims=True)
        return xc * jax.lax.rsqrt(v + EPS)

    def mod_vec(p):
        return mod_s[0:1, p * D:(p + 1) * D]

    def mix(g, slot, r, n):
        x = q_s[g, r:r + n, :].astype(f32)
        x1 = x + (_ln(x) * mod_vec(1) + mod_vec(0)) * x1_s[slot, r:r + n, :]
        x1_s[slot, r:r + n, :] = x1
        return _ln(x1)

    def adaln(g, slot):
        h2_s[slot] = (mix(g, slot, 0, BM) * mod_vec(4) + mod_vec(3)).astype(bf16)

    def mod_part(p):
        c = c_s[...].astype(f32)
        sc = (c * jax.nn.sigmoid(c)).astype(bf16)
        mod_s[:, p * D:(p + 1) * D] = jnp.dot(jnp.broadcast_to(sc, (8, D)), wm_s[:, p * D:(p + 1) * D],
                                              preferred_element_type=f32)

    class Ffn:
        def __init__(self, slot):
            self.slot = slot
            self.h2 = h2_s[slot]
            self.acc = None

        def g(self, c):
            self.gate = jnp.dot(self.h2, w1_s[:, c * FC:(c + 1) * FC], preferred_element_type=f32)

        def u(self, c):
            up = jnp.dot(self.h2, w3_s[:, c * FC:(c + 1) * FC], preferred_element_type=f32)
            hg = 0.5 * self.gate
            self.hh = ((hg + hg * jnp.tanh(hg)) * up).astype(bf16)

        def d(self, c):
            p = jnp.dot(self.hh, w2_s[c * FC:(c + 1) * FC, :], preferred_element_type=f32)
            self.acc = p if self.acc is None else self.acc + p

        def out(self, g, oslot):
            o_s[oslot] = (x1_s[self.slot] + mod_vec(5) * self.acc).astype(bf16)
            cp_o(g, oslot).start()

    @pl.when(step == 0)
    def _():
        smalls = cp_small()
        start(cp_s(0), *smalls, cp_k(0), cp_v(0), *cp_conv(1), cp_q(0), cp_q(1))
        start(cp_wm(0, 3), cp_wm(3, 2))
        start(cp_w1(0), cp_w3(0), cp_w2(0), cp_w1(1), cp_w3(1), cp_w2(1), *cp_conv(2))
        start(cp_w1(2), cp_w3(2), cp_w2(2), cp_wm(5, 1), cp_q(2))
        for g in range(3, NG):
            start(*cp_conv(g), cp_q(g))
        for i, row in enumerate(TABLE):
            for t, term in enumerate(row):
                for e in range(4):
                    tbl[(i * T_SLOTS + t) * 4 + e] = jnp.int32(term[e])
        pp[0] = jnp.zeros(pp.shape[1:], f32)
        k_s[0, KPAD - 16:KPAD, :] = jnp.zeros((16, D), bf16)

        wait(*smalls, *cp_conv(0))
        skt_s[0:4, :] = sk_s[...].astype(f32)
        run(fwd_tasks(0))
        hf[0, 0:CH, :] = hf[0, 0:CH, :] + dd_s[...].astype(f32).reshape(1, D)
        static_terms(PRO_TERMS[:3])
        inverse(0, 0)
        wait(*cp_conv(1))
        run(fwd_tasks(1))
        static_terms(PRO_TERMS[3:])
        inverse(1, 1)

        wait(cp_wm(0, 3), cp_q(0), cp_q(1))
        for p in (2, 1, 0):
            mod_part(p)
        ga = mod_s[:, 2 * D:3 * D]
        mod_s[:, 0:D] = ga * mod_s[:, 0:D]
        mod_s[:, D:2 * D] = ga * (1.0 + mod_s[:, D:2 * D])
        for g in range(2):
            for r in range(0, BM, 64):
                xn_s[g, r:r + 64, :] = mix(g, g, r, 64)
        wait(cp_wm(3, 2))
        mod_part(4)
        mod_s[:, 4 * D:5 * D] = 1.0 + mod_s[:, 4 * D:5 * D]
        mod_part(3)
        for g in range(2):
            for r in range(0, BM, 64):
                h2_s[g, r:r + 64, :] = (xn_s[g, r:r + 64, :] * mod_vec(4) + mod_vec(3)).astype(bf16)

        fa, fb = Ffn(0), Ffn(1)
        wait(cp_w1(0)); fa.g(0)
        wait(cp_w3(0)); fa.u(0); fb.g(0)
        wait(cp_w2(0)); fb.u(0); fa.d(0); fb.d(0)
        wait(cp_w1(1), cp_w3(1), cp_w2(1))
        fa.g(1); fa.u(1); fb.g(1); fb.u(1); fa.d(1); fb.d(1)
        wait(cp_w1(2), cp_w3(2), cp_w2(2), cp_q(2), cp_wm(5, 1), *cp_conv(2))
        cs = table_tasks(0, T0, 3)
        mod_part(5)
        run(fwd_tasks(2)); fa.g(2); run(cs[0]); fa.u(2); run(cs[1]); fb.g(2); run(cs[2]); fb.u(2)
        inverse(2, 2); adaln(2, 2)
        fa.d(2); fa.out(0, 0); fb.d(2); fb.out(1, 1)

    gi = step + 1

    @pl.when(step >= 1)
    def _():
        cp_o(gi - 2, jax.lax.rem(gi, NOS)).wait()

    @pl.when(jnp.logical_and(step >= 1, step <= NG - 3))
    def _():
        wait(*cp_conv(gi + 1), cp_q(gi + 1))

    @pl.when(jnp.logical_and(step >= 1, step <= NG - 3))
    def _():
        g = gi + 1
        nxt = jax.lax.rem(g, NSL)
        cs = table_tasks(gi - 1, T_SLOTS, 7)
        f = Ffn(jax.lax.rem(gi, NSL))
        f.g(0); run(fwd_tasks(g)); run(cs[0])
        f.u(0); run(cs[1])
        f.d(0); run(cs[2])
        f.g(1); run(cs[3])
        f.u(1); run(cs[4])
        f.d(1); run(cs[5])
        f.g(2); run(cs[6])
        f.u(2); inverse(g, nxt); adaln(g, nxt)
        f.d(2)
        f.out(gi, jax.lax.rem(gi, NOS))

    @pl.when(step == NG - 2)
    def _():
        g = NG - 1
        slot, oslot = g % NSL, g % NOS
        f = Ffn(slot)
        for c in range(NFC - 1):
            f.g(c); f.u(c); f.d(c)
        f.g(NFC - 1); f.u(NFC - 1)
        n = BM // LSPL
        for k in range(LSPL):
            rows = slice(k * n, (k + 1) * n)
            p = jnp.dot(f.hh[rows], w2_s[(NFC - 1) * FC:, :], preferred_element_type=f32)
            o_s[oslot, rows, :] = (x1_s[slot, rows, :] + mod_vec(5) * (f.acc[rows] + p)).astype(bf16)
            cp_o(g, oslot, k * n, n, sem=NOS + k).start()
        cp_o(g - 1, (g - 1) % NOS).wait()
        for k in range(LSPL):
            cp_o(g, oslot, k * n, n, sem=NOS + k).wait()


@jax.jit
def pallas_adaLN_cond__ssm_conv_h3__glu_gated_swiglu__prompt_kernel(
    A_q: jax.Array,
    A_k: jax.Array,
    A_v: jax.Array,
    A_shift_k: jax.Array,
    A_ssm_k: jax.Array,
    A_ssm_D: jax.Array,
    B_x: jax.Array,
    B_w1: jax.Array,
    B_w3: jax.Array,
    B_w2: jax.Array,
    c: jax.Array,
    w_mod: jax.Array,
):
    fm, gm = _dft_consts()
    any_spec = pl.BlockSpec(memory_space=pl.ANY)
    vm = pltpu.VMEM
    scratch = [
        vm((8, 6 * D), f32), vm((8, D), f32),
        vm((NG, BM, D), bf16), vm((NG, KPAD + BM, D), bf16), vm((NG, BM, D), bf16),
        vm((NG, D, BM), bf16), vm((D, 6 * D), bf16),
        vm((D, FF), bf16), vm((D, FF), bf16), vm((FF, D), bf16),
        vm((NCH, 2 * CH, D), f32), vm((NCH, 2 * CH, D), f32), vm((NCH + 1, 2 * CH, D), f32),
        vm((BM, D), bf16), vm((2, 2 * CH, D), bf16),
        vm((NSL, BM, D), bf16), vm((NSL, BM, D), f32), vm((2, BM, D), f32), vm((NOS, BM, D), bf16),
        vm((2 * CH, CH), bf16), vm((CH, 2 * CH), bf16), vm((4, D), bf16), vm((D,), bf16), vm((1, D), bf16),
        pltpu.SMEM((len(TABLE) * T_SLOTS * 4,), jnp.int32),
        pltpu.SemaphoreType.DMA((4 * NG + 6 + 3 * NFC + 5,)),
        pltpu.SemaphoreType.DMA((NOS + LSPL,)),
    ]
    return pl.pallas_call(
        _kernel,
        grid=(NG - 1,),
        in_specs=[any_spec] * 13,
        out_specs=any_spec,
        out_shape=jax.ShapeDtypeStruct((1, S, D), bf16),
        scratch_shapes=scratch,
        compiler_params=pltpu.CompilerParams(dimension_semantics=("arbitrary",),
                                             vmem_limit_bytes=110 * 1024 * 1024),
    )(A_q, A_k, A_v, A_shift_k.T, A_ssm_k, A_ssm_D, B_w1, B_w3, B_w2, c, w_mod,
      jnp.asarray(fm, bf16), jnp.asarray(gm, bf16))
```

```python
import functools

import jax
import jax.numpy as jnp
import numpy as np
from jax.experimental import pallas as pl
from jax.experimental.pallas import tpu as pltpu

S, D, FF = 2048, 640, 1536
CH = 128
NCH = S // CH
BM = 256
NG = S // BM
FC = 512
NFC = FF // FC
EPS = 1e-5
NSL = 3
NOS = 2
KPAD = 64
RB = 8
LSPL = 4
T0 = 11
f32, bf16 = jnp.float32, jnp.bfloat16


def _dft_consts():
    f = np.concatenate([np.arange(0, CH, 2), np.arange(1, CH, 2)])
    n = np.arange(CH)
    th = np.pi * (2 * f[:, None] + 1) * n[None, :] / (2 * CH)
    fm = np.concatenate([np.cos(th), -np.sin(th)], axis=0)
    gm = fm.T / CH
    return fm.astype(np.float32), gm.astype(np.float32)


def _schedule():
    done, touched = set(), set()

    def mk(u, j):
        s = u + j
        src = s + 1 if s in touched else 0
        touched.add(s)
        done.add((u, j))
        return (u, j, s + 1, src)

    pro = [mk(u, s - u) for s in range(4) for u in range(s + 1)]
    t_reg = (NCH * (NCH + 1) // 2 - len(pro) - T0) // 5
    table = []
    for i in range(1, 7):
        n = 2 * i + 4
        avail = sorted((u + j, u, j) for u in range(n) for j in range(n) if u + j < NCH and (u, j) not in done)
        table.append([mk(u, j) for _, u, j in avail[:(T0 if i == 1 else t_reg)]])
        assert len(table[-1]) == (T0 if i == 1 else t_reg)
        assert all((u, s - u) in done for s in range(n) for u in range(s + 1))
    assert len(done) == NCH * (NCH + 1) // 2
    return pro, table


PRO_TERMS, TABLE = _schedule()
T_SLOTS = len(TABLE[1])


def _kernel(q_hbm, k_hbm, v_hbm, sk_hbm, ssm_hbm, dd_hbm, w1_hbm, w3_hbm, w2_hbm, c_hbm, wm_hbm, fm_hbm, gm_hbm,
            o_hbm,
            mod_s, skt_s, q_s, k_s, v_s, ssm_s, wm_s, w1_s, w3_s, w2_s,
            xf, hf, pp, kv_s, yy_s, h2_s, x1_s, xn_s, o_s, fm_s, gm_s, sk_s, dd_s, c_s, tbl, sems, osems):
    step = pl.program_id(0)

    def al(x, m):
        return x if isinstance(x, int) else pl.multiple_of(x, m)

    S_G0, S_G1, S_WMA, S_WMB, S_W1, S_W3, S_W2, S_C1, S_C2, S_GRP = range(10)

    def sem_conv(g):
        return sems.at[{0: S_G0, 1: S_G1, 2: S_C2}[g] if isinstance(g, int) and g < 3 else S_GRP + g - 3]

    def sem_q(g):
        return sems.at[{0: S_WMA, 1: S_WMA, 2: S_C2}[g] if isinstance(g, int) and g < 3 else S_GRP + g - 3]

    def sem_w(first, c):
        return sems.at[(first, S_C1, S_C2)[c]]

    def cp_q(g):
        return pltpu.make_async_copy(q_hbm.at[0, pl.ds(g * BM, BM), :], q_s.at[g], sem_q(g))

    def cp_k(g):
        if isinstance(g, int) and g == 0:
            return pltpu.make_async_copy(k_hbm.at[0, pl.ds(0, BM), :], k_s.at[0, pl.ds(KPAD, BM), :], sem_conv(g))
        return pltpu.make_async_copy(k_hbm.at[0, pl.ds(al(g * BM - 16, 16), BM + 16), :],
                                     k_s.at[g, pl.ds(KPAD - 16, BM + 16), :], sem_conv(g))

    def cp_v(g):
        return pltpu.make_async_copy(v_hbm.at[0, pl.ds(g * BM, BM), :], v_s.at[g], sem_conv(g))

    def cp_s(g):
        return pltpu.make_async_copy(ssm_hbm.at[:, pl.ds(g * BM, BM)], ssm_s.at[g], sem_conv(g))

    def cp_wm(p0, n):
        return pltpu.make_async_copy(wm_hbm.at[:, pl.ds(p0 * D, n * D)], wm_s.at[:, pl.ds(p0 * D, n * D)],
                                     sems.at[{0: S_WMA, 3: S_WMB, 5: S_C2}[p0]])

    def cp_w1(c):
        return pltpu.make_async_copy(w1_hbm.at[:, pl.ds(c * FC, FC)], w1_s.at[:, pl.ds(c * FC, FC)], sem_w(S_W1, c))

    def cp_w3(c):
        return pltpu.make_async_copy(w3_hbm.at[:, pl.ds(c * FC, FC)], w3_s.at[:, pl.ds(c * FC, FC)], sem_w(S_W3, c))

    def cp_w2(c):
        return pltpu.make_async_copy(w2_hbm.at[pl.ds(c * FC, FC), :], w2_s.at[pl.ds(c * FC, FC), :], sem_w(S_W2, c))

    def cp_small():
        pairs = [(fm_hbm, fm_s), (sk_hbm, sk_s), (dd_hbm, dd_s), (gm_hbm, gm_s), (c_hbm, c_s)]
        return [pltpu.make_async_copy(a, b, sems.at[S_G0]) for a, b in pairs]

    def cp_conv(g):
        return [cp_s(g), cp_k(g), cp_v(g)]

    def cp_o(g, oslot, r0=0, n=BM, sem=None):
        return pltpu.make_async_copy(o_s.at[oslot, pl.ds(r0, n), :], o_hbm.at[0, pl.ds(al(g * BM + r0, 16), n), :],
                                     osems.at[oslot if sem is None else sem])

    def start(*cs):
        for c_ in cs:
            c_.start()

    def wait(*cs):
        for c_ in cs:
            c_.wait()

    def run(tasks):
        for t in tasks:
            t()

    def kv_chunk(g, h):
        r = h * CH
        kw = k_s[g, KPAD - 16 + r:KPAD + r + CH, :].astype(f32)
        ks = kw[16:, :] * skt_s[0:1, :]
        for j in range(1, 4):
            ks = ks + kw[16 - j:16 - j + CH, :] * skt_s[j:j + 1, :]
        kv_s[r:r + CH, :] = (ks * v_s[g, r:r + CH, :].astype(f32)).astype(bf16)

    def x_dot(g, h):
        xf[2 * g + h] = jnp.dot(fm_s[...], kv_s[h * CH:(h + 1) * CH, :], preferred_element_type=f32)

    def h_dot(g, h):
        hf[2 * g + h] = jax.lax.dot_general(fm_s[...], ssm_s[g, :, h * CH:(h + 1) * CH], (((1,), (1,)), ((), ())),
                                            preferred_element_type=f32)

    def fwd_tasks(g):
        part = functools.partial
        return [part(h_dot, g, 0), part(h_dot, g, 1), part(kv_chunk, g, 0), part(x_dot, g, 0),
                part(kv_chunk, g, 1), part(x_dot, g, 1)]

    def term_piece(u, j, dst, src, r):
        xr = xf[u, r:r + RB, :]; xi = xf[u, CH + r:CH + r + RB, :]
        hr = hf[j, r:r + RB, :]; hi = hf[j, CH + r:CH + r + RB, :]
        pr = pp[src, r:r + RB, :]; pi = pp[src, CH + r:CH + r + RB, :]
        nr = pr + (xr * hr - xi * hi)
        ni = pi + (xr * hi + xi * hr)
        pp[dst, r:r + RB, :] = nr
        pp[dst, CH + r:CH + r + RB, :] = ni

    def static_terms(terms):
        for term in terms:
            for r in range(0, CH, RB):
                term_piece(*term, r)

    def table_piece(row, t, r):
        b = (row * T_SLOTS + t) * 4
        term_piece(tbl[b], tbl[b + 1], tbl[b + 2], tbl[b + 3], r)

    def table_tasks(row, nterms, nparts):
        ts = [functools.partial(table_piece, row, t, r) for t in range(nterms) for r in range(0, CH, RB)]
        return [ts[len(ts) * k // nparts:len(ts) * (k + 1) // nparts] for k in range(nparts)]

    def yy_piece(g, h, r):
        n = 2 * g + h
        cre = pp[n + 1, r:r + 16, :]; pim = pp[n, CH + r:CH + r + 16, :]
        cim = pp[n + 1, CH + r:CH + r + 16, :]; pre = pp[n, r:r + 16, :]
        if r < CH // 2:
            a = cre - pim; b = cim + pre
        else:
            a = cre + pim; b = cim - pre
        yy_s[h, r:r + 16, :] = a.astype(bf16)
        yy_s[h, CH + r:CH + r + 16, :] = b.astype(bf16)

    def inv_dot(slot, h):
        x1_s[slot, h * CH:(h + 1) * CH, :] = jnp.dot(gm_s[...], yy_s[h], preferred_element_type=f32)

    def inverse(g, slot):
        for h in range(2):
            for r in range(0, CH, 16):
                yy_piece(g, h, r)
            inv_dot(slot, h)

    def _ln(x):
        m = jnp.mean(x, axis=-1, keepdims=True)
        xc = x - m
        v = jnp.mean(xc * xc, axis=-1, keepdims=True)
        return xc * jax.lax.rsqrt(v + EPS)

    def mod_vec(p):
        return mod_s[0:1, p * D:(p + 1) * D]

    def mix(g, slot, r, n):
        x = q_s[g, r:r + n, :].astype(f32)
        x1 = x + (_ln(x) * mod_vec(1) + mod_vec(0)) * x1_s[slot, r:r + n, :]
        x1_s[slot, r:r + n, :] = x1
        return _ln(x1)

    def adaln(g, slot):
        h2_s[slot] = (mix(g, slot, 0, BM) * mod_vec(4) + mod_vec(3)).astype(bf16)

    def mod_part(p):
        c = c_s[...].astype(f32)
        sc = (c * jax.nn.sigmoid(c)).astype(bf16)
        mod_s[:, p * D:(p + 1) * D] = jnp.dot(jnp.broadcast_to(sc, (8, D)), wm_s[:, p * D:(p + 1) * D],
                                              preferred_element_type=f32)

    class Ffn:
        def __init__(self, slot):
            self.slot = slot
            self.h2 = h2_s[slot]
            self.acc = None

        def g(self, c):
            self.gate = jnp.dot(self.h2, w1_s[:, c * FC:(c + 1) * FC], preferred_element_type=f32)

        def u(self, c):
            up = jnp.dot(self.h2, w3_s[:, c * FC:(c + 1) * FC], preferred_element_type=f32)
            hg = 0.5 * self.gate
            self.hh = ((hg + hg * jnp.tanh(hg)) * up).astype(bf16)

        def d(self, c):
            p = jnp.dot(self.hh, w2_s[c * FC:(c + 1) * FC, :], preferred_element_type=f32)
            self.acc = p if self.acc is None else self.acc + p

        def out(self, g, oslot):
            o_s[oslot] = (x1_s[self.slot] + mod_vec(5) * self.acc).astype(bf16)
            cp_o(g, oslot).start()

    @pl.when(step == 0)
    def _():
        smalls = cp_small()
        start(cp_s(0), *smalls, cp_k(0), cp_v(0), *cp_conv(1), cp_q(0), cp_q(1))
        start(cp_wm(0, 3), cp_wm(3, 2))
        start(cp_w1(0), cp_w3(0), cp_w2(0), cp_w1(1), cp_w3(1), cp_w2(1), *cp_conv(2))
        start(cp_w1(2), cp_w3(2), cp_w2(2), cp_wm(5, 1), cp_q(2))
        for g in range(3, NG):
            start(*cp_conv(g), cp_q(g))
        for i, row in enumerate(TABLE):
            for t, term in enumerate(row):
                for e in range(4):
                    tbl[(i * T_SLOTS + t) * 4 + e] = jnp.int32(term[e])
        pp[0] = jnp.zeros(pp.shape[1:], f32)
        k_s[0, KPAD - 16:KPAD, :] = jnp.zeros((16, D), bf16)

        wait(*smalls, *cp_conv(0))
        skt_s[0:4, :] = sk_s[...].astype(f32)
        run(fwd_tasks(0))
        hf[0, 0:CH, :] = hf[0, 0:CH, :] + dd_s[...].astype(f32).reshape(1, D)
        static_terms(PRO_TERMS[:3])
        inverse(0, 0)
        wait(*cp_conv(1))
        run(fwd_tasks(1))
        static_terms(PRO_TERMS[3:])
        inverse(1, 1)

        wait(cp_wm(0, 3), cp_q(0), cp_q(1))
        for p in (2, 1, 0):
            mod_part(p)
        ga = mod_s[:, 2 * D:3 * D]
        mod_s[:, 0:D] = ga * mod_s[:, 0:D]
        mod_s[:, D:2 * D] = ga * (1.0 + mod_s[:, D:2 * D])
        for g in range(2):
            for r in range(0, BM, 64):
                xn_s[g, r:r + 64, :] = mix(g, g, r, 64)
        wait(cp_wm(3, 2))
        mod_part(4)
        mod_s[:, 4 * D:5 * D] = 1.0 + mod_s[:, 4 * D:5 * D]
        mod_part(3)
        for g in range(2):
            for r in range(0, BM, 64):
                h2_s[g, r:r + 64, :] = (xn_s[g, r:r + 64, :] * mod_vec(4) + mod_vec(3)).astype(bf16)

        fa, fb = Ffn(0), Ffn(1)
        wait(cp_w1(0)); fa.g(0)
        wait(cp_w3(0)); fa.u(0); fb.g(0)
        wait(cp_w2(0)); fb.u(0); fa.d(0); fb.d(0)
        wait(cp_w1(1), cp_w3(1), cp_w2(1))
        fa.g(1); fa.u(1); fb.g(1); fb.u(1); fa.d(1); fb.d(1)
        wait(cp_w1(2), cp_w3(2), cp_w2(2), cp_q(2), cp_wm(5, 1), *cp_conv(2))
        cs = table_tasks(0, T0, 3)
        mod_part(5)
        run(fwd_tasks(2)); fa.g(2); run(cs[0]); fa.u(2); run(cs[1]); fb.g(2); run(cs[2]); fb.u(2)
        inverse(2, 2); adaln(2, 2)
        fa.d(2); fa.out(0, 0); fb.d(2); fb.out(1, 1)

    gi = step + 1

    @pl.when(step >= 1)
    def _():
        cp_o(gi - 2, jax.lax.rem(gi, NOS)).wait()

    @pl.when(jnp.logical_and(step >= 1, step <= NG - 3))
    def _():
        wait(*cp_conv(gi + 1), cp_q(gi + 1))

    @pl.when(jnp.logical_and(step >= 1, step <= NG - 3))
    def _():
        g = gi + 1
        nxt = jax.lax.rem(g, NSL)
        cs = table_tasks(gi - 1, T_SLOTS, 7)
        f = Ffn(jax.lax.rem(gi, NSL))
        f.g(0); run(fwd_tasks(g)); run(cs[0])
        f.u(0); run(cs[1])
        f.d(0); run(cs[2])
        f.g(1); run(cs[3])
        f.u(1); run(cs[4])
        f.d(1); run(cs[5])
        f.g(2); run(cs[6])
        f.u(2); inverse(g, nxt); adaln(g, nxt)
        f.d(2)
        f.out(gi, jax.lax.rem(gi, NOS))

    @pl.when(step == NG - 2)
    def _():
        g = NG - 1
        slot, oslot = g % NSL, g % NOS
        f = Ffn(slot)
        for c in range(NFC - 1):
            f.g(c); f.u(c); f.d(c)
        f.g(NFC - 1); f.u(NFC - 1)
        n = BM // LSPL
        for k in range(LSPL):
            rows = slice(k * n, (k + 1) * n)
            p = jnp.dot(f.hh[rows], w2_s[(NFC - 1) * FC:, :], preferred_element_type=f32)
            o_s[oslot, rows, :] = (x1_s[slot, rows, :] + mod_vec(5) * (f.acc[rows] + p)).astype(bf16)
            cp_o(g, oslot, k * n, n, sem=NOS).start()
        cp_o(g - 1, (g - 1) % NOS).wait()
        for k in range(LSPL):
            cp_o(g, oslot, k * n, n, sem=NOS).wait()


@jax.jit
def pallas_adaLN_cond__ssm_conv_h3__glu_gated_swiglu__prompt_kernel(
    A_q: jax.Array,
    A_k: jax.Array,
    A_v: jax.Array,
    A_shift_k: jax.Array,
    A_ssm_k: jax.Array,
    A_ssm_D: jax.Array,
    B_x: jax.Array,
    B_w1: jax.Array,
    B_w3: jax.Array,
    B_w2: jax.Array,
    c: jax.Array,
    w_mod: jax.Array,
):
    fm, gm = _dft_consts()
    any_spec = pl.BlockSpec(memory_space=pl.ANY)
    vm = pltpu.VMEM
    scratch = [
        vm((8, 6 * D), f32), vm((8, D), f32),
        vm((NG, BM, D), bf16), vm((NG, KPAD + BM, D), bf16), vm((NG, BM, D), bf16),
        vm((NG, D, BM), bf16), vm((D, 6 * D), bf16),
        vm((D, FF), bf16), vm((D, FF), bf16), vm((FF, D), bf16),
        vm((NCH, 2 * CH, D), f32), vm((NCH, 2 * CH, D), f32), vm((NCH + 1, 2 * CH, D), f32),
        vm((BM, D), bf16), vm((2, 2 * CH, D), bf16),
        vm((NSL, BM, D), bf16), vm((NSL, BM, D), f32), vm((2, BM, D), f32), vm((NOS, BM, D), bf16),
        vm((2 * CH, CH), bf16), vm((CH, 2 * CH), bf16), vm((4, D), bf16), vm((D,), bf16), vm((1, D), bf16),
        pltpu.SMEM((len(TABLE) * T_SLOTS * 4,), jnp.int32),
        pltpu.SemaphoreType.DMA((9 + NG - 3,)),
        pltpu.SemaphoreType.DMA((NOS + 1,)),
    ]
    return pl.pallas_call(
        _kernel,
        grid=(NG - 1,),
        in_specs=[any_spec] * 13,
        out_specs=any_spec,
        out_shape=jax.ShapeDtypeStruct((1, S, D), bf16),
        scratch_shapes=scratch,
        compiler_params=pltpu.CompilerParams(dimension_semantics=("arbitrary",),
                                             vmem_limit_bytes=110 * 1024 * 1024),
    )(A_q, A_k, A_v, A_shift_k.T, A_ssm_k, A_ssm_D, B_w1, B_w3, B_w2, c, w_mod,
      jnp.asarray(fm, bf16), jnp.asarray(gm, bf16))
```

```python
import functools

import jax
import jax.numpy as jnp
import numpy as np
from jax.experimental import pallas as pl
from jax.experimental.pallas import tpu as pltpu

S, D, FF = 2048, 640, 1536
CH = 128
NCH = S // CH
BM = 256
NG = S // BM
FC = 512
NFC = FF // FC
EPS = 1e-5
NSL = 3
NOS = 2
KPAD = 64
RB = 8
LSPL = 4
T0 = 11
f32, bf16 = jnp.float32, jnp.bfloat16


def _dft_consts():
    f = np.concatenate([np.arange(0, CH, 2), np.arange(1, CH, 2)])
    n = np.arange(CH)
    th = np.pi * (2 * f[:, None] + 1) * n[None, :] / (2 * CH)
    fm = np.concatenate([np.cos(th), -np.sin(th)], axis=0)
    gm = fm.T / CH
    return fm.astype(np.float32), gm.astype(np.float32)


def _schedule():
    done, touched = set(), set()

    def mk(u, j):
        s = u + j
        src = s + 1 if s in touched else 0
        touched.add(s)
        done.add((u, j))
        return (u, j, s + 1, src)

    pro = [mk(u, s - u) for s in range(4) for u in range(s + 1)]
    t_reg = (NCH * (NCH + 1) // 2 - len(pro) - T0) // 5
    table = []
    for i in range(1, 7):
        n = 2 * i + 4
        avail = sorted((u + j, u, j) for u in range(n) for j in range(n) if u + j < NCH and (u, j) not in done)
        table.append([mk(u, j) for _, u, j in avail[:(T0 if i == 1 else t_reg)]])
        assert len(table[-1]) == (T0 if i == 1 else t_reg)
        assert all((u, s - u) in done for s in range(n) for u in range(s + 1))
    assert len(done) == NCH * (NCH + 1) // 2
    return pro, table


PRO_TERMS, TABLE = _schedule()
T_SLOTS = len(TABLE[1])


def _kernel(q_hbm, k_hbm, v_hbm, sk_hbm, ssm_hbm, dd_hbm, w1_hbm, w3_hbm, w2_hbm, c_hbm, wm_hbm, fm_hbm, gm_hbm,
            o_hbm,
            mod_s, skt_s, q_s, k_s, v_s, ssm_s, wm_s, w1_s, w3_s, w2_s,
            xf, hf, pp, kv_s, yy_s, h2_s, x1_s, xn_s, o_s, fm_s, gm_s, sk_s, dd_s, c_s, tbl, sems, osems):
    step = pl.program_id(0)

    def al(x, m):
        return x if isinstance(x, int) else pl.multiple_of(x, m)

    S_G0, S_G1, S_WMA, S_WMB, S_FA, S_FB, S_FC, S_FD, S_GRP = range(9)

    def sem_conv(g):
        return sems.at[{0: S_G0, 1: S_G1, 2: S_FD}[g] if isinstance(g, int) and g < 3 else S_GRP + g - 3]

    def sem_q(g):
        return sems.at[{0: S_WMA, 1: S_WMA, 2: S_FD}[g] if isinstance(g, int) and g < 3 else S_GRP + g - 3]

    def cp_q(g):
        return pltpu.make_async_copy(q_hbm.at[0, pl.ds(g * BM, BM), :], q_s.at[g], sem_q(g))

    def cp_k(g):
        if isinstance(g, int) and g == 0:
            return pltpu.make_async_copy(k_hbm.at[0, pl.ds(0, BM), :], k_s.at[0, pl.ds(KPAD, BM), :], sem_conv(g))
        return pltpu.make_async_copy(k_hbm.at[0, pl.ds(al(g * BM - 16, 16), BM + 16), :],
                                     k_s.at[g, pl.ds(KPAD - 16, BM + 16), :], sem_conv(g))

    def cp_v(g):
        return pltpu.make_async_copy(v_hbm.at[0, pl.ds(g * BM, BM), :], v_s.at[g], sem_conv(g))

    def cp_s(g):
        return pltpu.make_async_copy(ssm_hbm.at[:, pl.ds(g * BM, BM)], ssm_s.at[g], sem_conv(g))

    def cp_wm(p0, n):
        return pltpu.make_async_copy(wm_hbm.at[:, pl.ds(p0 * D, n * D)], wm_s.at[:, pl.ds(p0 * D, n * D)],
                                     sems.at[{0: S_WMA, 3: S_WMB, 5: S_FD}[p0]])

    def cp_w1(c):
        return pltpu.make_async_copy(w1_hbm.at[:, pl.ds(c * FC, FC)], w1_s.at[:, pl.ds(c * FC, FC)],
                                     sems.at[(S_FA, S_FB, S_FD)[c]])

    def cp_w3(c):
        return pltpu.make_async_copy(w3_hbm.at[:, pl.ds(c * FC, FC)], w3_s.at[:, pl.ds(c * FC, FC)],
                                     sems.at[(S_FB, S_FC, S_FD)[c]])

    def cp_w2(c):
        return pltpu.make_async_copy(w2_hbm.at[pl.ds(c * FC, FC), :], w2_s.at[pl.ds(c * FC, FC), :],
                                     sems.at[(S_FC, S_FC, S_FD)[c]])

    def cp_small():
        pairs = [(fm_hbm, fm_s), (sk_hbm, sk_s), (dd_hbm, dd_s), (gm_hbm, gm_s), (c_hbm, c_s)]
        return [pltpu.make_async_copy(a, b, sems.at[S_G0]) for a, b in pairs]

    def cp_conv(g):
        return [cp_s(g), cp_k(g), cp_v(g)]

    def cp_o(g, oslot, r0=0, n=BM, sem=None):
        return pltpu.make_async_copy(o_s.at[oslot, pl.ds(r0, n), :], o_hbm.at[0, pl.ds(al(g * BM + r0, 16), n), :],
                                     osems.at[oslot if sem is None else sem])

    def start(*cs):
        for c_ in cs:
            c_.start()

    def wait(*cs):
        for c_ in cs:
            c_.wait()

    def run(tasks):
        for t in tasks:
            t()

    def kv_chunk(g, h):
        r = h * CH
        kw = k_s[g, KPAD - 16 + r:KPAD + r + CH, :].astype(f32)
        ks = kw[16:, :] * skt_s[0:1, :]
        for j in range(1, 4):
            ks = ks + kw[16 - j:16 - j + CH, :] * skt_s[j:j + 1, :]
        kv_s[r:r + CH, :] = (ks * v_s[g, r:r + CH, :].astype(f32)).astype(bf16)

    def x_dot(g, h):
        xf[2 * g + h] = jnp.dot(fm_s[...], kv_s[h * CH:(h + 1) * CH, :], preferred_element_type=f32)

    def h_dot(g, h):
        hf[2 * g + h] = jax.lax.dot_general(fm_s[...], ssm_s[g, :, h * CH:(h + 1) * CH], (((1,), (1,)), ((), ())),
                                            preferred_element_type=f32)

    def fwd_tasks(g):
        part = functools.partial
        return [part(h_dot, g, 0), part(h_dot, g, 1), part(kv_chunk, g, 0), part(x_dot, g, 0),
                part(kv_chunk, g, 1), part(x_dot, g, 1)]

    def term_piece(u, j, dst, src, r):
        xr = xf[u, r:r + RB, :]; xi = xf[u, CH + r:CH + r + RB, :]
        hr = hf[j, r:r + RB, :]; hi = hf[j, CH + r:CH + r + RB, :]
        pr = pp[src, r:r + RB, :]; pi = pp[src, CH + r:CH + r + RB, :]
        nr = pr + (xr * hr - xi * hi)
        ni = pi + (xr * hi + xi * hr)
        pp[dst, r:r + RB, :] = nr
        pp[dst, CH + r:CH + r + RB, :] = ni

    def static_terms(terms):
        for term in terms:
            for r in range(0, CH, RB):
                term_piece(*term, r)

    def table_piece(row, t, r):
        b = (row * T_SLOTS + t) * 4
        term_piece(tbl[b], tbl[b + 1], tbl[b + 2], tbl[b + 3], r)

    def table_tasks(row, nterms, nparts):
        ts = [functools.partial(table_piece, row, t, r) for t in range(nterms) for r in range(0, CH, RB)]
        return [ts[len(ts) * k // nparts:len(ts) * (k + 1) // nparts] for k in range(nparts)]

    def yy_piece(g, h, r):
        n = 2 * g + h
        cre = pp[n + 1, r:r + 16, :]; pim = pp[n, CH + r:CH + r + 16, :]
        cim = pp[n + 1, CH + r:CH + r + 16, :]; pre = pp[n, r:r + 16, :]
        if r < CH // 2:
            a = cre - pim; b = cim + pre
        else:
            a = cre + pim; b = cim - pre
        yy_s[h, r:r + 16, :] = a.astype(bf16)
        yy_s[h, CH + r:CH + r + 16, :] = b.astype(bf16)

    def inv_dot(slot, h):
        x1_s[slot, h * CH:(h + 1) * CH, :] = jnp.dot(gm_s[...], yy_s[h], preferred_element_type=f32)

    def inverse(g, slot):
        for h in range(2):
            for r in range(0, CH, 16):
                yy_piece(g, h, r)
            inv_dot(slot, h)

    def _ln(x):
        m = jnp.mean(x, axis=-1, keepdims=True)
        xc = x - m
        v = jnp.mean(xc * xc, axis=-1, keepdims=True)
        return xc * jax.lax.rsqrt(v + EPS)

    def mod_vec(p):
        return mod_s[0:1, p * D:(p + 1) * D]

    def mix(g, slot, r, n):
        x = q_s[g, r:r + n, :].astype(f32)
        x1 = x + (_ln(x) * mod_vec(1) + mod_vec(0)) * x1_s[slot, r:r + n, :]
        x1_s[slot, r:r + n, :] = x1
        return _ln(x1)

    def adaln(g, slot):
        h2_s[slot] = (mix(g, slot, 0, BM) * mod_vec(4) + mod_vec(3)).astype(bf16)

    def mod_part(p):
        c = c_s[...].astype(f32)
        sc = (c * jax.nn.sigmoid(c)).astype(bf16)
        mod_s[:, p * D:(p + 1) * D] = jnp.dot(jnp.broadcast_to(sc, (8, D)), wm_s[:, p * D:(p + 1) * D],
                                              preferred_element_type=f32)

    class Ffn:
        def __init__(self, slot):
            self.slot = slot
            self.h2 = h2_s[slot]
            self.acc = None

        def g(self, c):
            self.gate = jnp.dot(self.h2, w1_s[:, c * FC:(c + 1) * FC], preferred_element_type=f32)

        def u(self, c):
            up = jnp.dot(self.h2, w3_s[:, c * FC:(c + 1) * FC], preferred_element_type=f32)
            hg = 0.5 * self.gate
            self.hh = ((hg + hg * jnp.tanh(hg)) * up).astype(bf16)

        def d(self, c, hh=None):
            hh = self.hh if hh is None else hh
            p = jnp.dot(hh, w2_s[c * FC:(c + 1) * FC, :], preferred_element_type=f32)
            self.acc = p if self.acc is None else self.acc + p

        def out(self, g, oslot):
            o_s[oslot] = (x1_s[self.slot] + mod_vec(5) * self.acc).astype(bf16)
            cp_o(g, oslot).start()

    @pl.when(step == 0)
    def _():
        smalls = cp_small()
        start(cp_s(0), *smalls, cp_k(0), cp_v(0), *cp_conv(1), cp_q(0), cp_q(1))
        start(cp_wm(0, 3), cp_wm(3, 2))
        start(cp_w1(0), cp_w3(0), cp_w1(1), cp_w3(1), cp_w2(0), cp_w2(1), *cp_conv(2))
        start(cp_w1(2), cp_w3(2), cp_w2(2), cp_wm(5, 1), cp_q(2))
        for g in range(3, NG):
            start(*cp_conv(g), cp_q(g))
        for i, row in enumerate(TABLE):
            for t, term in enumerate(row):
                for e in range(4):
                    tbl[(i * T_SLOTS + t) * 4 + e] = jnp.int32(term[e])
        pp[0] = jnp.zeros(pp.shape[1:], f32)
        k_s[0, KPAD - 16:KPAD, :] = jnp.zeros((16, D), bf16)

        wait(*smalls, *cp_conv(0))
        skt_s[0:4, :] = sk_s[...].astype(f32)
        run(fwd_tasks(0))
        hf[0, 0:CH, :] = hf[0, 0:CH, :] + dd_s[...].astype(f32).reshape(1, D)
        static_terms(PRO_TERMS[:3])
        inverse(0, 0)
        wait(*cp_conv(1))
        run(fwd_tasks(1))
        static_terms(PRO_TERMS[3:])
        inverse(1, 1)

        wait(cp_wm(0, 3), cp_q(0), cp_q(1))
        for p in (2, 1, 0):
            mod_part(p)
        ga = mod_s[:, 2 * D:3 * D]
        mod_s[:, 0:D] = ga * mod_s[:, 0:D]
        mod_s[:, D:2 * D] = ga * (1.0 + mod_s[:, D:2 * D])
        for g in range(2):
            for r in range(0, BM, 64):
                xn_s[g, r:r + 64, :] = mix(g, g, r, 64)
        wait(cp_wm(3, 2))
        mod_part(4)
        mod_s[:, 4 * D:5 * D] = 1.0 + mod_s[:, 4 * D:5 * D]
        mod_part(3)
        for g in range(2):
            for r in range(0, BM, 64):
                h2_s[g, r:r + 64, :] = (xn_s[g, r:r + 64, :] * mod_vec(4) + mod_vec(3)).astype(bf16)

        fa, fb = Ffn(0), Ffn(1)
        wait(cp_w1(0))
        fa.g(0); fb.g(0)
        wait(cp_w3(0), cp_w1(1))
        fa.u(0); fb.u(0)
        ha0, hb0 = fa.hh, fb.hh
        fa.g(1); fb.g(1)
        wait(cp_w3(1), cp_w2(0), cp_w2(1))
        fa.u(1); fb.u(1)
        fa.d(0, ha0); fb.d(0, hb0); fa.d(1); fb.d(1)
        wait(cp_w1(2), cp_w3(2), cp_w2(2), cp_q(2), cp_wm(5, 1), *cp_conv(2))
        cs = table_tasks(0, T0, 3)
        mod_part(5)
        run(fwd_tasks(2)); fa.g(2); run(cs[0]); fa.u(2); run(cs[1]); fb.g(2); run(cs[2]); fb.u(2)
        inverse(2, 2); adaln(2, 2)
        fa.d(2); fa.out(0, 0); fb.d(2); fb.out(1, 1)

    gi = step + 1

    @pl.when(step >= 1)
    def _():
        cp_o(gi - 2, jax.lax.rem(gi, NOS)).wait()

    @pl.when(jnp.logical_and(step >= 1, step <= NG - 3))
    def _():
        wait(*cp_conv(gi + 1), cp_q(gi + 1))

    @pl.when(jnp.logical_and(step >= 1, step <= NG - 3))
    def _():
        g = gi + 1
        nxt = jax.lax.rem(g, NSL)
        cs = table_tasks(gi - 1, T_SLOTS, 7)
        f = Ffn(jax.lax.rem(gi, NSL))
        f.g(0); run(fwd_tasks(g)); run(cs[0])
        f.u(0); run(cs[1])
        f.d(0); run(cs[2])
        f.g(1); run(cs[3])
        f.u(1); run(cs[4])
        f.d(1); run(cs[5])
        f.g(2); run(cs[6])
        f.u(2); inverse(g, nxt); adaln(g, nxt)
        f.d(2)
        f.out(gi, jax.lax.rem(gi, NOS))

    @pl.when(step == NG - 2)
    def _():
        g = NG - 1
        slot, oslot = g % NSL, g % NOS
        f = Ffn(slot)
        for c in range(NFC - 1):
            f.g(c); f.u(c); f.d(c)
        f.g(NFC - 1); f.u(NFC - 1)
        n = BM // LSPL
        for k in range(LSPL):
            rows = slice(k * n, (k + 1) * n)
            p = jnp.dot(f.hh[rows], w2_s[(NFC - 1) * FC:, :], preferred_element_type=f32)
            o_s[oslot, rows, :] = (x1_s[slot, rows, :] + mod_vec(5) * (f.acc[rows] + p)).astype(bf16)
            cp_o(g, oslot, k * n, n, sem=NOS).start()
        cp_o(g - 1, (g - 1) % NOS).wait()
        for k in range(LSPL):
            cp_o(g, oslot, k * n, n, sem=NOS).wait()


@jax.jit
def pallas_adaLN_cond__ssm_conv_h3__glu_gated_swiglu__prompt_kernel(
    A_q: jax.Array,
    A_k: jax.Array,
    A_v: jax.Array,
    A_shift_k: jax.Array,
    A_ssm_k: jax.Array,
    A_ssm_D: jax.Array,
    B_x: jax.Array,
    B_w1: jax.Array,
    B_w3: jax.Array,
    B_w2: jax.Array,
    c: jax.Array,
    w_mod: jax.Array,
):
    fm, gm = _dft_consts()
    any_spec = pl.BlockSpec(memory_space=pl.ANY)
    vm = pltpu.VMEM
    scratch = [
        vm((8, 6 * D), f32), vm((8, D), f32),
        vm((NG, BM, D), bf16), vm((NG, KPAD + BM, D), bf16), vm((NG, BM, D), bf16),
        vm((NG, D, BM), bf16), vm((D, 6 * D), bf16),
        vm((D, FF), bf16), vm((D, FF), bf16), vm((FF, D), bf16),
        vm((NCH, 2 * CH, D), f32), vm((NCH, 2 * CH, D), f32), vm((NCH + 1, 2 * CH, D), f32),
        vm((BM, D), bf16), vm((2, 2 * CH, D), bf16),
        vm((NSL, BM, D), bf16), vm((NSL, BM, D), f32), vm((2, BM, D), f32), vm((NOS, BM, D), bf16),
        vm((2 * CH, CH), bf16), vm((CH, 2 * CH), bf16), vm((4, D), bf16), vm((D,), bf16), vm((1, D), bf16),
        pltpu.SMEM((len(TABLE) * T_SLOTS * 4,), jnp.int32),
        pltpu.SemaphoreType.DMA((8 + NG - 3,)),
        pltpu.SemaphoreType.DMA((NOS + 1,)),
    ]
    return pl.pallas_call(
        _kernel,
        grid=(NG - 1,),
        in_specs=[any_spec] * 13,
        out_specs=any_spec,
        out_shape=jax.ShapeDtypeStruct((1, S, D), bf16),
        scratch_shapes=scratch,
        compiler_params=pltpu.CompilerParams(dimension_semantics=("arbitrary",),
                                             vmem_limit_bytes=110 * 1024 * 1024),
    )(A_q, A_k, A_v, A_shift_k.T, A_ssm_k, A_ssm_D, B_w1, B_w3, B_w2, c, w_mod,
      jnp.asarray(fm, bf16), jnp.asarray(gm, bf16))
```

```python
import functools

import jax
import jax.numpy as jnp
import numpy as np
from jax.experimental import pallas as pl
from jax.experimental.pallas import tpu as pltpu

S, D, FF = 2048, 640, 1536
CH = 128
NCH = S // CH
BM = 256
NG = S // BM
FC = 512
NFC = FF // FC
EPS = 1e-5
NSL = 3
NOS = 2
KPAD = 64
RB = 8
LSPL = 4
NPRO = 15
T0 = 6
f32, bf16 = jnp.float32, jnp.bfloat16


def _dft_consts():
    f = np.concatenate([np.arange(0, CH, 2), np.arange(1, CH, 2)])
    n = np.arange(CH)
    th = np.pi * (2 * f[:, None] + 1) * n[None, :] / (2 * CH)
    fm = np.concatenate([np.cos(th), -np.sin(th)], axis=0)
    gm = fm.T / CH
    return fm.astype(np.float32), gm.astype(np.float32)


def _schedule():
    done, touched = set(), set()

    def mk(u, j):
        s = u + j
        src = s + 1 if s in touched else 0
        touched.add(s)
        done.add((u, j))
        return (u, j, s + 1, src)

    pro = [mk(u, j) for _, u, j in sorted((u + j, u, j) for u in range(4) for j in range(4))[:NPRO]]
    t_reg = (NCH * (NCH + 1) // 2 - len(pro) - T0) // 5
    table = []
    for i in range(1, 7):
        n = 2 * i + 4
        avail = sorted((u + j, u, j) for u in range(n) for j in range(n) if u + j < NCH and (u, j) not in done)
        table.append([mk(u, j) for _, u, j in avail[:(T0 if i == 1 else t_reg)]])
        assert len(table[-1]) == (T0 if i == 1 else t_reg)
        assert all((u, s - u) in done for s in range(n) for u in range(s + 1))
    assert len(done) == NCH * (NCH + 1) // 2
    return pro, table


PRO_TERMS, TABLE = _schedule()
T_SLOTS = len(TABLE[1])


def _kernel(q_hbm, k_hbm, v_hbm, sk_hbm, ssm_hbm, dd_hbm, w1_hbm, w3_hbm, w2_hbm, c_hbm, wm_hbm, fm_hbm, gm_hbm,
            o_hbm,
            mod_s, skt_s, q_s, k_s, v_s, ssm_s, wm_s, w1_s, w3_s, w2_s,
            xf, hf, pp, kv_s, yy_s, h2_s, x1_s, xn_s, o_s, fm_s, gm_s, sk_s, dd_s, c_s, tbl, sems, osems):
    step = pl.program_id(0)

    def al(x, m):
        return x if isinstance(x, int) else pl.multiple_of(x, m)

    S_G0, S_G1, S_WMA, S_WMB, S_FA, S_FB, S_FC, S_FD, S_GRP = range(9)

    def sem_conv(g):
        return sems.at[{0: S_G0, 1: S_G1, 2: S_FD}[g] if isinstance(g, int) and g < 3 else S_GRP + g - 3]

    def sem_q(g):
        return sems.at[{0: S_WMA, 1: S_WMA, 2: S_FD}[g] if isinstance(g, int) and g < 3 else S_GRP + g - 3]

    def cp_q(g):
        return pltpu.make_async_copy(q_hbm.at[0, pl.ds(g * BM, BM), :], q_s.at[g], sem_q(g))

    def cp_k(g):
        if isinstance(g, int) and g == 0:
            return pltpu.make_async_copy(k_hbm.at[0, pl.ds(0, BM), :], k_s.at[0, pl.ds(KPAD, BM), :], sem_conv(g))
        return pltpu.make_async_copy(k_hbm.at[0, pl.ds(al(g * BM - 16, 16), BM + 16), :],
                                     k_s.at[g, pl.ds(KPAD - 16, BM + 16), :], sem_conv(g))

    def cp_v(g):
        return pltpu.make_async_copy(v_hbm.at[0, pl.ds(g * BM, BM), :], v_s.at[g], sem_conv(g))

    def cp_s(g):
        return pltpu.make_async_copy(ssm_hbm.at[:, pl.ds(g * BM, BM)], ssm_s.at[g], sem_conv(g))

    def cp_wm(p0, n):
        return pltpu.make_async_copy(wm_hbm.at[:, pl.ds(p0 * D, n * D)], wm_s.at[:, pl.ds(p0 * D, n * D)],
                                     sems.at[{0: S_WMA, 3: S_WMB, 5: S_FD}[p0]])

    def cp_w1(c):
        return pltpu.make_async_copy(w1_hbm.at[:, pl.ds(c * FC, FC)], w1_s.at[:, pl.ds(c * FC, FC)],
                                     sems.at[(S_FA, S_FB, S_FD)[c]])

    def cp_w3(c):
        return pltpu.make_async_copy(w3_hbm.at[:, pl.ds(c * FC, FC)], w3_s.at[:, pl.ds(c * FC, FC)],
                                     sems.at[(S_FB, S_FC, S_FD)[c]])

    def cp_w2(c):
        return pltpu.make_async_copy(w2_hbm.at[pl.ds(c * FC, FC), :], w2_s.at[pl.ds(c * FC, FC), :],
                                     sems.at[(S_FC, S_FC, S_FD)[c]])

    def cp_small():
        pairs = [(fm_hbm, fm_s), (sk_hbm, sk_s), (dd_hbm, dd_s), (gm_hbm, gm_s), (c_hbm, c_s)]
        return [pltpu.make_async_copy(a, b, sems.at[S_G0]) for a, b in pairs]

    def cp_conv(g):
        return [cp_s(g), cp_k(g), cp_v(g)]

    def cp_o(g, oslot, r0=0, n=BM, sem=None):
        return pltpu.make_async_copy(o_s.at[oslot, pl.ds(r0, n), :], o_hbm.at[0, pl.ds(al(g * BM + r0, 16), n), :],
                                     osems.at[oslot if sem is None else sem])

    def start(*cs):
        for c_ in cs:
            c_.start()

    def wait(*cs):
        for c_ in cs:
            c_.wait()

    def run(tasks):
        for t in tasks:
            t()

    def kv_chunk(g, h):
        r = h * CH
        kw = k_s[g, KPAD - 16 + r:KPAD + r + CH, :].astype(f32)
        ks = kw[16:, :] * skt_s[0:1, :]
        for j in range(1, 4):
            ks = ks + kw[16 - j:16 - j + CH, :] * skt_s[j:j + 1, :]
        kv_s[r:r + CH, :] = (ks * v_s[g, r:r + CH, :].astype(f32)).astype(bf16)

    def x_dot(g, h):
        xf[2 * g + h] = jnp.dot(fm_s[...], kv_s[h * CH:(h + 1) * CH, :], preferred_element_type=f32)

    def h_dot(g, h):
        hf[2 * g + h] = jax.lax.dot_general(fm_s[...], ssm_s[g, :, h * CH:(h + 1) * CH], (((1,), (1,)), ((), ())),
                                            preferred_element_type=f32)

    def fwd_tasks(g):
        part = functools.partial
        return [part(h_dot, g, 0), part(h_dot, g, 1), part(kv_chunk, g, 0), part(x_dot, g, 0),
                part(kv_chunk, g, 1), part(x_dot, g, 1)]

    def term_piece(u, j, dst, src, r):
        xr = xf[u, r:r + RB, :]; xi = xf[u, CH + r:CH + r + RB, :]
        hr = hf[j, r:r + RB, :]; hi = hf[j, CH + r:CH + r + RB, :]
        pr = pp[src, r:r + RB, :]; pi = pp[src, CH + r:CH + r + RB, :]
        nr = pr + (xr * hr - xi * hi)
        ni = pi + (xr * hi + xi * hr)
        pp[dst, r:r + RB, :] = nr
        pp[dst, CH + r:CH + r + RB, :] = ni

    def static_terms(terms):
        for term in terms:
            for r in range(0, CH, RB):
                term_piece(*term, r)

    def table_piece(row, t, r):
        b = (row * T_SLOTS + t) * 4
        term_piece(tbl[b], tbl[b + 1], tbl[b + 2], tbl[b + 3], r)

    def table_tasks(row, nterms, nparts):
        ts = [functools.partial(table_piece, row, t, r) for t in range(nterms) for r in range(0, CH, RB)]
        return [ts[len(ts) * k // nparts:len(ts) * (k + 1) // nparts] for k in range(nparts)]

    def yy_piece(g, h, r):
        n = 2 * g + h
        cre = pp[n + 1, r:r + 16, :]; pim = pp[n, CH + r:CH + r + 16, :]
        cim = pp[n + 1, CH + r:CH + r + 16, :]; pre = pp[n, r:r + 16, :]
        if r < CH // 2:
            a = cre - pim; b = cim + pre
        else:
            a = cre + pim; b = cim - pre
        yy_s[h, r:r + 16, :] = a.astype(bf16)
        yy_s[h, CH + r:CH + r + 16, :] = b.astype(bf16)

    def inv_dot(slot, h):
        x1_s[slot, h * CH:(h + 1) * CH, :] = jnp.dot(gm_s[...], yy_s[h], preferred_element_type=f32)

    def inverse(g, slot):
        for h in range(2):
            for r in range(0, CH, 16):
                yy_piece(g, h, r)
            inv_dot(slot, h)

    def _ln(x):
        m = jnp.mean(x, axis=-1, keepdims=True)
        xc = x - m
        v = jnp.mean(xc * xc, axis=-1, keepdims=True)
        return xc * jax.lax.rsqrt(v + EPS)

    def mod_vec(p):
        return mod_s[0:1, p * D:(p + 1) * D]

    def mix(g, slot, r, n):
        x = q_s[g, r:r + n, :].astype(f32)
        x1 = x + (_ln(x) * mod_vec(1) + mod_vec(0)) * x1_s[slot, r:r + n, :]
        x1_s[slot, r:r + n, :] = x1
        return _ln(x1)

    def adaln(g, slot):
        h2_s[slot] = (mix(g, slot, 0, BM) * mod_vec(4) + mod_vec(3)).astype(bf16)

    def mod_part(p):
        c = c_s[...].astype(f32)
        sc = (c * jax.nn.sigmoid(c)).astype(bf16)
        mod_s[:, p * D:(p + 1) * D] = jnp.dot(jnp.broadcast_to(sc, (8, D)), wm_s[:, p * D:(p + 1) * D],
                                              preferred_element_type=f32)

    class Ffn:
        def __init__(self, slot):
            self.slot = slot
            self.h2 = h2_s[slot]
            self.acc = None

        def g(self, c):
            self.gate = jnp.dot(self.h2, w1_s[:, c * FC:(c + 1) * FC], preferred_element_type=f32)

        def u(self, c):
            up = jnp.dot(self.h2, w3_s[:, c * FC:(c + 1) * FC], preferred_element_type=f32)
            hg = 0.5 * self.gate
            self.hh = ((hg + hg * jnp.tanh(hg)) * up).astype(bf16)

        def d(self, c, hh=None):
            hh = self.hh if hh is None else hh
            p = jnp.dot(hh, w2_s[c * FC:(c + 1) * FC, :], preferred_element_type=f32)
            self.acc = p if self.acc is None else self.acc + p

        def out(self, g, oslot):
            o_s[oslot] = (x1_s[self.slot] + mod_vec(5) * self.acc).astype(bf16)
            cp_o(g, oslot).start()

    @pl.when(step == 0)
    def _():
        smalls = cp_small()
        start(cp_s(0), *smalls, cp_k(0), cp_v(0), *cp_conv(1), cp_q(0), cp_q(1))
        start(cp_wm(0, 3), cp_wm(3, 2))
        start(cp_w1(0), cp_w3(0), cp_w1(1), cp_w3(1), cp_w2(0), cp_w2(1), *cp_conv(2))
        start(cp_w1(2), cp_w3(2), cp_w2(2), cp_wm(5, 1), cp_q(2))
        for g in range(3, NG):
            start(*cp_conv(g), cp_q(g))
        for i, row in enumerate(TABLE):
            for t, term in enumerate(row):
                for e in range(4):
                    tbl[(i * T_SLOTS + t) * 4 + e] = jnp.int32(term[e])
        pp[0] = jnp.zeros(pp.shape[1:], f32)
        k_s[0, KPAD - 16:KPAD, :] = jnp.zeros((16, D), bf16)

        wait(*smalls, *cp_conv(0))
        skt_s[0:4, :] = sk_s[...].astype(f32)
        run(fwd_tasks(0))
        hf[0, 0:CH, :] = hf[0, 0:CH, :] + dd_s[...].astype(f32).reshape(1, D)
        static_terms(PRO_TERMS[:3])
        inverse(0, 0)
        wait(*cp_conv(1))
        run(fwd_tasks(1))
        static_terms(PRO_TERMS[3:10])
        inverse(1, 1)
        static_terms(PRO_TERMS[10:12])

        wait(cp_wm(0, 3), cp_q(0), cp_q(1))
        for p in (2, 1, 0):
            mod_part(p)
        ga = mod_s[:, 2 * D:3 * D]
        mod_s[:, 0:D] = ga * mod_s[:, 0:D]
        mod_s[:, D:2 * D] = ga * (1.0 + mod_s[:, D:2 * D])
        for g in range(2):
            for r in range(0, BM, 64):
                xn_s[g, r:r + 64, :] = mix(g, g, r, 64)
        static_terms(PRO_TERMS[12:])
        wait(cp_wm(3, 2))
        mod_part(4)
        mod_s[:, 4 * D:5 * D] = 1.0 + mod_s[:, 4 * D:5 * D]
        mod_part(3)
        for g in range(2):
            for r in range(0, BM, 64):
                h2_s[g, r:r + 64, :] = (xn_s[g, r:r + 64, :] * mod_vec(4) + mod_vec(3)).astype(bf16)

        fa, fb = Ffn(0), Ffn(1)
        wait(cp_w1(0))
        fa.g(0); fb.g(0)
        wait(cp_w3(0), cp_w1(1))
        fa.u(0); fb.u(0)
        ha0, hb0 = fa.hh, fb.hh
        fa.g(1); fb.g(1)
        wait(cp_w3(1), cp_w2(0), cp_w2(1))
        fa.u(1); fb.u(1)
        fa.d(0, ha0); fb.d(0, hb0); fa.d(1); fb.d(1)
        wait(cp_w1(2), cp_w3(2), cp_w2(2), cp_q(2), cp_wm(5, 1), *cp_conv(2))
        cs = table_tasks(0, T0, 3)
        mod_part(5)
        run(fwd_tasks(2)); fa.g(2); run(cs[0]); fa.u(2); run(cs[1]); fb.g(2); run(cs[2]); fb.u(2)
        inverse(2, 2); adaln(2, 2)
        fa.d(2); fa.out(0, 0); fb.d(2); fb.out(1, 1)

    gi = step + 1

    @pl.when(jnp.logical_and(step >= 1, step <= NG - 3))
    def _():
        g = gi + 1
        wait(cp_o(gi - 2, jax.lax.rem(gi, NOS)), *cp_conv(g), cp_q(g))
        nxt = jax.lax.rem(g, NSL)
        cs = table_tasks(gi - 1, T_SLOTS, 7)
        f = Ffn(jax.lax.rem(gi, NSL))
        f.g(0); run(fwd_tasks(g)); run(cs[0])
        f.u(0); run(cs[1])
        f.d(0); run(cs[2])
        f.g(1); run(cs[3])
        f.u(1); run(cs[4])
        f.d(1); run(cs[5])
        f.g(2); run(cs[6])
        f.u(2); inverse(g, nxt); adaln(g, nxt)
        f.d(2)
        f.out(gi, jax.lax.rem(gi, NOS))

    @pl.when(step == NG - 2)
    def _():
        g = NG - 1
        slot, oslot = g % NSL, g % NOS
        cp_o(g - 2, oslot).wait()
        f = Ffn(slot)
        for c in range(NFC - 1):
            f.g(c); f.u(c); f.d(c)
        f.g(NFC - 1); f.u(NFC - 1)
        n = BM // LSPL
        for k in range(LSPL):
            rows = slice(k * n, (k + 1) * n)
            p = jnp.dot(f.hh[rows], w2_s[(NFC - 1) * FC:, :], preferred_element_type=f32)
            o_s[oslot, rows, :] = (x1_s[slot, rows, :] + mod_vec(5) * (f.acc[rows] + p)).astype(bf16)
            cp_o(g, oslot, k * n, n, sem=NOS).start()
        cp_o(g - 1, (g - 1) % NOS).wait()
        for k in range(LSPL):
            cp_o(g, oslot, k * n, n, sem=NOS).wait()


@jax.jit
def pallas_adaLN_cond__ssm_conv_h3__glu_gated_swiglu__prompt_kernel(
    A_q: jax.Array,
    A_k: jax.Array,
    A_v: jax.Array,
    A_shift_k: jax.Array,
    A_ssm_k: jax.Array,
    A_ssm_D: jax.Array,
    B_x: jax.Array,
    B_w1: jax.Array,
    B_w3: jax.Array,
    B_w2: jax.Array,
    c: jax.Array,
    w_mod: jax.Array,
):
    fm, gm = _dft_consts()
    any_spec = pl.BlockSpec(memory_space=pl.ANY)
    vm = pltpu.VMEM
    scratch = [
        vm((8, 6 * D), f32), vm((8, D), f32),
        vm((NG, BM, D), bf16), vm((NG, KPAD + BM, D), bf16), vm((NG, BM, D), bf16),
        vm((NG, D, BM), bf16), vm((D, 6 * D), bf16),
        vm((D, FF), bf16), vm((D, FF), bf16), vm((FF, D), bf16),
        vm((NCH, 2 * CH, D), f32), vm((NCH, 2 * CH, D), f32), vm((NCH + 1, 2 * CH, D), f32),
        vm((BM, D), bf16), vm((2, 2 * CH, D), bf16),
        vm((NSL, BM, D), bf16), vm((NSL, BM, D), f32), vm((2, BM, D), f32), vm((NOS, BM, D), bf16),
        vm((2 * CH, CH), bf16), vm((CH, 2 * CH), bf16), vm((4, D), bf16), vm((D,), bf16), vm((1, D), bf16),
        pltpu.SMEM((len(TABLE) * T_SLOTS * 4,), jnp.int32),
        pltpu.SemaphoreType.DMA((8 + NG - 3,)),
        pltpu.SemaphoreType.DMA((NOS + 1,)),
    ]
    return pl.pallas_call(
        _kernel,
        grid=(NG - 1,),
        in_specs=[any_spec] * 13,
        out_specs=any_spec,
        out_shape=jax.ShapeDtypeStruct((1, S, D), bf16),
        scratch_shapes=scratch,
        compiler_params=pltpu.CompilerParams(dimension_semantics=("arbitrary",),
                                             vmem_limit_bytes=110 * 1024 * 1024),
    )(A_q, A_k, A_v, A_shift_k.T, A_ssm_k, A_ssm_D, B_w1, B_w3, B_w2, c, w_mod,
      jnp.asarray(fm, bf16), jnp.asarray(gm, bf16))
```

```python
import functools

import jax
import jax.numpy as jnp
import numpy as np
from jax.experimental import pallas as pl
from jax.experimental.pallas import tpu as pltpu

S, D, FF = 2048, 640, 1536
CH = 128
NCH = S // CH
BM = 256
NG = S // BM
FC = 512
NFC = FF // FC
EPS = 1e-5
NSL = 3
NOS = 2
KPAD = 64
RB = 8
LSPL = 4
NPRO = 15
T0 = 6
f32, bf16 = jnp.float32, jnp.bfloat16


def _schedule():
    done, touched = set(), set()

    def mk(u, j):
        s = u + j
        src = s + 1 if s in touched else 0
        touched.add(s)
        done.add((u, j))
        return (u, j, s + 1, src)

    pro = [mk(u, j) for _, u, j in sorted((u + j, u, j) for u in range(4) for j in range(4))[:NPRO]]
    t_reg = (NCH * (NCH + 1) // 2 - len(pro) - T0) // 5
    table = []
    for i in range(1, 7):
        n = 2 * i + 4
        avail = sorted((u + j, u, j) for u in range(n) for j in range(n) if u + j < NCH and (u, j) not in done)
        table.append([mk(u, j) for _, u, j in avail[:(T0 if i == 1 else t_reg)]])
        assert len(table[-1]) == (T0 if i == 1 else t_reg)
        assert all((u, s - u) in done for s in range(n) for u in range(s + 1))
    assert len(done) == NCH * (NCH + 1) // 2
    return pro, table


PRO_TERMS, TABLE = _schedule()
T_SLOTS = len(TABLE[1])


def _kernel(q_hbm, k_hbm, v_hbm, sk_hbm, ssm_hbm, dd_hbm, w1_hbm, w3_hbm, w2_hbm, c_hbm, wm_hbm,
            o_hbm,
            mod_s, skt_s, q_s, k_s, v_s, ssm_s, wm_s, w1_s, w3_s, w2_s,
            xf, hf, pp, kv_s, yy_s, h2_s, x1_s, xn_s, o_s, fm_s, gm_s, sk_s, dd_s, c_s, tbl, sems, osems):
    step = pl.program_id(0)

    def al(x, m):
        return x if isinstance(x, int) else pl.multiple_of(x, m)

    S_G0, S_G1, S_WMA, S_CB, S_SB, S_FA0, S_FA1, S_FB, S_FC, S_FD, S_GRP = range(11)

    def sem_conv(g):
        return sems.at[{0: S_G0, 1: S_G1, 2: S_FD}[g] if isinstance(g, int) and g < 3 else S_GRP + g - 3]

    def sem_q(g):
        return sems.at[{0: S_WMA, 1: S_WMA, 2: S_FD}[g] if isinstance(g, int) and g < 3 else S_GRP + g - 3]

    def cp_q(g):
        return pltpu.make_async_copy(q_hbm.at[0, pl.ds(g * BM, BM), :], q_s.at[g], sem_q(g))

    def cp_k(g):
        if isinstance(g, int) and g == 0:
            return pltpu.make_async_copy(k_hbm.at[0, pl.ds(0, BM), :], k_s.at[0, pl.ds(KPAD, BM), :], sem_conv(g))
        return pltpu.make_async_copy(k_hbm.at[0, pl.ds(al(g * BM - 16, 16), BM + 16), :],
                                     k_s.at[g, pl.ds(KPAD - 16, BM + 16), :], sem_conv(g))

    def cp_v(g):
        return pltpu.make_async_copy(v_hbm.at[0, pl.ds(g * BM, BM), :], v_s.at[g], sem_conv(g))

    def cp_s(g):
        return pltpu.make_async_copy(ssm_hbm.at[:, pl.ds(g * BM, BM)], ssm_s.at[g], sem_conv(g))

    def cp_wm(p0, n):
        return pltpu.make_async_copy(wm_hbm.at[:, pl.ds(p0 * D, n * D)], wm_s.at[:, pl.ds(p0 * D, n * D)],
                                     sems.at[{0: S_WMA, 3: S_SB, 4: S_CB, 5: S_FD}[p0]])

    def cp_w1(c):
        return pltpu.make_async_copy(w1_hbm.at[:, pl.ds(c * FC, FC)], w1_s.at[:, pl.ds(c * FC, FC)],
                                     sems.at[(None, S_FB, S_FD)[c]])

    def cp_w1_half(h):
        return pltpu.make_async_copy(w1_hbm.at[:, pl.ds(h * FC // 2, FC // 2)], w1_s.at[:, pl.ds(h * FC // 2, FC // 2)],
                                     sems.at[(S_FA0, S_FA1)[h]])

    def cp_w3(c):
        return pltpu.make_async_copy(w3_hbm.at[:, pl.ds(c * FC, FC)], w3_s.at[:, pl.ds(c * FC, FC)],
                                     sems.at[(S_FB, S_FC, S_FD)[c]])

    def cp_w2(c):
        return pltpu.make_async_copy(w2_hbm.at[pl.ds(c * FC, FC), :], w2_s.at[pl.ds(c * FC, FC), :],
                                     sems.at[(S_FC, S_FC, S_FD)[c]])

    def cp_small():
        pairs = [(sk_hbm, sk_s), (dd_hbm, dd_s), (c_hbm, c_s)]
        return [pltpu.make_async_copy(a, b, sems.at[S_G0]) for a, b in pairs]

    def cp_conv(g):
        return [cp_s(g), cp_k(g), cp_v(g)]

    def cp_o(g, oslot, r0=0, n=BM, sem=None):
        return pltpu.make_async_copy(o_s.at[oslot, pl.ds(r0, n), :], o_hbm.at[0, pl.ds(al(g * BM + r0, 16), n), :],
                                     osems.at[oslot if sem is None else sem])

    def start(*cs):
        for c_ in cs:
            c_.start()

    def wait(*cs):
        for c_ in cs:
            c_.wait()

    def run(tasks):
        for t in tasks:
            t()

    def kv_chunk(g, h):
        r = h * CH
        kw = k_s[g, KPAD - 16 + r:KPAD + r + CH, :].astype(f32)
        ks = kw[16:, :] * skt_s[0:1, :]
        for j in range(1, 4):
            ks = ks + kw[16 - j:16 - j + CH, :] * skt_s[j:j + 1, :]
        kv_s[r:r + CH, :] = (ks * v_s[g, r:r + CH, :].astype(f32)).astype(bf16)

    def x_dot(g, h):
        xf[2 * g + h] = jnp.dot(fm_s[...], kv_s[h * CH:(h + 1) * CH, :], preferred_element_type=f32)

    def h_dot(g, h):
        hf[2 * g + h] = jax.lax.dot_general(fm_s[...], ssm_s[g, :, h * CH:(h + 1) * CH], (((1,), (1,)), ((), ())),
                                            preferred_element_type=f32)

    def fwd_tasks(g):
        part = functools.partial
        return [part(h_dot, g, 0), part(h_dot, g, 1), part(kv_chunk, g, 0), part(x_dot, g, 0),
                part(kv_chunk, g, 1), part(x_dot, g, 1)]

    def term_piece(u, j, dst, src, r):
        xr = xf[u, r:r + RB, :]; xi = xf[u, CH + r:CH + r + RB, :]
        hr = hf[j, r:r + RB, :]; hi = hf[j, CH + r:CH + r + RB, :]
        pr = pp[src, r:r + RB, :]; pi = pp[src, CH + r:CH + r + RB, :]
        nr = pr + (xr * hr - xi * hi)
        ni = pi + (xr * hi + xi * hr)
        pp[dst, r:r + RB, :] = nr
        pp[dst, CH + r:CH + r + RB, :] = ni

    def static_terms(terms):
        for term in terms:
            for r in range(0, CH, RB):
                term_piece(*term, r)

    def table_piece(row, t, r):
        b = (row * T_SLOTS + t) * 4
        term_piece(tbl[b], tbl[b + 1], tbl[b + 2], tbl[b + 3], r)

    def table_tasks(row, nterms, nparts):
        ts = [functools.partial(table_piece, row, t, r) for t in range(nterms) for r in range(0, CH, RB)]
        return [ts[len(ts) * k // nparts:len(ts) * (k + 1) // nparts] for k in range(nparts)]

    def yy_piece(g, h, r):
        n = 2 * g + h
        cre = pp[n + 1, r:r + 16, :]; pim = pp[n, CH + r:CH + r + 16, :]
        cim = pp[n + 1, CH + r:CH + r + 16, :]; pre = pp[n, r:r + 16, :]
        if r < CH // 2:
            a = cre - pim; b = cim + pre
        else:
            a = cre + pim; b = cim - pre
        yy_s[h, r:r + 16, :] = a.astype(bf16)
        yy_s[h, CH + r:CH + r + 16, :] = b.astype(bf16)

    def inv_dot(slot, h):
        x1_s[slot, h * CH:(h + 1) * CH, :] = jnp.dot(gm_s[...], yy_s[h], preferred_element_type=f32)

    def inverse(g, slot):
        for h in range(2):
            for r in range(0, CH, 16):
                yy_piece(g, h, r)
            inv_dot(slot, h)

    def _ln(x):
        m = jnp.mean(x, axis=-1, keepdims=True)
        xc = x - m
        v = jnp.mean(xc * xc, axis=-1, keepdims=True)
        return xc * jax.lax.rsqrt(v + EPS)

    def mod_vec(p):
        return mod_s[0:1, p * D:(p + 1) * D]

    def mix(g, slot, r, n):
        x = q_s[g, r:r + n, :].astype(f32)
        x1 = x + (_ln(x) * mod_vec(1) + mod_vec(0)) * x1_s[slot, r:r + n, :]
        x1_s[slot, r:r + n, :] = x1
        return _ln(x1)

    def adaln(g, slot):
        h2_s[slot] = (mix(g, slot, 0, BM) * mod_vec(4) + mod_vec(3)).astype(bf16)

    def mod_part(p):
        c = c_s[...].astype(f32)
        sc = (c * jax.nn.sigmoid(c)).astype(bf16)
        mod_s[:, p * D:(p + 1) * D] = jnp.dot(jnp.broadcast_to(sc, (8, D)), wm_s[:, p * D:(p + 1) * D],
                                              preferred_element_type=f32)

    class Ffn:
        def __init__(self, slot):
            self.slot = slot
            self.h2 = h2_s[slot]
            self.acc = None

        def g(self, c):
            self.gate = jnp.dot(self.h2, w1_s[:, c * FC:(c + 1) * FC], preferred_element_type=f32)

        def u(self, c):
            up = jnp.dot(self.h2, w3_s[:, c * FC:(c + 1) * FC], preferred_element_type=f32)
            hg = 0.5 * self.gate
            self.hh = ((hg + hg * jnp.tanh(hg)) * up).astype(bf16)

        def d(self, c, hh=None):
            hh = self.hh if hh is None else hh
            p = jnp.dot(hh, w2_s[c * FC:(c + 1) * FC, :], preferred_element_type=f32)
            self.acc = p if self.acc is None else self.acc + p

        def out(self, g, oslot):
            o_s[oslot] = (x1_s[self.slot] + mod_vec(5) * self.acc).astype(bf16)
            cp_o(g, oslot).start()

    @pl.when(step == 0)
    def _():
        smalls = cp_small()
        start(cp_s(0), *smalls, cp_k(0), cp_v(0), *cp_conv(1), cp_q(0), cp_q(1))
        start(cp_wm(0, 3), cp_wm(4, 1), cp_wm(3, 1))
        start(cp_w1_half(0), cp_w1_half(1), cp_w3(0), cp_w1(1), cp_w3(1), cp_w2(0), cp_w2(1), *cp_conv(2))
        start(cp_w1(2), cp_w3(2), cp_w2(2), cp_wm(5, 1), cp_q(2))
        for g in range(3, NG):
            start(*cp_conv(g), cp_q(g))
        for i, row in enumerate(TABLE):
            for t, term in enumerate(row):
                for e in range(4):
                    tbl[(i * T_SLOTS + t) * 4 + e] = jnp.int32(term[e])
        pp[0] = jnp.zeros(pp.shape[1:], f32)
        k_s[0, KPAD - 16:KPAD, :] = jnp.zeros((16, D), bf16)

        row = jax.lax.broadcasted_iota(jnp.int32, (2 * CH, CH), 0)
        col = jax.lax.broadcasted_iota(jnp.int32, (2 * CH, CH), 1)
        fi = row % CH
        freq = jnp.where(fi < CH // 2, 2 * fi, 2 * fi - (CH - 1))
        ang = ((2 * freq + 1) * col + jnp.where(row >= CH, CH, 0)) % (4 * CH)
        fmv = jnp.cos(ang.astype(f32) * (np.pi / (2 * CH)))
        fm_s[...] = fmv.astype(bf16)
        gm_s[...] = (fmv.T * (1.0 / CH)).astype(bf16)

        wait(*smalls, *cp_conv(0))
        skt_s[0:4, :] = sk_s[...].astype(f32)
        run(fwd_tasks(0))
        hf[0, 0:CH, :] = hf[0, 0:CH, :] + dd_s[...].astype(f32).reshape(1, D)
        static_terms(PRO_TERMS[:3])
        inverse(0, 0)
        wait(*cp_conv(1))
        run(fwd_tasks(1))
        static_terms(PRO_TERMS[3:10])
        inverse(1, 1)
        static_terms(PRO_TERMS[10:12])

        wait(cp_wm(0, 3), cp_q(0), cp_q(1))
        for p in (2, 1, 0):
            mod_part(p)
        ga = mod_s[:, 2 * D:3 * D]
        mod_s[:, 0:D] = ga * mod_s[:, 0:D]
        mod_s[:, D:2 * D] = ga * (1.0 + mod_s[:, D:2 * D])
        for g in range(2):
            for r in range(0, BM, 64):
                xn_s[g, r:r + 64, :] = mix(g, g, r, 64)
        static_terms(PRO_TERMS[12:])
        wait(cp_wm(4, 1))
        mod_part(4)
        mod_s[:, 4 * D:5 * D] = 1.0 + mod_s[:, 4 * D:5 * D]
        wait(cp_wm(3, 1))
        mod_part(3)
        for g in range(2):
            for r in range(0, BM, 64):
                h2_s[g, r:r + 64, :] = (xn_s[g, r:r + 64, :] * mod_vec(4) + mod_vec(3)).astype(bf16)

        fa, fb = Ffn(0), Ffn(1)
        halves = []
        for h in range(2):
            wait(cp_w1_half(h))
            w = w1_s[:, h * FC // 2:(h + 1) * FC // 2]
            halves.append([jnp.dot(f_.h2, w, preferred_element_type=f32) for f_ in (fa, fb)])
        fa.gate = jnp.concatenate([halves[0][0], halves[1][0]], axis=1)
        fb.gate = jnp.concatenate([halves[0][1], halves[1][1]], axis=1)
        wait(cp_w3(0), cp_w1(1))
        fa.u(0); fb.u(0)
        ha0, hb0 = fa.hh, fb.hh
        fa.g(1); fb.g(1)
        wait(cp_w3(1), cp_w2(0), cp_w2(1))
        fa.u(1); fb.u(1)
        fa.d(0, ha0); fb.d(0, hb0); fa.d(1); fb.d(1)
        wait(cp_w1(2), cp_w3(2), cp_w2(2), cp_q(2), cp_wm(5, 1), *cp_conv(2))
        cs = table_tasks(0, T0, 3)
        mod_part(5)
        run(fwd_tasks(2)); fa.g(2); run(cs[0]); fa.u(2); run(cs[1]); fb.g(2); run(cs[2]); fb.u(2)
        inverse(2, 2); adaln(2, 2)
        fa.d(2); fa.out(0, 0); fb.d(2); fb.out(1, 1)

    gi = step + 1

    @pl.when(jnp.logical_and(step >= 1, step <= NG - 3))
    def _():
        g = gi + 1
        wait(cp_o(gi - 2, jax.lax.rem(gi, NOS)), *cp_conv(g), cp_q(g))
        nxt = jax.lax.rem(g, NSL)
        cs = table_tasks(gi - 1, T_SLOTS, 7)
        f = Ffn(jax.lax.rem(gi, NSL))
        f.g(0); run(fwd_tasks(g)); run(cs[0])
        f.u(0); run(cs[1])
        f.d(0); run(cs[2])
        f.g(1); run(cs[3])
        f.u(1); run(cs[4])
        f.d(1); run(cs[5])
        f.g(2); run(cs[6])
        f.u(2); inverse(g, nxt); adaln(g, nxt)
        f.d(2)
        f.out(gi, jax.lax.rem(gi, NOS))

    @pl.when(step == NG - 2)
    def _():
        g = NG - 1
        slot, oslot = g % NSL, g % NOS
        cp_o(g - 2, oslot).wait()
        f = Ffn(slot)
        for c in range(NFC - 1):
            f.g(c); f.u(c); f.d(c)
        f.g(NFC - 1); f.u(NFC - 1)
        n = BM // LSPL
        for k in range(LSPL):
            rows = slice(k * n, (k + 1) * n)
            p = jnp.dot(f.hh[rows], w2_s[(NFC - 1) * FC:, :], preferred_element_type=f32)
            o_s[oslot, rows, :] = (x1_s[slot, rows, :] + mod_vec(5) * (f.acc[rows] + p)).astype(bf16)
            cp_o(g, oslot, k * n, n, sem=NOS).start()
        cp_o(g - 1, (g - 1) % NOS).wait()
        for k in range(LSPL):
            cp_o(g, oslot, k * n, n, sem=NOS).wait()


@jax.jit
def pallas_adaLN_cond__ssm_conv_h3__glu_gated_swiglu__prompt_kernel(
    A_q: jax.Array,
    A_k: jax.Array,
    A_v: jax.Array,
    A_shift_k: jax.Array,
    A_ssm_k: jax.Array,
    A_ssm_D: jax.Array,
    B_x: jax.Array,
    B_w1: jax.Array,
    B_w3: jax.Array,
    B_w2: jax.Array,
    c: jax.Array,
    w_mod: jax.Array,
):
    any_spec = pl.BlockSpec(memory_space=pl.ANY)
    vm = pltpu.VMEM
    scratch = [
        vm((8, 6 * D), f32), vm((8, D), f32),
        vm((NG, BM, D), bf16), vm((NG, KPAD + BM, D), bf16), vm((NG, BM, D), bf16),
        vm((NG, D, BM), bf16), vm((D, 6 * D), bf16),
        vm((D, FF), bf16), vm((D, FF), bf16), vm((FF, D), bf16),
        vm((NCH, 2 * CH, D), f32), vm((NCH, 2 * CH, D), f32), vm((NCH + 1, 2 * CH, D), f32),
        vm((BM, D), bf16), vm((2, 2 * CH, D), bf16),
        vm((NSL, BM, D), bf16), vm((NSL, BM, D), f32), vm((2, BM, D), f32), vm((NOS, BM, D), bf16),
        vm((2 * CH, CH), bf16), vm((CH, 2 * CH), bf16), vm((4, D), bf16), vm((D,), bf16), vm((1, D), bf16),
        pltpu.SMEM((len(TABLE) * T_SLOTS * 4,), jnp.int32),
        pltpu.SemaphoreType.DMA((10 + NG - 3,)),
        pltpu.SemaphoreType.DMA((NOS + 1,)),
    ]
    return pl.pallas_call(
        _kernel,
        grid=(NG - 1,),
        in_specs=[any_spec] * 11,
        out_specs=any_spec,
        out_shape=jax.ShapeDtypeStruct((1, S, D), bf16),
        scratch_shapes=scratch,
        compiler_params=pltpu.CompilerParams(dimension_semantics=("arbitrary",),
                                             vmem_limit_bytes=110 * 1024 * 1024),
    )(A_q, A_k, A_v, A_shift_k.T, A_ssm_k, A_ssm_D, B_w1, B_w3, B_w2, c, w_mod)
```

```python
import functools

import jax
import jax.numpy as jnp
import numpy as np
from jax.experimental import pallas as pl
from jax.experimental.pallas import tpu as pltpu

S, D, FF = 2048, 640, 1536
CH = 128
NCH = S // CH
BM = 256
NG = S // BM
FC = 512
NFC = FF // FC
EPS = 1e-5
NSL = 3
NOS = 2
KPAD = 64
RB = 8
LSPL = 8
NPRO = 15
T0 = 6
f32, bf16 = jnp.float32, jnp.bfloat16


def _schedule():
    done, touched = set(), set()

    def mk(u, j):
        s = u + j
        src = s + 1 if s in touched else 0
        touched.add(s)
        done.add((u, j))
        return (u, j, s + 1, src)

    pro = [mk(u, j) for _, u, j in sorted((u + j, u, j) for u in range(4) for j in range(4))[:NPRO]]
    t_reg = (NCH * (NCH + 1) // 2 - len(pro) - T0) // 5
    table = []
    for i in range(1, 7):
        n = 2 * i + 4
        avail = sorted((u + j, u, j) for u in range(n) for j in range(n) if u + j < NCH and (u, j) not in done)
        table.append([mk(u, j) for _, u, j in avail[:(T0 if i == 1 else t_reg)]])
        assert len(table[-1]) == (T0 if i == 1 else t_reg)
        assert all((u, s - u) in done for s in range(n) for u in range(s + 1))
    assert len(done) == NCH * (NCH + 1) // 2
    return pro, table


PRO_TERMS, TABLE = _schedule()
T_SLOTS = len(TABLE[1])


def _kernel(q_hbm, k_hbm, v_hbm, sk_hbm, ssm_hbm, dd_hbm, w1_hbm, w3_hbm, w2_hbm, c_hbm, wm_hbm,
            o_hbm,
            mod_s, skt_s, q_s, k_s, v_s, ssm_s, wm_s, w1_s, w3_s, w2_s,
            xf, hf, pp, kv_s, yy_s, h2_s, x1_s, xn_s, o_s, fm_s, gm_s, sk_s, dd_s, c_s, tbl, sems, osems):
    step = pl.program_id(0)

    def al(x, m):
        return x if isinstance(x, int) else pl.multiple_of(x, m)

    S_G0, S_G1, S_WMA, S_CB, S_SB, S_FA0, S_FA1, S_FB, S_FC, S_FD, S_GRP = range(11)

    def sem_conv(g):
        return sems.at[{0: S_G0, 1: S_G1, 2: S_FD}[g] if isinstance(g, int) and g < 3 else S_GRP + g - 3]

    def sem_q(g):
        return sems.at[{0: S_WMA, 1: S_WMA, 2: S_FD}[g] if isinstance(g, int) and g < 3 else S_GRP + g - 3]

    def cp_q(g):
        return pltpu.make_async_copy(q_hbm.at[0, pl.ds(g * BM, BM), :], q_s.at[g], sem_q(g))

    def cp_k(g):
        if isinstance(g, int) and g == 0:
            return pltpu.make_async_copy(k_hbm.at[0, pl.ds(0, BM), :], k_s.at[0, pl.ds(KPAD, BM), :], sem_conv(g))
        return pltpu.make_async_copy(k_hbm.at[0, pl.ds(al(g * BM - 16, 16), BM + 16), :],
                                     k_s.at[g, pl.ds(KPAD - 16, BM + 16), :], sem_conv(g))

    def cp_v(g):
        return pltpu.make_async_copy(v_hbm.at[0, pl.ds(g * BM, BM), :], v_s.at[g], sem_conv(g))

    def cp_s(g):
        return pltpu.make_async_copy(ssm_hbm.at[:, pl.ds(g * BM, BM)], ssm_s.at[g], sem_conv(g))

    def cp_wm(p0, n):
        return pltpu.make_async_copy(wm_hbm.at[:, pl.ds(p0 * D, n * D)], wm_s.at[:, pl.ds(p0 * D, n * D)],
                                     sems.at[{0: S_WMA, 3: S_SB, 4: S_CB, 5: S_FD}[p0]])

    def cp_w1(c):
        return pltpu.make_async_copy(w1_hbm.at[:, pl.ds(c * FC, FC)], w1_s.at[:, pl.ds(c * FC, FC)],
                                     sems.at[(None, S_FB, S_FD)[c]])

    def cp_w1_half(h):
        return pltpu.make_async_copy(w1_hbm.at[:, pl.ds(h * FC // 2, FC // 2)], w1_s.at[:, pl.ds(h * FC // 2, FC // 2)],
                                     sems.at[(S_FA0, S_FA1)[h]])

    def cp_w3(c):
        return pltpu.make_async_copy(w3_hbm.at[:, pl.ds(c * FC, FC)], w3_s.at[:, pl.ds(c * FC, FC)],
                                     sems.at[(S_FB, S_FC, S_FD)[c]])

    def cp_w2(c):
        return pltpu.make_async_copy(w2_hbm.at[pl.ds(c * FC, FC), :], w2_s.at[pl.ds(c * FC, FC), :],
                                     sems.at[(S_FC, S_FC, S_FD)[c]])

    def cp_small():
        pairs = [(sk_hbm, sk_s), (dd_hbm, dd_s), (c_hbm, c_s)]
        return [pltpu.make_async_copy(a, b, sems.at[S_G0]) for a, b in pairs]

    def cp_conv(g):
        return [cp_s(g), cp_k(g), cp_v(g)]

    def cp_o(g, oslot, r0=0, n=BM, sem=None):
        return pltpu.make_async_copy(o_s.at[oslot, pl.ds(r0, n), :], o_hbm.at[0, pl.ds(al(g * BM + r0, 16), n), :],
                                     osems.at[oslot if sem is None else sem])

    def start(*cs):
        for c_ in cs:
            c_.start()

    def wait(*cs):
        for c_ in cs:
            c_.wait()

    def run(tasks):
        for t in tasks:
            t()

    def kv_chunk(g, h):
        r = h * CH
        kw = k_s[g, KPAD - 16 + r:KPAD + r + CH, :].astype(f32)
        ks = kw[16:, :] * skt_s[0:1, :]
        for j in range(1, 4):
            ks = ks + kw[16 - j:16 - j + CH, :] * skt_s[j:j + 1, :]
        kv_s[r:r + CH, :] = (ks * v_s[g, r:r + CH, :].astype(f32)).astype(bf16)

    def x_dot(g, h):
        xf[2 * g + h] = jnp.dot(fm_s[...], kv_s[h * CH:(h + 1) * CH, :], preferred_element_type=f32)

    def h_dot(g, h):
        hf[2 * g + h] = jax.lax.dot_general(fm_s[...], ssm_s[g, :, h * CH:(h + 1) * CH], (((1,), (1,)), ((), ())),
                                            preferred_element_type=f32)

    def fwd_tasks(g):
        part = functools.partial
        return [part(h_dot, g, 0), part(h_dot, g, 1), part(kv_chunk, g, 0), part(x_dot, g, 0),
                part(kv_chunk, g, 1), part(x_dot, g, 1)]

    def term_piece(u, j, dst, src, r):
        xr = xf[u, r:r + RB, :]; xi = xf[u, CH + r:CH + r + RB, :]
        hr = hf[j, r:r + RB, :]; hi = hf[j, CH + r:CH + r + RB, :]
        pr = pp[src, r:r + RB, :]; pi = pp[src, CH + r:CH + r + RB, :]
        nr = pr + (xr * hr - xi * hi)
        ni = pi + (xr * hi + xi * hr)
        pp[dst, r:r + RB, :] = nr
        pp[dst, CH + r:CH + r + RB, :] = ni

    def static_terms(terms):
        for term in terms:
            for r in range(0, CH, RB):
                term_piece(*term, r)

    def table_piece(row, t, r):
        b = (row * T_SLOTS + t) * 4
        term_piece(tbl[b], tbl[b + 1], tbl[b + 2], tbl[b + 3], r)

    def table_tasks(row, nterms, nparts):
        ts = [functools.partial(table_piece, row, t, r) for t in range(nterms) for r in range(0, CH, RB)]
        return [ts[len(ts) * k // nparts:len(ts) * (k + 1) // nparts] for k in range(nparts)]

    def yy_piece(g, h, r):
        n = 2 * g + h
        cre = pp[n + 1, r:r + 16, :]; pim = pp[n, CH + r:CH + r + 16, :]
        cim = pp[n + 1, CH + r:CH + r + 16, :]; pre = pp[n, r:r + 16, :]
        if r < CH // 2:
            a = cre - pim; b = cim + pre
        else:
            a = cre + pim; b = cim - pre
        yy_s[h, r:r + 16, :] = a.astype(bf16)
        yy_s[h, CH + r:CH + r + 16, :] = b.astype(bf16)

    def inv_dot(slot, h):
        x1_s[slot, h * CH:(h + 1) * CH, :] = jnp.dot(gm_s[...], yy_s[h], preferred_element_type=f32)

    def inverse(g, slot):
        for h in range(2):
            for r in range(0, CH, 16):
                yy_piece(g, h, r)
            inv_dot(slot, h)

    def _ln(x):
        m = jnp.mean(x, axis=-1, keepdims=True)
        xc = x - m
        v = jnp.mean(xc * xc, axis=-1, keepdims=True)
        return xc * jax.lax.rsqrt(v + EPS)

    def mod_vec(p):
        return mod_s[0:1, p * D:(p + 1) * D]

    def mix(g, slot, r, n):
        x = q_s[g, r:r + n, :].astype(f32)
        x1 = x + (_ln(x) * mod_vec(1) + mod_vec(0)) * x1_s[slot, r:r + n, :]
        x1_s[slot, r:r + n, :] = x1
        return _ln(x1)

    def adaln(g, slot):
        h2_s[slot] = (mix(g, slot, 0, BM) * mod_vec(4) + mod_vec(3)).astype(bf16)

    def mod_part(p):
        c = c_s[...].astype(f32)
        sc = (c * jax.nn.sigmoid(c)).astype(bf16)
        mod_s[:, p * D:(p + 1) * D] = jnp.dot(jnp.broadcast_to(sc, (8, D)), wm_s[:, p * D:(p + 1) * D],
                                              preferred_element_type=f32)

    class Ffn:
        def __init__(self, slot):
            self.slot = slot
            self.h2 = h2_s[slot]
            self.acc = None

        def g(self, c):
            self.gate = jnp.dot(self.h2, w1_s[:, c * FC:(c + 1) * FC], preferred_element_type=f32)

        def u(self, c):
            up = jnp.dot(self.h2, w3_s[:, c * FC:(c + 1) * FC], preferred_element_type=f32)
            hg = 0.5 * self.gate
            self.hh = ((hg + hg * jnp.tanh(hg)) * up).astype(bf16)

        def d(self, c, hh=None):
            hh = self.hh if hh is None else hh
            p = jnp.dot(hh, w2_s[c * FC:(c + 1) * FC, :], preferred_element_type=f32)
            self.acc = p if self.acc is None else self.acc + p

        def out(self, g, oslot):
            o_s[oslot] = (x1_s[self.slot] + mod_vec(5) * self.acc).astype(bf16)
            cp_o(g, oslot).start()

    @pl.when(step == 0)
    def _():
        smalls = cp_small()
        start(cp_s(0), *smalls, cp_k(0), cp_v(0), *cp_conv(1), cp_q(0), cp_q(1))
        start(cp_wm(0, 3), cp_wm(4, 1), cp_wm(3, 1))
        start(cp_w1_half(0), cp_w1_half(1), cp_w3(0), cp_w1(1), cp_w3(1), cp_w2(0), cp_w2(1), *cp_conv(2))
        start(cp_w1(2), cp_w3(2), cp_w2(2), cp_wm(5, 1), cp_q(2))
        for g in range(3, NG):
            start(*cp_conv(g), cp_q(g))
        for i, row in enumerate(TABLE):
            for t, term in enumerate(row):
                for e in range(4):
                    tbl[(i * T_SLOTS + t) * 4 + e] = jnp.int32(term[e])
        pp[0] = jnp.zeros(pp.shape[1:], f32)
        k_s[0, KPAD - 16:KPAD, :] = jnp.zeros((16, D), bf16)

        row = jax.lax.broadcasted_iota(jnp.int32, (2 * CH, CH), 0)
        col = jax.lax.broadcasted_iota(jnp.int32, (2 * CH, CH), 1)
        fi = row % CH
        freq = jnp.where(fi < CH // 2, 2 * fi, 2 * fi - (CH - 1))
        ang = ((2 * freq + 1) * col + jnp.where(row >= CH, CH, 0)) % (4 * CH)
        fmv = jnp.cos(ang.astype(f32) * (np.pi / (2 * CH)))
        fm_s[...] = fmv.astype(bf16)
        gm_s[...] = (fmv.T * (1.0 / CH)).astype(bf16)

        wait(*smalls, *cp_conv(0))
        skt_s[0:4, :] = sk_s[...].astype(f32)
        run(fwd_tasks(0))
        hf[0, 0:CH, :] = hf[0, 0:CH, :] + dd_s[...].astype(f32).reshape(1, D)
        static_terms(PRO_TERMS[:3])
        inverse(0, 0)
        wait(*cp_conv(1))
        run(fwd_tasks(1))
        static_terms(PRO_TERMS[3:10])
        inverse(1, 1)
        static_terms(PRO_TERMS[10:12])

        wait(cp_wm(0, 3), cp_q(0), cp_q(1))
        for p in (2, 1, 0):
            mod_part(p)
        ga = mod_s[:, 2 * D:3 * D]
        mod_s[:, 0:D] = ga * mod_s[:, 0:D]
        mod_s[:, D:2 * D] = ga * (1.0 + mod_s[:, D:2 * D])
        for g in range(2):
            for r in range(0, BM, 64):
                xn_s[g, r:r + 64, :] = mix(g, g, r, 64)
        static_terms(PRO_TERMS[12:])
        wait(cp_wm(4, 1))
        mod_part(4)
        mod_s[:, 4 * D:5 * D] = 1.0 + mod_s[:, 4 * D:5 * D]
        wait(cp_wm(3, 1))
        mod_part(3)
        for g in range(2):
            for r in range(0, BM, 64):
                h2_s[g, r:r + 64, :] = (xn_s[g, r:r + 64, :] * mod_vec(4) + mod_vec(3)).astype(bf16)

        fa, fb = Ffn(0), Ffn(1)
        halves = []
        for h in range(2):
            wait(cp_w1_half(h))
            w = w1_s[:, h * FC // 2:(h + 1) * FC // 2]
            halves.append([jnp.dot(f_.h2, w, preferred_element_type=f32) for f_ in (fa, fb)])
        fa.gate = jnp.concatenate([halves[0][0], halves[1][0]], axis=1)
        fb.gate = jnp.concatenate([halves[0][1], halves[1][1]], axis=1)
        wait(cp_w3(0), cp_w1(1))
        fa.u(0); fb.u(0)
        ha0, hb0 = fa.hh, fb.hh
        fa.g(1); fb.g(1)
        wait(cp_w3(1), cp_w2(0), cp_w2(1))
        fa.u(1); fb.u(1)
        fa.d(0, ha0); fb.d(0, hb0); fa.d(1); fb.d(1)
        wait(cp_w1(2), cp_w3(2), cp_w2(2), cp_q(2), cp_wm(5, 1), *cp_conv(2))
        cs = table_tasks(0, T0, 3)
        mod_part(5)
        run(fwd_tasks(2)); fa.g(2); run(cs[0]); fa.u(2); run(cs[1]); fb.g(2); run(cs[2]); fb.u(2)
        inverse(2, 2); adaln(2, 2)
        fa.d(2); fa.out(0, 0); fb.d(2); fb.out(1, 1)

    gi = step + 1

    @pl.when(jnp.logical_and(step >= 1, step <= NG - 3))
    def _():
        g = gi + 1
        wait(cp_o(gi - 2, jax.lax.rem(gi, NOS)), *cp_conv(g), cp_q(g))
        nxt = jax.lax.rem(g, NSL)
        cs = table_tasks(gi - 1, T_SLOTS, 7)
        f = Ffn(jax.lax.rem(gi, NSL))
        f.g(0); run(fwd_tasks(g)); run(cs[0])
        f.u(0); h0 = f.hh; run(cs[1])
        f.g(1); run(cs[2])
        f.u(1); h1 = f.hh; run(cs[3])
        f.g(2); run(cs[4])
        f.u(2); run(cs[5])
        f.d(0, h0); run(cs[6])
        f.d(1, h1); inverse(g, nxt); adaln(g, nxt)
        f.d(2)
        f.out(gi, jax.lax.rem(gi, NOS))

    @pl.when(step == NG - 2)
    def _():
        g = NG - 1
        slot, oslot = g % NSL, g % NOS
        cp_o(g - 2, oslot).wait()
        f = Ffn(slot)
        for c in range(NFC - 1):
            f.g(c); f.u(c); f.d(c)
        f.g(NFC - 1); f.u(NFC - 1)
        n = BM // LSPL
        for k in range(LSPL):
            rows = slice(k * n, (k + 1) * n)
            p = jnp.dot(f.hh[rows], w2_s[(NFC - 1) * FC:, :], preferred_element_type=f32)
            o_s[oslot, rows, :] = (x1_s[slot, rows, :] + mod_vec(5) * (f.acc[rows] + p)).astype(bf16)
            cp_o(g, oslot, k * n, n, sem=NOS).start()
        cp_o(g - 1, (g - 1) % NOS).wait()
        for k in range(LSPL):
            cp_o(g, oslot, k * n, n, sem=NOS).wait()


@jax.jit
def pallas_adaLN_cond__ssm_conv_h3__glu_gated_swiglu__prompt_kernel(
    A_q: jax.Array,
    A_k: jax.Array,
    A_v: jax.Array,
    A_shift_k: jax.Array,
    A_ssm_k: jax.Array,
    A_ssm_D: jax.Array,
    B_x: jax.Array,
    B_w1: jax.Array,
    B_w3: jax.Array,
    B_w2: jax.Array,
    c: jax.Array,
    w_mod: jax.Array,
):
    any_spec = pl.BlockSpec(memory_space=pl.ANY)
    vm = pltpu.VMEM
    scratch = [
        vm((8, 6 * D), f32), vm((8, D), f32),
        vm((NG, BM, D), bf16), vm((NG, KPAD + BM, D), bf16), vm((NG, BM, D), bf16),
        vm((NG, D, BM), bf16), vm((D, 6 * D), bf16),
        vm((D, FF), bf16), vm((D, FF), bf16), vm((FF, D), bf16),
        vm((NCH, 2 * CH, D), f32), vm((NCH, 2 * CH, D), f32), vm((NCH + 1, 2 * CH, D), f32),
        vm((BM, D), bf16), vm((2, 2 * CH, D), bf16),
        vm((NSL, BM, D), bf16), vm((NSL, BM, D), f32), vm((2, BM, D), f32), vm((NOS, BM, D), bf16),
        vm((2 * CH, CH), bf16), vm((CH, 2 * CH), bf16), vm((4, D), bf16), vm((D,), bf16), vm((1, D), bf16),
        pltpu.SMEM((len(TABLE) * T_SLOTS * 4,), jnp.int32),
        pltpu.SemaphoreType.DMA((10 + NG - 3,)),
        pltpu.SemaphoreType.DMA((NOS + 1,)),
    ]
    return pl.pallas_call(
        _kernel,
        grid=(NG - 1,),
        in_specs=[any_spec] * 11,
        out_specs=any_spec,
        out_shape=jax.ShapeDtypeStruct((1, S, D), bf16),
        scratch_shapes=scratch,
        compiler_params=pltpu.CompilerParams(dimension_semantics=("arbitrary",),
                                             vmem_limit_bytes=110 * 1024 * 1024),
    )(A_q, A_k, A_v, A_shift_k.T, A_ssm_k, A_ssm_D, B_w1, B_w3, B_w2, c, w_mod)
```

```python
import functools

import jax
import jax.numpy as jnp
import numpy as np
from jax.experimental import pallas as pl
from jax.experimental.pallas import tpu as pltpu

S, D, FF = 2048, 640, 1536
CH = 128
NCH = S // CH
BM = 256
NG = S // BM
FC = 512
NFC = FF // FC
EPS = 1e-5
NSL = 3
NOS = 2
KPAD = 64
RB = 8
LSPL = 8
NPRO = 15
T0 = 6
f32, bf16 = jnp.float32, jnp.bfloat16


def _schedule():
    done, touched = set(), set()

    def mk(u, j):
        s = u + j
        src = s + 1 if s in touched else 0
        touched.add(s)
        done.add((u, j))
        return (u, j, s + 1, src)

    pro = [mk(u, j) for _, u, j in sorted((u + j, u, j) for u in range(4) for j in range(4))[:NPRO]]
    t_reg = (NCH * (NCH + 1) // 2 - len(pro) - T0) // 5
    table = []
    for i in range(1, 7):
        n = 2 * i + 4
        avail = sorted((u + j, u, j) for u in range(n) for j in range(n) if u + j < NCH and (u, j) not in done)
        table.append([mk(u, j) for _, u, j in avail[:(T0 if i == 1 else t_reg)]])
        assert len(table[-1]) == (T0 if i == 1 else t_reg)
        assert all((u, s - u) in done for s in range(n) for u in range(s + 1))
    assert len(done) == NCH * (NCH + 1) // 2
    return pro, table


PRO_TERMS, TABLE = _schedule()
T_SLOTS = len(TABLE[1])


def _kernel(q_hbm, k_hbm, v_hbm, sk_hbm, ssm_hbm, dd_hbm, w1_hbm, w3_hbm, w2_hbm, c_hbm, wm_hbm,
            o_hbm,
            mod_s, skt_s, q_s, k_s, v_s, ssm_s, wm_s, w1_s, w3_s, w2_s,
            xf, hf, pp, kv_s, yy_s, h2_s, x1_s, xn_s, o_s, fm_s, gm_s, sk_s, dd_s, c_s, tbl, sems, osems):
    step = pl.program_id(0)

    def al(x, m):
        return x if isinstance(x, int) else pl.multiple_of(x, m)

    S_G0, S_G1, S_WMA, S_CB, S_SB, S_FA0, S_FA1, S_FB, S_FC, S_FD, S_GRP = range(11)

    def sem_conv(g):
        return sems.at[{0: S_G0, 1: S_G1, 2: S_FD}[g] if isinstance(g, int) and g < 3 else S_GRP + g - 3]

    def sem_q(g):
        return sems.at[{0: S_WMA, 1: S_WMA, 2: S_FD}[g] if isinstance(g, int) and g < 3 else S_GRP + g - 3]

    def cp_q(g):
        return pltpu.make_async_copy(q_hbm.at[0, pl.ds(g * BM, BM), :], q_s.at[g], sem_q(g))

    def cp_k(g):
        if isinstance(g, int) and g == 0:
            return pltpu.make_async_copy(k_hbm.at[0, pl.ds(0, BM), :], k_s.at[0, pl.ds(KPAD, BM), :], sem_conv(g))
        return pltpu.make_async_copy(k_hbm.at[0, pl.ds(al(g * BM - 16, 16), BM + 16), :],
                                     k_s.at[g, pl.ds(KPAD - 16, BM + 16), :], sem_conv(g))

    def cp_v(g):
        return pltpu.make_async_copy(v_hbm.at[0, pl.ds(g * BM, BM), :], v_s.at[g], sem_conv(g))

    def cp_s(g):
        return pltpu.make_async_copy(ssm_hbm.at[:, pl.ds(g * BM, BM)], ssm_s.at[g], sem_conv(g))

    def cp_wm(p0, n):
        return pltpu.make_async_copy(wm_hbm.at[:, pl.ds(p0 * D, n * D)], wm_s.at[:, pl.ds(p0 * D, n * D)],
                                     sems.at[{0: S_WMA, 3: S_SB, 4: S_CB, 5: S_FD}[p0]])

    def cp_w1(c):
        return pltpu.make_async_copy(w1_hbm.at[:, pl.ds(c * FC, FC)], w1_s.at[:, pl.ds(c * FC, FC)],
                                     sems.at[(None, S_FB, S_FD)[c]])

    def cp_w1_half(h):
        return pltpu.make_async_copy(w1_hbm.at[:, pl.ds(h * FC // 2, FC // 2)], w1_s.at[:, pl.ds(h * FC // 2, FC // 2)],
                                     sems.at[(S_FA0, S_FA1)[h]])

    def cp_w3(c):
        return pltpu.make_async_copy(w3_hbm.at[:, pl.ds(c * FC, FC)], w3_s.at[:, pl.ds(c * FC, FC)],
                                     sems.at[(S_FB, S_FC, S_FD)[c]])

    def cp_w2(c):
        return pltpu.make_async_copy(w2_hbm.at[pl.ds(c * FC, FC), :], w2_s.at[pl.ds(c * FC, FC), :],
                                     sems.at[(S_FC, S_FC, S_FD)[c]])

    def cp_small():
        pairs = [(sk_hbm, sk_s), (dd_hbm, dd_s), (c_hbm, c_s)]
        return [pltpu.make_async_copy(a, b, sems.at[S_G0]) for a, b in pairs]

    def cp_conv(g):
        return [cp_s(g), cp_k(g), cp_v(g)]

    def cp_o(g, oslot, r0=0, n=BM, sem=None):
        return pltpu.make_async_copy(o_s.at[oslot, pl.ds(r0, n), :], o_hbm.at[0, pl.ds(al(g * BM + r0, 16), n), :],
                                     osems.at[oslot if sem is None else sem])

    def start(*cs):
        for c_ in cs:
            c_.start()

    def wait(*cs):
        for c_ in cs:
            c_.wait()

    def run(tasks):
        for t in tasks:
            t()

    def kv_chunk(g, h):
        r = h * CH
        kw = k_s[g, KPAD - 16 + r:KPAD + r + CH, :].astype(f32)
        ks = kw[16:, :] * skt_s[0:1, :]
        for j in range(1, 4):
            ks = ks + kw[16 - j:16 - j + CH, :] * skt_s[j:j + 1, :]
        kv_s[r:r + CH, :] = (ks * v_s[g, r:r + CH, :].astype(f32)).astype(bf16)

    def x_dot(g, h):
        xf[2 * g + h] = jnp.dot(fm_s[...], kv_s[h * CH:(h + 1) * CH, :], preferred_element_type=f32)

    def h_dot(g, h):
        hf[2 * g + h] = jax.lax.dot_general(fm_s[...], ssm_s[g, :, h * CH:(h + 1) * CH], (((1,), (1,)), ((), ())),
                                            preferred_element_type=f32)

    def fwd(g, h):
        kv_chunk(g, h)
        x_dot(g, h)
        h_dot(g, h)

    def fwd_group(g):
        h_dot(g, 0); h_dot(g, 1)
        for h in range(2):
            kv_chunk(g, h)
            x_dot(g, h)

    def term_piece(u, j, dst, src, r):
        xr = xf[u, r:r + RB, :]; xi = xf[u, CH + r:CH + r + RB, :]
        hr = hf[j, r:r + RB, :]; hi = hf[j, CH + r:CH + r + RB, :]
        pr = pp[src, r:r + RB, :]; pi = pp[src, CH + r:CH + r + RB, :]
        nr = pr + (xr * hr - xi * hi)
        ni = pi + (xr * hi + xi * hr)
        pp[dst, r:r + RB, :] = nr
        pp[dst, CH + r:CH + r + RB, :] = ni

    def static_terms(terms):
        for term in terms:
            for r in range(0, CH, RB):
                term_piece(*term, r)

    def table_piece(row, t, r):
        b = (row * T_SLOTS + t) * 4
        term_piece(tbl[b], tbl[b + 1], tbl[b + 2], tbl[b + 3], r)

    def table_tasks(row, nterms, nparts):
        ts = [functools.partial(table_piece, row, t, r) for t in range(nterms) for r in range(0, CH, RB)]
        return [ts[len(ts) * k // nparts:len(ts) * (k + 1) // nparts] for k in range(nparts)]

    def yy_piece(g, h, r):
        n = 2 * g + h
        cre = pp[n + 1, r:r + 16, :]; pim = pp[n, CH + r:CH + r + 16, :]
        cim = pp[n + 1, CH + r:CH + r + 16, :]; pre = pp[n, r:r + 16, :]
        if r < CH // 2:
            a = cre - pim; b = cim + pre
        else:
            a = cre + pim; b = cim - pre
        yy_s[h, r:r + 16, :] = a.astype(bf16)
        yy_s[h, CH + r:CH + r + 16, :] = b.astype(bf16)

    def inv_dot(slot, h):
        x1_s[slot, h * CH:(h + 1) * CH, :] = jnp.dot(gm_s[...], yy_s[h], preferred_element_type=f32)

    def inverse(g, slot):
        for h in range(2):
            for r in range(0, CH, 16):
                yy_piece(g, h, r)
            inv_dot(slot, h)

    def _ln(x):
        m = jnp.mean(x, axis=-1, keepdims=True)
        xc = x - m
        v = jnp.mean(xc * xc, axis=-1, keepdims=True)
        return xc * jax.lax.rsqrt(v + EPS)

    def mod_vec(p):
        return mod_s[0:1, p * D:(p + 1) * D]

    def mix(g, slot, r, n):
        x = q_s[g, r:r + n, :].astype(f32)
        x1 = x + (_ln(x) * mod_vec(1) + mod_vec(0)) * x1_s[slot, r:r + n, :]
        x1_s[slot, r:r + n, :] = x1
        return _ln(x1)

    def adaln(g, slot):
        h2_s[slot] = (mix(g, slot, 0, BM) * mod_vec(4) + mod_vec(3)).astype(bf16)

    def mod_part(p):
        c = c_s[...].astype(f32)
        sc = (c * jax.nn.sigmoid(c)).astype(bf16)
        mod_s[:, p * D:(p + 1) * D] = jnp.dot(jnp.broadcast_to(sc, (8, D)), wm_s[:, p * D:(p + 1) * D],
                                              preferred_element_type=f32)

    class Ffn:
        def __init__(self, slot):
            self.slot = slot
            self.h2 = h2_s[slot]
            self.acc = None

        def g(self, c):
            self.gate = jnp.dot(self.h2, w1_s[:, c * FC:(c + 1) * FC], preferred_element_type=f32)

        def g_half(self, c, h):
            lo = c * FC + h * (FC // 2)
            part = jnp.dot(self.h2, w1_s[:, lo:lo + FC // 2], preferred_element_type=f32)
            self.gate = part if h == 0 else jnp.concatenate([self.gate, part], axis=1)

        def u(self, c):
            up = jnp.dot(self.h2, w3_s[:, c * FC:(c + 1) * FC], preferred_element_type=f32)
            hg = 0.5 * self.gate
            self.hh = ((hg + hg * jnp.tanh(hg)) * up).astype(bf16)

        def d(self, c, hh=None):
            hh = self.hh if hh is None else hh
            p = jnp.dot(hh, w2_s[c * FC:(c + 1) * FC, :], preferred_element_type=f32)
            self.acc = p if self.acc is None else self.acc + p

        def out(self, g, oslot):
            o_s[oslot] = (x1_s[self.slot] + mod_vec(5) * self.acc).astype(bf16)
            cp_o(g, oslot).start()

    @pl.when(step == 0)
    def _():
        smalls = cp_small()
        start(cp_s(0), *smalls, cp_k(0), cp_v(0), *cp_conv(1), cp_q(0), cp_q(1))
        start(cp_wm(0, 3), cp_wm(4, 1), cp_wm(3, 1))
        start(cp_w1_half(0), cp_w1_half(1), cp_w3(0), cp_w1(1), cp_w3(1), cp_w2(0), cp_w2(1), *cp_conv(2))
        start(cp_w1(2), cp_w3(2), cp_w2(2), cp_wm(5, 1), cp_q(2))
        for g in range(3, NG):
            start(*cp_conv(g), cp_q(g))
        for i, row in enumerate(TABLE):
            for t, term in enumerate(row):
                for e in range(4):
                    tbl[(i * T_SLOTS + t) * 4 + e] = jnp.int32(term[e])
        pp[0] = jnp.zeros(pp.shape[1:], f32)
        k_s[0, KPAD - 16:KPAD, :] = jnp.zeros((16, D), bf16)

        row = jax.lax.broadcasted_iota(jnp.int32, (2 * CH, CH), 0)
        col = jax.lax.broadcasted_iota(jnp.int32, (2 * CH, CH), 1)
        fi = row % CH
        freq = jnp.where(fi < CH // 2, 2 * fi, 2 * fi - (CH - 1))
        ang = ((2 * freq + 1) * col + jnp.where(row >= CH, CH, 0)) % (4 * CH)
        fmv = jnp.cos(ang.astype(f32) * (np.pi / (2 * CH)))
        fm_s[...] = fmv.astype(bf16)
        gm_s[...] = (fmv.T * (1.0 / CH)).astype(bf16)

        wait(*smalls, *cp_conv(0))
        skt_s[0:4, :] = sk_s[...].astype(f32)
        fwd_group(0)
        hf[0, 0:CH, :] = hf[0, 0:CH, :] + dd_s[...].astype(f32).reshape(1, D)
        static_terms(PRO_TERMS[:3])
        inverse(0, 0)
        wait(*cp_conv(1))
        fwd_group(1)
        static_terms(PRO_TERMS[3:10])
        inverse(1, 1)
        static_terms(PRO_TERMS[10:12])

        wait(cp_wm(0, 3), cp_q(0), cp_q(1))
        for p in (2, 1, 0):
            mod_part(p)
        ga = mod_s[:, 2 * D:3 * D]
        mod_s[:, 0:D] = ga * mod_s[:, 0:D]
        mod_s[:, D:2 * D] = ga * (1.0 + mod_s[:, D:2 * D])
        for g in range(2):
            for r in range(0, BM, 64):
                xn_s[g, r:r + 64, :] = mix(g, g, r, 64)
        static_terms(PRO_TERMS[12:])
        wait(cp_wm(4, 1))
        mod_part(4)
        mod_s[:, 4 * D:5 * D] = 1.0 + mod_s[:, 4 * D:5 * D]
        wait(cp_wm(3, 1))
        mod_part(3)
        for g in range(2):
            for r in range(0, BM, 64):
                h2_s[g, r:r + 64, :] = (xn_s[g, r:r + 64, :] * mod_vec(4) + mod_vec(3)).astype(bf16)

        fa, fb = Ffn(0), Ffn(1)
        for h in range(2):
            wait(cp_w1_half(h))
            fa.g_half(0, h); fb.g_half(0, h)
        wait(cp_w3(0), cp_w1(1))
        fa.u(0); fb.u(0)
        ha0, hb0 = fa.hh, fb.hh
        fa.g(1); fb.g(1)
        wait(cp_w3(1), cp_w2(0), cp_w2(1))
        fa.u(1); fb.u(1)
        fa.d(0, ha0); fb.d(0, hb0); fa.d(1); fb.d(1)
        wait(cp_w1(2), cp_w3(2), cp_w2(2), cp_q(2), cp_wm(5, 1), *cp_conv(2))
        cs = table_tasks(0, T0, 3)
        mod_part(5)
        fa.g_half(2, 0); fwd(2, 0); fa.g_half(2, 1); fwd(2, 1); run(cs[0]); fb.g(2); run(cs[1]); fa.u(2); run(cs[2]); fb.u(2)
        inverse(2, 2); adaln(2, 2)
        fa.d(2); fa.out(0, 0); fb.d(2); fb.out(1, 1)

    gi = step + 1

    @pl.when(jnp.logical_and(step >= 1, step <= NG - 3))
    def _():
        g = gi + 1
        wait(cp_o(gi - 2, jax.lax.rem(gi, NOS)), *cp_conv(g), cp_q(g))
        nxt = jax.lax.rem(g, NSL)
        cs = table_tasks(gi - 1, T_SLOTS, 7)
        f = Ffn(jax.lax.rem(gi, NSL))
        f.g_half(0, 0); fwd(g, 0); f.g_half(0, 1); fwd(g, 1); run(cs[0])
        f.u(0); h0 = f.hh; run(cs[1])
        f.g(1); run(cs[2])
        f.u(1); h1 = f.hh; run(cs[3])
        f.g(2); run(cs[4])
        f.u(2); run(cs[5])
        f.d(0, h0); run(cs[6])
        f.d(1, h1); inverse(g, nxt); adaln(g, nxt)
        f.d(2)
        f.out(gi, jax.lax.rem(gi, NOS))

    @pl.when(step == NG - 2)
    def _():
        g = NG - 1
        slot, oslot = g % NSL, g % NOS
        cp_o(g - 2, oslot).wait()
        f = Ffn(slot)
        for c in range(NFC - 1):
            f.g(c); f.u(c); f.d(c)
        f.g(NFC - 1); f.u(NFC - 1)
        n = BM // LSPL
        for k in range(LSPL):
            rows = slice(k * n, (k + 1) * n)
            p = jnp.dot(f.hh[rows], w2_s[(NFC - 1) * FC:, :], preferred_element_type=f32)
            o_s[oslot, rows, :] = (x1_s[slot, rows, :] + mod_vec(5) * (f.acc[rows] + p)).astype(bf16)
            cp_o(g, oslot, k * n, n, sem=NOS).start()
        cp_o(g - 1, (g - 1) % NOS).wait()
        for k in range(LSPL):
            cp_o(g, oslot, k * n, n, sem=NOS).wait()


@jax.jit
def pallas_adaLN_cond__ssm_conv_h3__glu_gated_swiglu__prompt_kernel(
    A_q: jax.Array,
    A_k: jax.Array,
    A_v: jax.Array,
    A_shift_k: jax.Array,
    A_ssm_k: jax.Array,
    A_ssm_D: jax.Array,
    B_x: jax.Array,
    B_w1: jax.Array,
    B_w3: jax.Array,
    B_w2: jax.Array,
    c: jax.Array,
    w_mod: jax.Array,
):
    any_spec = pl.BlockSpec(memory_space=pl.ANY)
    vm = pltpu.VMEM
    scratch = [
        vm((8, 6 * D), f32), vm((8, D), f32),
        vm((NG, BM, D), bf16), vm((NG, KPAD + BM, D), bf16), vm((NG, BM, D), bf16),
        vm((NG, D, BM), bf16), vm((D, 6 * D), bf16),
        vm((D, FF), bf16), vm((D, FF), bf16), vm((FF, D), bf16),
        vm((NCH, 2 * CH, D), f32), vm((NCH, 2 * CH, D), f32), vm((NCH + 1, 2 * CH, D), f32),
        vm((BM, D), bf16), vm((2, 2 * CH, D), bf16),
        vm((NSL, BM, D), bf16), vm((NSL, BM, D), f32), vm((2, BM, D), f32), vm((NOS, BM, D), bf16),
        vm((2 * CH, CH), bf16), vm((CH, 2 * CH), bf16), vm((4, D), bf16), vm((D,), bf16), vm((1, D), bf16),
        pltpu.SMEM((len(TABLE) * T_SLOTS * 4,), jnp.int32),
        pltpu.SemaphoreType.DMA((10 + NG - 3,)),
        pltpu.SemaphoreType.DMA((NOS + 1,)),
    ]
    return pl.pallas_call(
        _kernel,
        grid=(NG - 1,),
        in_specs=[any_spec] * 11,
        out_specs=any_spec,
        out_shape=jax.ShapeDtypeStruct((1, S, D), bf16),
        scratch_shapes=scratch,
        compiler_params=pltpu.CompilerParams(dimension_semantics=("arbitrary",),
                                             vmem_limit_bytes=110 * 1024 * 1024),
    )(A_q, A_k, A_v, A_shift_k.T, A_ssm_k, A_ssm_D, B_w1, B_w3, B_w2, c, w_mod)
```

```python
import functools

import jax
import jax.numpy as jnp
import numpy as np
from jax.experimental import pallas as pl
from jax.experimental.pallas import tpu as pltpu

S, D, FF = 2048, 640, 1536
CH = 128
NCH = S // CH
BM = 256
NG = S // BM
FC = 512
NFC = FF // FC
EPS = 1e-5
NSL = 3
NOS = 2
KPAD = 64
RB = 8
LSPL = 8
NPRO = 15
T0 = 6
f32, bf16 = jnp.float32, jnp.bfloat16


def _schedule():
    done, touched = set(), set()

    def mk(u, j):
        s = u + j
        src = s + 1 if s in touched else 0
        touched.add(s)
        done.add((u, j))
        return (u, j, s + 1, src)

    pro = [mk(u, j) for _, u, j in sorted((u + j, u, j) for u in range(4) for j in range(4))[:NPRO]]
    t_reg = (NCH * (NCH + 1) // 2 - len(pro) - T0) // 5
    table = []
    for i in range(1, 7):
        n = 2 * i + 4
        avail = sorted((u + j, u, j) for u in range(n) for j in range(n) if u + j < NCH and (u, j) not in done)
        table.append([mk(u, j) for _, u, j in avail[:(T0 if i == 1 else t_reg)]])
        assert len(table[-1]) == (T0 if i == 1 else t_reg)
        assert all((u, s - u) in done for s in range(n) for u in range(s + 1))
    assert len(done) == NCH * (NCH + 1) // 2
    return pro, table


PRO_TERMS, TABLE = _schedule()
T_SLOTS = len(TABLE[1])


def _kernel(q_hbm, k_hbm, v_hbm, sk_hbm, ssm_hbm, dd_hbm, w1_hbm, w3_hbm, w2_hbm, c_hbm, wm_hbm,
            o_hbm,
            mod_s, skt_s, q_s, k_s, v_s, ssm_s, wm_s, w1_s, w3_s, w2_s,
            xf, hf, pp, kv_s, yy_s, h2_s, x1_s, xn_s, o_s, fm_s, gm_s, sk_s, dd_s, c_s, tbl, sems, osems):
    step = pl.program_id(0)

    def al(x, m):
        return x if isinstance(x, int) else pl.multiple_of(x, m)

    S_G0, S_G1, S_WMA, S_CB, S_SB, S_FA0, S_FA1, S_FB, S_FC, S_FD, S_GRP = range(11)

    def sem_conv(g):
        return sems.at[{0: S_G0, 1: S_G1, 2: S_FD}[g] if isinstance(g, int) and g < 3 else S_GRP + g - 3]

    def sem_q(g):
        return sems.at[{0: S_WMA, 1: S_WMA, 2: S_FD}[g] if isinstance(g, int) and g < 3 else S_GRP + g - 3]

    def cp_q(g):
        return pltpu.make_async_copy(q_hbm.at[0, pl.ds(g * BM, BM), :], q_s.at[g], sem_q(g))

    def cp_k(g):
        if isinstance(g, int) and g == 0:
            return pltpu.make_async_copy(k_hbm.at[0, pl.ds(0, BM), :], k_s.at[0, pl.ds(KPAD, BM), :], sem_conv(g))
        return pltpu.make_async_copy(k_hbm.at[0, pl.ds(al(g * BM - 16, 16), BM + 16), :],
                                     k_s.at[g, pl.ds(KPAD - 16, BM + 16), :], sem_conv(g))

    def cp_v(g):
        return pltpu.make_async_copy(v_hbm.at[0, pl.ds(g * BM, BM), :], v_s.at[g], sem_conv(g))

    def cp_s(g):
        return pltpu.make_async_copy(ssm_hbm.at[:, pl.ds(g * BM, BM)], ssm_s.at[g], sem_conv(g))

    def cp_wm(p0, n):
        return pltpu.make_async_copy(wm_hbm.at[:, pl.ds(p0 * D, n * D)], wm_s.at[:, pl.ds(p0 * D, n * D)],
                                     sems.at[{0: S_WMA, 3: S_SB, 4: S_CB, 5: S_FD}[p0]])

    def cp_w1(c):
        return pltpu.make_async_copy(w1_hbm.at[:, pl.ds(c * FC, FC)], w1_s.at[:, pl.ds(c * FC, FC)],
                                     sems.at[(None, S_FB, S_FD)[c]])

    def cp_w1_half(h):
        return pltpu.make_async_copy(w1_hbm.at[:, pl.ds(h * FC // 2, FC // 2)], w1_s.at[:, pl.ds(h * FC // 2, FC // 2)],
                                     sems.at[(S_FA0, S_FA1)[h]])

    def cp_w3(c):
        return pltpu.make_async_copy(w3_hbm.at[:, pl.ds(c * FC, FC)], w3_s.at[:, pl.ds(c * FC, FC)],
                                     sems.at[(S_FB, S_FC, S_FD)[c]])

    def cp_w2(c):
        return pltpu.make_async_copy(w2_hbm.at[pl.ds(c * FC, FC), :], w2_s.at[pl.ds(c * FC, FC), :],
                                     sems.at[(S_FC, S_FC, S_FD)[c]])

    def cp_small():
        pairs = [(sk_hbm, sk_s), (dd_hbm, dd_s), (c_hbm, c_s)]
        return [pltpu.make_async_copy(a, b, sems.at[S_G0]) for a, b in pairs]

    def cp_conv(g):
        return [cp_s(g), cp_k(g), cp_v(g)]

    def cp_o(g, oslot, r0=0, n=BM, sem=None):
        return pltpu.make_async_copy(o_s.at[oslot, pl.ds(r0, n), :], o_hbm.at[0, pl.ds(al(g * BM + r0, 16), n), :],
                                     osems.at[oslot if sem is None else sem])

    def start(*cs):
        for c_ in cs:
            c_.start()

    def wait(*cs):
        for c_ in cs:
            c_.wait()

    def run(tasks):
        for t in tasks:
            t()

    def kv_chunk(g, h):
        r = h * CH
        kw = k_s[g, KPAD - 16 + r:KPAD + r + CH, :].astype(f32)
        ks = kw[16:, :] * skt_s[0:1, :]
        for j in range(1, 4):
            ks = ks + kw[16 - j:16 - j + CH, :] * skt_s[j:j + 1, :]
        kv_s[r:r + CH, :] = (ks * v_s[g, r:r + CH, :].astype(f32)).astype(bf16)

    def x_dot(g, h):
        xf[2 * g + h] = jnp.dot(fm_s[...], kv_s[h * CH:(h + 1) * CH, :], preferred_element_type=f32)

    def h_dot(g, h):
        hf[2 * g + h] = jax.lax.dot_general(fm_s[...], ssm_s[g, :, h * CH:(h + 1) * CH], (((1,), (1,)), ((), ())),
                                            preferred_element_type=f32)

    def fwd_under(f, c, g):
        f.g_half(c, 0)
        kv_chunk(g, 0); x_dot(g, 0)
        f.g_half(c, 1)
        h_dot(g, 0)
        kv_chunk(g, 1); x_dot(g, 1)
        h_dot(g, 1)

    def fwd_group(g):
        h_dot(g, 0); h_dot(g, 1)
        for h in range(2):
            kv_chunk(g, h)
            x_dot(g, h)

    def term_piece(u, j, dst, src, r):
        xr = xf[u, r:r + RB, :]; xi = xf[u, CH + r:CH + r + RB, :]
        hr = hf[j, r:r + RB, :]; hi = hf[j, CH + r:CH + r + RB, :]
        pr = pp[src, r:r + RB, :]; pi = pp[src, CH + r:CH + r + RB, :]
        nr = pr + (xr * hr - xi * hi)
        ni = pi + (xr * hi + xi * hr)
        pp[dst, r:r + RB, :] = nr
        pp[dst, CH + r:CH + r + RB, :] = ni

    def static_terms(terms):
        for term in terms:
            for r in range(0, CH, RB):
                term_piece(*term, r)

    def table_piece(row, t, r):
        b = (row * T_SLOTS + t) * 4
        term_piece(tbl[b], tbl[b + 1], tbl[b + 2], tbl[b + 3], r)

    def table_tasks(row, nterms, nparts):
        ts = [functools.partial(table_piece, row, t, r) for t in range(nterms) for r in range(0, CH, RB)]
        return [ts[len(ts) * k // nparts:len(ts) * (k + 1) // nparts] for k in range(nparts)]

    def yy_piece(g, h, r):
        n = 2 * g + h
        cre = pp[n + 1, r:r + 16, :]; pim = pp[n, CH + r:CH + r + 16, :]
        cim = pp[n + 1, CH + r:CH + r + 16, :]; pre = pp[n, r:r + 16, :]
        if r < CH // 2:
            a = cre - pim; b = cim + pre
        else:
            a = cre + pim; b = cim - pre
        yy_s[h, r:r + 16, :] = a.astype(bf16)
        yy_s[h, CH + r:CH + r + 16, :] = b.astype(bf16)

    def inv_dot(slot, h):
        x1_s[slot, h * CH:(h + 1) * CH, :] = jnp.dot(gm_s[...], yy_s[h], preferred_element_type=f32)

    def inverse(g, slot):
        for h in range(2):
            for r in range(0, CH, 16):
                yy_piece(g, h, r)
            inv_dot(slot, h)

    def _ln(x):
        m = jnp.mean(x, axis=-1, keepdims=True)
        xc = x - m
        v = jnp.mean(xc * xc, axis=-1, keepdims=True)
        return xc * jax.lax.rsqrt(v + EPS)

    def mod_vec(p):
        return mod_s[0:1, p * D:(p + 1) * D]

    def mix(g, slot, r, n):
        x = q_s[g, r:r + n, :].astype(f32)
        x1 = x + (_ln(x) * mod_vec(1) + mod_vec(0)) * x1_s[slot, r:r + n, :]
        x1_s[slot, r:r + n, :] = x1
        return _ln(x1)

    def adaln(g, slot):
        h2_s[slot] = (mix(g, slot, 0, BM) * mod_vec(4) + mod_vec(3)).astype(bf16)

    def mod_part(p):
        c = c_s[...].astype(f32)
        sc = (c * jax.nn.sigmoid(c)).astype(bf16)
        mod_s[:, p * D:(p + 1) * D] = jnp.dot(jnp.broadcast_to(sc, (8, D)), wm_s[:, p * D:(p + 1) * D],
                                              preferred_element_type=f32)

    class Ffn:
        def __init__(self, slot):
            self.slot = slot
            self.h2 = h2_s[slot]
            self.acc = None

        def g(self, c):
            self.gate = jnp.dot(self.h2, w1_s[:, c * FC:(c + 1) * FC], preferred_element_type=f32)

        def g_half(self, c, h):
            lo = c * FC + h * (FC // 2)
            part = jnp.dot(self.h2, w1_s[:, lo:lo + FC // 2], preferred_element_type=f32)
            self.gate = part if h == 0 else jnp.concatenate([self.gate, part], axis=1)

        def u(self, c):
            up = jnp.dot(self.h2, w3_s[:, c * FC:(c + 1) * FC], preferred_element_type=f32)
            hg = 0.5 * self.gate
            self.hh = ((hg + hg * jnp.tanh(hg)) * up).astype(bf16)

        def d(self, c, hh=None):
            hh = self.hh if hh is None else hh
            p = jnp.dot(hh, w2_s[c * FC:(c + 1) * FC, :], preferred_element_type=f32)
            self.acc = p if self.acc is None else self.acc + p

        def out(self, g, oslot):
            o_s[oslot] = (x1_s[self.slot] + mod_vec(5) * self.acc).astype(bf16)
            cp_o(g, oslot).start()

    @pl.when(step == 0)
    def _():
        smalls = cp_small()
        start(cp_s(0), *smalls, cp_k(0), cp_v(0), *cp_conv(1), cp_q(0), cp_q(1))
        start(cp_wm(0, 3), cp_wm(4, 1), cp_wm(3, 1))
        start(cp_w1_half(0), cp_w1_half(1), cp_w3(0), cp_w1(1), cp_w3(1), cp_w2(0), cp_w2(1), *cp_conv(2))
        start(cp_w1(2), cp_w3(2), cp_w2(2), cp_wm(5, 1), cp_q(2))
        for g in range(3, NG):
            start(*cp_conv(g), cp_q(g))
        for i, row in enumerate(TABLE):
            for t, term in enumerate(row):
                for e in range(4):
                    tbl[(i * T_SLOTS + t) * 4 + e] = jnp.int32(term[e])
        pp[0] = jnp.zeros(pp.shape[1:], f32)
        k_s[0, KPAD - 16:KPAD, :] = jnp.zeros((16, D), bf16)

        row = jax.lax.broadcasted_iota(jnp.int32, (2 * CH, CH), 0)
        col = jax.lax.broadcasted_iota(jnp.int32, (2 * CH, CH), 1)
        fi = row % CH
        freq = jnp.where(fi < CH // 2, 2 * fi, 2 * fi - (CH - 1))
        ang = ((2 * freq + 1) * col + jnp.where(row >= CH, CH, 0)) % (4 * CH)
        fmv = jnp.cos(ang.astype(f32) * (np.pi / (2 * CH)))
        fm_s[...] = fmv.astype(bf16)
        gm_s[...] = (fmv.T * (1.0 / CH)).astype(bf16)

        wait(*smalls, *cp_conv(0))
        skt_s[0:4, :] = sk_s[...].astype(f32)
        fwd_group(0)
        hf[0, 0:CH, :] = hf[0, 0:CH, :] + dd_s[...].astype(f32).reshape(1, D)
        static_terms(PRO_TERMS[:3])
        inverse(0, 0)
        wait(*cp_conv(1))
        fwd_group(1)
        static_terms(PRO_TERMS[3:10])
        inverse(1, 1)
        static_terms(PRO_TERMS[10:12])

        wait(cp_wm(0, 3), cp_q(0), cp_q(1))
        for p in (2, 1, 0):
            mod_part(p)
        ga = mod_s[:, 2 * D:3 * D]
        mod_s[:, 0:D] = ga * mod_s[:, 0:D]
        mod_s[:, D:2 * D] = ga * (1.0 + mod_s[:, D:2 * D])
        for g in range(2):
            for r in range(0, BM, 64):
                xn_s[g, r:r + 64, :] = mix(g, g, r, 64)
        static_terms(PRO_TERMS[12:])
        wait(cp_wm(4, 1))
        mod_part(4)
        mod_s[:, 4 * D:5 * D] = 1.0 + mod_s[:, 4 * D:5 * D]
        wait(cp_wm(3, 1))
        mod_part(3)
        for g in range(2):
            for r in range(0, BM, 64):
                h2_s[g, r:r + 64, :] = (xn_s[g, r:r + 64, :] * mod_vec(4) + mod_vec(3)).astype(bf16)

        fa, fb = Ffn(0), Ffn(1)
        for h in range(2):
            wait(cp_w1_half(h))
            fa.g_half(0, h); fb.g_half(0, h)
        wait(cp_w3(0), cp_w1(1))
        fa.u(0); fb.u(0)
        ha0, hb0 = fa.hh, fb.hh
        fa.g(1); fb.g(1)
        wait(cp_w3(1), cp_w2(0), cp_w2(1))
        fa.u(1); fb.u(1)
        fa.d(0, ha0); fb.d(0, hb0); fa.d(1); fb.d(1)
        wait(cp_w1(2), cp_w3(2), cp_w2(2), cp_q(2), cp_wm(5, 1), *cp_conv(2))
        cs = table_tasks(0, T0, 3)
        fwd_under(fa, 2, 2); mod_part(5); run(cs[0]); fb.g(2); run(cs[1]); fa.u(2); run(cs[2]); fb.u(2)
        inverse(2, 2); adaln(2, 2)
        fa.d(2); fa.out(0, 0); fb.d(2); fb.out(1, 1)

    gi = step + 1

    @pl.when(jnp.logical_and(step >= 1, step <= NG - 3))
    def _():
        g = gi + 1
        wait(cp_o(gi - 2, jax.lax.rem(gi, NOS)), *cp_conv(g), cp_q(g))
        nxt = jax.lax.rem(g, NSL)
        cs = table_tasks(gi - 1, T_SLOTS, 7)
        f = Ffn(jax.lax.rem(gi, NSL))
        fwd_under(f, 0, g); run(cs[0])
        f.u(0); h0 = f.hh; run(cs[1])
        f.g(1); run(cs[2])
        f.u(1); h1 = f.hh; run(cs[3])
        f.g(2); run(cs[4])
        f.u(2); run(cs[5])
        f.d(0, h0); run(cs[6])
        f.d(1, h1); inverse(g, nxt); adaln(g, nxt)
        f.d(2)
        f.out(gi, jax.lax.rem(gi, NOS))

    @pl.when(step == NG - 2)
    def _():
        g = NG - 1
        slot, oslot = g % NSL, g % NOS
        cp_o(g - 2, oslot).wait()
        f = Ffn(slot)
        for c in range(NFC - 1):
            f.g(c); f.u(c); f.d(c)
        f.g(NFC - 1); f.u(NFC - 1)
        n = BM // LSPL
        for k in range(LSPL):
            rows = slice(k * n, (k + 1) * n)
            p = jnp.dot(f.hh[rows], w2_s[(NFC - 1) * FC:, :], preferred_element_type=f32)
            o_s[oslot, rows, :] = (x1_s[slot, rows, :] + mod_vec(5) * (f.acc[rows] + p)).astype(bf16)
            cp_o(g, oslot, k * n, n, sem=NOS).start()
        cp_o(g - 1, (g - 1) % NOS).wait()
        for k in range(LSPL):
            cp_o(g, oslot, k * n, n, sem=NOS).wait()


@jax.jit
def pallas_adaLN_cond__ssm_conv_h3__glu_gated_swiglu__prompt_kernel(
    A_q: jax.Array,
    A_k: jax.Array,
    A_v: jax.Array,
    A_shift_k: jax.Array,
    A_ssm_k: jax.Array,
    A_ssm_D: jax.Array,
    B_x: jax.Array,
    B_w1: jax.Array,
    B_w3: jax.Array,
    B_w2: jax.Array,
    c: jax.Array,
    w_mod: jax.Array,
):
    any_spec = pl.BlockSpec(memory_space=pl.ANY)
    vm = pltpu.VMEM
    scratch = [
        vm((8, 6 * D), f32), vm((8, D), f32),
        vm((NG, BM, D), bf16), vm((NG, KPAD + BM, D), bf16), vm((NG, BM, D), bf16),
        vm((NG, D, BM), bf16), vm((D, 6 * D), bf16),
        vm((D, FF), bf16), vm((D, FF), bf16), vm((FF, D), bf16),
        vm((NCH, 2 * CH, D), f32), vm((NCH, 2 * CH, D), f32), vm((NCH + 1, 2 * CH, D), f32),
        vm((BM, D), bf16), vm((2, 2 * CH, D), bf16),
        vm((NSL, BM, D), bf16), vm((NSL, BM, D), f32), vm((2, BM, D), f32), vm((NOS, BM, D), bf16),
        vm((2 * CH, CH), bf16), vm((CH, 2 * CH), bf16), vm((4, D), bf16), vm((D,), bf16), vm((1, D), bf16),
        pltpu.SMEM((len(TABLE) * T_SLOTS * 4,), jnp.int32),
        pltpu.SemaphoreType.DMA((10 + NG - 3,)),
        pltpu.SemaphoreType.DMA((NOS + 1,)),
    ]
    return pl.pallas_call(
        _kernel,
        grid=(NG - 1,),
        in_specs=[any_spec] * 11,
        out_specs=any_spec,
        out_shape=jax.ShapeDtypeStruct((1, S, D), bf16),
        scratch_shapes=scratch,
        compiler_params=pltpu.CompilerParams(dimension_semantics=("arbitrary",),
                                             vmem_limit_bytes=110 * 1024 * 1024),
    )(A_q, A_k, A_v, A_shift_k.T, A_ssm_k, A_ssm_D, B_w1, B_w3, B_w2, c, w_mod)
```
